```python
import jax
import jax.numpy as jnp

def _softmax(x, axis=-1):
    return jax.nn.softmax(x, axis=axis)

def _gelu(x):
    return jax.nn.gelu(x, approximate=True)

def _silu(x):
    return jax.nn.silu(x)

def _sigmoid(x):
    return jax.nn.sigmoid(x)

def _layernorm(x, axis=-1, eps=1e-05):
    m = jnp.mean(x, axis=axis, keepdims=True)
    v = jnp.var(x, axis=axis, keepdims=True)
    return (x - m) / jnp.sqrt(v + eps)

def _scatter_add(tgt, idx, src, axis=0):
    return tgt.at[idx].add(src)

def _segment_sum(src, seg, n):
    return jax.ops.segment_sum(src, seg, n)

class _Rng:

    def __init__(self, key):
        self._k = key

    def _next(self):
        self._k, sub = jax.random.split(self._k)
        return sub

    def normal(self, shape):
        return jax.random.normal(self._next(), shape, dtype=jnp.bfloat16)

    def randint(self, lo, hi, shape):
        return jax.random.randint(self._next(), shape, lo, hi, dtype=jnp.int32)

    def uniform(self, shape, lo=0.0, hi=1.0):
        return jax.random.uniform(self._next(), shape, jnp.bfloat16, lo, hi)

    def permutation(self, n):
        return jax.random.permutation(self._next(), n)
kernel_name = 'interleave_layers__memory_aug_recurrent_mem_tr__glu_gated_swiglu__prompt'

def setup_inputs():
    _rng = _Rng(jax.random.key(int.from_bytes(__import__("os").urandom(4), "little")))
    _w = lambda a: (lambda t: t.astype(jnp.bfloat16) if jnp.issubdtype(t.dtype, jnp.floating) else t)(jnp.asarray(a))

    def _A_setup():
        B, S, Dm = (1, 2048, 576)
        H, Dh = (32, 128)
        M, seg = (8, 32)
        seg = min(seg, S)
        S = S // seg * seg
        return {'x': _w((lambda *s: _rng.normal(s) * 0.05)(B, S, Dm)), 'mem0': _w((lambda *s: _rng.normal(s) * 0.05)(B, M, Dm)), 'Wq': _w((lambda *s: _rng.normal(s) * 0.05)(Dm, H, Dh) * Dm ** (-0.5)), 'Wk': _w((lambda *s: _rng.normal(s) * 0.05)(Dm, H, Dh) * Dm ** (-0.5)), 'Wv': _w((lambda *s: _rng.normal(s) * 0.05)(Dm, H, Dh) * Dm ** (-0.5)), 'Wo': _w((lambda *s: _rng.normal(s) * 0.05)(H, Dh, Dm) * (H * Dh) ** (-0.5)), 'seg_len': seg}
    _A_in = _A_setup()

    def _B_setup():
        B, S, D, F = (1, 2048, 576, 4608)
        return {'x': _w((lambda *s: _rng.normal(s) * 0.05)(B, S, D)), 'w1': _w((lambda *s: _rng.normal(s) * 0.05)(D, F) * (2.0 / D) ** 0.5), 'w3': _w((lambda *s: _rng.normal(s) * 0.05)(D, F) * (2.0 / D) ** 0.5), 'w2': _w((lambda *s: _rng.normal(s) * 0.05)(F, D) * (2.0 / F) ** 0.5)}
    _B_in = _B_setup()
    return {'A_x': _A_in['x'], 'A_mem0': _A_in['mem0'], 'A_Wq': _A_in['Wq'], 'A_Wk': _A_in['Wk'], 'A_Wv': _A_in['Wv'], 'A_Wo': _A_in['Wo'], 'A_seg_len': _A_in['seg_len'], 'B_x': _B_in['x'], 'B_w1': _B_in['w1'], 'B_w3': _B_in['w3'], 'B_w2': _B_in['w2']}

def reference(A_x, A_mem0, A_Wq, A_Wk, A_Wv, A_Wo, A_seg_len, B_x, B_w1, B_w3, B_w2):

    def _A_ref(x, mem0, Wq, Wk, Wv, Wo, seg_len):
        B, S, Dm = x.shape
        H, Dh = (Wq.shape[1], Wq.shape[2])
        M = mem0.shape[1]
        scale = Dh ** (-0.5)
        n_seg = S // seg_len
        L = M + seg_len
        idx = jnp.arange(L)
        mask = (idx[:, None] < M) | (idx[:, None] >= idx[None, :])
        mem = mem0
        outs = []
        for s in range(n_seg):
            xs = x[:, s * seg_len:(s + 1) * seg_len, :].copy()
            h = jnp.concatenate([mem, xs], axis=1)
            q = jnp.einsum('btd,dhe->bhte', h, Wq)
            k = jnp.einsum('btd,dhe->bhte', h, Wk)
            v = jnp.einsum('btd,dhe->bhte', h, Wv)
            scores = jnp.einsum('bhqe,bhke->bhqk', q, k) * scale
            scores = jnp.where(mask[None, None], scores, -1000000000.0)
            p = _softmax(scores, axis=-1)
            o = jnp.einsum('bhqk,bhke->bhqe', p, v)
            o = jnp.einsum('bhte,hed->btd', o, Wo)
            mem = o[:, :M, :].copy()
            outs.append(o[:, M:, :])
        return jnp.concatenate(outs, axis=1)

    def _B_ref(x, w1, w3, w2):
        gate = jnp.einsum('bsd,df->bsf', x, w1)
        up = jnp.einsum('bsd,df->bsf', x, w3)
        h = _silu(gate) * up
        out = jnp.einsum('bsf,fd->bsd', h, w2)
        return out
    x = A_x
    x = x + _A_ref(_layernorm(x, axis=-1), A_mem0, A_Wq, A_Wk, A_Wv, A_Wo, A_seg_len)
    x = x + _B_ref(_layernorm(x, axis=-1), B_w1, B_w3, B_w2)
    x = x + _A_ref(_layernorm(x, axis=-1), A_mem0, A_Wq, A_Wk, A_Wv, A_Wo, A_seg_len)
    x = x + _B_ref(_layernorm(x, axis=-1), B_w1, B_w3, B_w2)
    return x
```

```python
import functools

import jax
import jax.numpy as jnp
import numpy as np
import jax.experimental.pallas as pl
import jax.experimental.pallas.tpu as pltpu

_EPS = 1e-5
_MASK_FILL = -1000000000.0
_HEADS_PER_DOT = 4
_FFN_CHUNK = 512
_XPOSE_CHUNK = 256

_F32 = jnp.float32
_BF16 = jnp.bfloat16


def _layernorm(x):
    mean = jnp.mean(x, axis=-1, keepdims=True)
    cen = x - mean
    var = jnp.mean(cen * cen, axis=-1, keepdims=True)
    return cen * jax.lax.rsqrt(var + _EPS)


def _dot(a, b):
    return jnp.dot(a, b, preferred_element_type=_F32)


def _dot_nt(a, b):
    return jax.lax.dot_general(a, b, (((1,), (1,)), ((), ())), preferred_element_type=_F32)


def _mask_tables(n_mem, seg):
    rows = 2 * (n_mem + seg)

    def split(idx):
        is_mem = idx < 2 * n_mem
        layer = jnp.where(is_mem, idx // n_mem, (idx - 2 * n_mem) // seg)
        pos = jnp.where(is_mem, idx % n_mem, n_mem + (idx - 2 * n_mem) % seg)
        return layer, pos

    q_layer, q_pos = split(jax.lax.broadcasted_iota(jnp.int32, (rows, rows), 0))
    k_layer, k_pos = split(jax.lax.broadcasted_iota(jnp.int32, (rows, rows), 1))
    same = q_layer == k_layer
    visible = same & ((q_pos < n_mem) | (q_pos >= k_pos))
    fill = jnp.where(same, _MASK_FILL, -jnp.inf).astype(_F32)
    return visible, fill


def _kernel(xt_hbm, mem0_ref, wq_hbm, wk_hbm, wv_hbm, wot_hbm, w1_hbm, w3_hbm, w2t_hbm,
            out_hbm,
            xt_ref, x_ref, rq_ref, rk_ref, rv_ref, wqkv_ref, wot_ref, wo_ref,
            w1_ref, w3_ref, w2t_ref, w2_ref,
            h_ref, o_ref, hid_ref, xa_ref, x1_ref, y_ref, sems, out_sems,
            *, seg, n_heads, dh):
    seq, dm = x_ref.shape
    n_mem = mem0_ref.shape[0]
    n_seg = seq // seg
    ffn = w1_ref.shape[1]
    scale = dh ** -0.5
    hpd = _HEADS_PER_DOT
    tok0 = 2 * n_mem

    copies = [
        pltpu.make_async_copy(src, dst, sems.at[n])
        for n, (src, dst) in enumerate((
            (xt_hbm, xt_ref), (wq_hbm, rq_ref), (wk_hbm, rk_ref), (wv_hbm, rv_ref),
            (wot_hbm, wot_ref), (w1_hbm, w1_ref), (w3_hbm, w3_ref), (w2t_hbm, w2t_ref)))
    ]

    def wait_and_refill(n):
        copies[n].wait()
        if n + 2 < len(copies):
            copies[n + 2].start()

    copies[0].start()
    copies[1].start()

    wait_and_refill(0)
    for t in range(0, seq, _XPOSE_CHUNK):
        x_ref[t:t + _XPOSE_CHUNK, :] = xt_ref[:, t:t + _XPOSE_CHUNK].T

    mem0 = mem0_ref[...].astype(_F32)
    x_first = x_ref[0:seg, :].astype(_F32)
    h_ref[0:tok0, :] = jnp.concatenate([mem0, mem0], axis=0).astype(_BF16)
    h_ref[tok0:tok0 + seg, :] = _layernorm(x_first).astype(_BF16)
    h_ref[tok0 + seg:, :] = jnp.zeros((seg, dm), _BF16)
    xa_ref[0:seg, :] = x_first
    xa_ref[seg:, :] = jnp.zeros((seg, dm), _F32)
    x1_ref[...] = jnp.zeros(x1_ref.shape, _F32)
    hid_ref[...] = jnp.zeros(hid_ref.shape, _BF16)

    for m, raw_ref in enumerate((rq_ref, rk_ref, rv_ref)):
        words = raw_ref.bitcast(jnp.uint32)
        wait_and_refill(m + 1)

        for j in range(n_heads // 2):
            even_d = words[pl.ds(j, dm // 2, stride=n_heads), :]
            odd_d = words[pl.ds(j + n_heads // 2, dm // 2, stride=n_heads), :]
            lo = (even_d & jnp.uint32(0xFFFF)) | (odd_d << 16)
            hi = (even_d >> 16) | (odd_d & jnp.uint32(0xFFFF0000))
            for half, val in enumerate((lo, hi)):
                grp, hh = divmod(2 * j + half, hpd)
                col = (hh * 3 + m) * dh
                wqkv_ref[grp, :, col:col + dh] = pltpu.bitcast(val, _BF16)
    wait_and_refill(4)
    for head in range(n_heads):
        wo_ref[head * dh:(head + 1) * dh, :] = wot_ref[head].T
    wait_and_refill(5)
    wait_and_refill(6)
    wait_and_refill(7)
    for c in range(0, ffn, _XPOSE_CHUNK):
        w2_ref[c:c + _XPOSE_CHUNK, :] = w2t_ref[:, c:c + _XPOSE_CHUNK].T

    def attention(qkv, grp, visible, fill):
        for hh in range(hpd):
            q, k, v = (qkv[:, (3 * hh + m) * dh:(3 * hh + m + 1) * dh].astype(_BF16)
                       for m in range(3))
            s = jnp.where(visible, _dot_nt(q, k) * scale, fill)
            p = jnp.exp(s - jnp.max(s, axis=-1, keepdims=True))
            inv = 1.0 / jnp.sum(p, axis=-1, keepdims=True)
            head = grp * hpd + hh
            o_ref[:, head * dh:(head + 1) * dh] = (_dot(p.astype(_BF16), v) * inv).astype(_BF16)

    def step(i, carry):
        visible, fill = _mask_tables(n_mem, seg)
        h = h_ref[...]
        n_grp = n_heads // hpd
        qkv = _dot(h, wqkv_ref[0])
        for grp in range(n_grp):
            nxt = _dot(h, wqkv_ref[grp + 1]) if grp + 1 < n_grp else None
            attention(qkv, grp, visible, fill)
            qkv = nxt

        half = ffn // 2
        y = x1_ref[...] + _dot(hid_ref[:, :half], w2_ref[:half, :])

        a = _dot(o_ref[...], wo_ref[...])
        mem2 = jnp.where(i == 1, mem0, a[n_mem:tok0])
        h_ref[0:tok0, :] = jnp.concatenate([a[0:n_mem], mem2], axis=0).astype(_BF16)
        x1 = xa_ref[...] + a[tok0:]
        x1_ref[...] = x1
        f_in = _layernorm(x1).astype(_BF16)

        y = y + _dot(hid_ref[:, half:], w2_ref[half:, :])
        out_row = pl.multiple_of(jnp.maximum(i - 3, 0) * seg, seg)
        y_ref[pl.ds(out_row, seg), :] = y[seg:].astype(y_ref.dtype)
        nxt_row = pl.multiple_of(jnp.minimum(i + 1, n_seg - 1) * seg, seg)
        xa = jnp.concatenate([x_ref[pl.ds(nxt_row, seg), :].astype(_F32), y[:seg]], axis=0)
        xa_ref[...] = xa
        h_ref[tok0:, :] = _layernorm(xa).astype(_BF16)

        for c in range(0, ffn, _FFN_CHUNK):
            gate = _dot(f_in, w1_ref[:, c:c + _FFN_CHUNK])
            up = _dot(f_in, w3_ref[:, c:c + _FFN_CHUNK])
            hid_ref[:, c:c + _FFN_CHUNK] = (gate * jax.nn.sigmoid(gate) * up).astype(_BF16)
        return carry

    jax.lax.fori_loop(0, n_seg + 3, step, 0)

    writes = []
    for n, t in enumerate(range(0, seq, _XPOSE_CHUNK)):
        xt_ref[:, t:t + _XPOSE_CHUNK] = y_ref[t:t + _XPOSE_CHUNK, :].T
        writes.append(pltpu.make_async_copy(
            xt_ref.at[:, t:t + _XPOSE_CHUNK], out_hbm.at[:, t:t + _XPOSE_CHUNK], out_sems.at[n]))
        writes[-1].start()
    for write in writes:
        write.wait()


@functools.partial(jax.jit, static_argnames=("A_seg_len",))
def pallas_interleave_layers__memory_aug_recurrent_mem_tr__glu_gated_swiglu__prompt_kernel(
    A_x: jax.Array,
    A_mem0: jax.Array,
    A_Wq: jax.Array,
    A_Wk: jax.Array,
    A_Wv: jax.Array,
    A_Wo: jax.Array,
    A_seg_len: int,
    B_x: jax.Array,
    B_w1: jax.Array,
    B_w3: jax.Array,
    B_w2: jax.Array,
):
    del B_x
    batch, seq, dm = A_x.shape
    _, n_heads, dh = A_Wq.shape
    n_mem = A_mem0.shape[1]
    ffn = B_w1.shape[1]
    seg = int(A_seg_len)
    assert batch == 1 and seq % seg == 0
    rows = 2 * (n_mem + seg)

    vmem = pl.BlockSpec(memory_space=pltpu.VMEM)
    hbm = pl.BlockSpec(memory_space=pltpu.HBM)
    out_t = pl.pallas_call(
        functools.partial(_kernel, seg=seg, n_heads=n_heads, dh=dh),
        out_shape=jax.ShapeDtypeStruct((dm, seq), A_x.dtype),
        in_specs=[hbm, vmem] + [hbm] * 7,
        out_specs=hbm,
        scratch_shapes=[
            pltpu.VMEM((dm, seq), _BF16),
            pltpu.VMEM((seq, dm), _BF16),
            pltpu.VMEM((dm * n_heads, dh), _BF16),
            pltpu.VMEM((dm * n_heads, dh), _BF16),
            pltpu.VMEM((dm * n_heads, dh), _BF16),
            pltpu.VMEM((n_heads // _HEADS_PER_DOT, dm, 3 * dh * _HEADS_PER_DOT), _BF16),
            pltpu.VMEM((n_heads, dm, dh), _BF16),
            pltpu.VMEM((n_heads * dh, dm), _BF16),
            pltpu.VMEM((dm, ffn), _BF16),
            pltpu.VMEM((dm, ffn), _BF16),
            pltpu.VMEM((dm, ffn), _BF16),
            pltpu.VMEM((ffn, dm), _BF16),
            pltpu.VMEM((rows, dm), _BF16),
            pltpu.VMEM((rows, n_heads * dh), _BF16),
            pltpu.VMEM((2 * seg, ffn), _BF16),
            pltpu.VMEM((2 * seg, dm), _F32),
            pltpu.VMEM((2 * seg, dm), _F32),
            pltpu.VMEM((seq, dm), _BF16),
            pltpu.SemaphoreType.DMA((8,)),
            pltpu.SemaphoreType.DMA((seq // _XPOSE_CHUNK,)),
        ],
        compiler_params=pltpu.CompilerParams(vmem_limit_bytes=110 * 1024 * 1024),
    )(
        A_x.reshape(seq, dm).T,
        A_mem0.reshape(n_mem, dm),
        A_Wq.reshape(dm * n_heads, dh),
        A_Wk.reshape(dm * n_heads, dh),
        A_Wv.reshape(dm * n_heads, dh),
        A_Wo.transpose(0, 2, 1),
        B_w1,
        B_w3,
        B_w2.T,
    )
    return out_t.T.reshape(batch, seq, dm)
```

```python
import functools

import jax
import jax.numpy as jnp
import numpy as np
import jax.experimental.pallas as pl
import jax.experimental.pallas.tpu as pltpu

_EPS = 1e-5
_MASK_FILL = -1000000000.0
_HEADS_PER_DOT = 2
_QK_LAG = 1
_PV_LAG = 2
_FFN_CHUNK = 512
_XPOSE_CHUNK = 256
_W2_XPOSE_CHUNK = 384
_FFN_DMA_CHUNKS = 4
_DMA_DEPTH = 2
_DOWN_CUTS = (0, 1152, 2304, 2816)

_F32 = jnp.float32
_BF16 = jnp.bfloat16


def _layernorm(x):
    mean = jnp.mean(x, axis=-1, keepdims=True)
    cen = x - mean
    var = jnp.mean(cen * cen, axis=-1, keepdims=True)
    return cen * jax.lax.rsqrt(var + _EPS)


def _dot(a, b):
    return jnp.dot(a, b, preferred_element_type=_F32)


def _dot_nt(a, b):
    return jax.lax.dot_general(a, b, (((1,), (1,)), ((), ())), preferred_element_type=_F32)


def _mask_tables(n_streams, n_mem, seg):
    tok0 = n_streams * n_mem
    rows = tok0 + n_streams * seg

    def split(axis):
        idx = jax.lax.broadcasted_iota(jnp.int32, (rows, rows), axis)
        is_mem = idx < tok0
        stream = jnp.where(is_mem, idx // n_mem, (idx - tok0) // seg)
        pos = jnp.where(is_mem, idx % n_mem, n_mem + (idx - tok0) % seg)
        return stream, pos

    q_stream, q_pos = split(0)
    k_stream, k_pos = split(1)
    same = q_stream == k_stream
    visible = same & ((q_pos < n_mem) | (q_pos >= k_pos))
    fill = jnp.where(same, _MASK_FILL, -jnp.inf).astype(_F32)
    return visible, fill


def _kernel(xt_hbm, mem0_ref, wq_hbm, wk_hbm, wv_hbm, wot_hbm, w1_hbm, w3_hbm, w2t_hbm,
            out_hbm,
            xt_ref, x_ref, rq_ref, rk_ref, rv_ref, wqkv_ref, wot_ref, wo_ref,
            w1_ref, w3_ref, w2t_ref, w2_ref,
            h_ref, o_ref, hid_ref, xa_ref, x1_ref, y_ref, in_sems, out_sems,
            *, seg, n_heads, dh):
    seq, dm = x_ref.shape
    n_mem = mem0_ref.shape[0]
    n_seg = seq // seg
    ffn = w1_ref.shape[1]
    scale = dh ** -0.5
    hpd = _HEADS_PER_DOT
    n_grp = n_heads // hpd
    tok0 = 2 * n_mem
    xc = _XPOSE_CHUNK
    wc = ffn // _FFN_DMA_CHUNKS

    def cols(ref, start, size):
        return ref.at[:, start:start + size]

    transfers = [("x_head", cols(xt_hbm, 0, xc), cols(xt_ref, 0, xc)),
                 ("wq", wq_hbm, rq_ref), ("wk", wk_hbm, rk_ref), ("wv", wv_hbm, rv_ref),
                 ("wo", wot_hbm, wot_ref)]
    for c in range(0, ffn, wc):
        transfers.append((("w1", c), cols(w1_hbm, c, wc), cols(w1_ref, c, wc)))
        transfers.append((("w3", c), cols(w3_hbm, c, wc), cols(w3_ref, c, wc)))
    for c in range(0, ffn, wc):
        transfers.append((("w2", c), cols(w2t_hbm, c, wc), cols(w2t_ref, c, wc)))
    transfers.append(("x_tail", cols(xt_hbm, xc, seq - xc), cols(xt_ref, xc, seq - xc)))
    order = [name for name, _, _ in transfers]
    copies = [pltpu.make_async_copy(src, dst, in_sems.at[n])
              for n, (_, src, dst) in enumerate(transfers)]

    def arrive(name):
        n = order.index(name)
        copies[n].wait()
        if n + _DMA_DEPTH < len(copies):
            copies[n + _DMA_DEPTH].start()

    def project(h, grp):
        qkv = _dot(h, wqkv_ref[grp]).astype(_BF16)
        return [[qkv[:, (3 * hh + m) * dh:(3 * hh + m + 1) * dh] for m in range(3)]
                for hh in range(hpd)]

    def probabilities(qkv, visible, fill):
        probs = []
        for q, k, _ in qkv:
            s = jnp.where(visible, _dot_nt(q, k) * scale, fill)
            p = jnp.exp(s - jnp.max(s, axis=-1, keepdims=True))
            probs.append((p * (1.0 / jnp.sum(p, axis=-1, keepdims=True))).astype(_BF16))
        return probs

    def attend(h, n_streams, fillers):
        rows = h.shape[0]
        visible, fill = _mask_tables(n_streams, n_mem, seg)
        qkv, probs = {}, {}
        for t in range(n_grp + _PV_LAG):
            if t < n_grp:
                qkv[t] = project(h, t)
            elif t - n_grp < len(fillers):
                fillers[t - n_grp]()
            if 0 <= t - _QK_LAG < n_grp:
                probs[t - _QK_LAG] = probabilities(qkv[t - _QK_LAG], visible, fill)
            if 0 <= t - _PV_LAG:
                grp = t - _PV_LAG
                for hh, (p, (_, _, v)) in enumerate(zip(probs.pop(grp), qkv.pop(grp))):
                    head = grp * hpd + hh
                    o_ref[0:rows, head * dh:(head + 1) * dh] = _dot(p, v).astype(_BF16)
        for filler in fillers[_PV_LAG:]:
            filler()
        return _dot(o_ref[0:rows, :], wo_ref[...])

    def gate_up(f_in, before_chunk=None):
        for c in range(0, ffn, _FFN_CHUNK):
            if before_chunk is not None:
                before_chunk(c)
            gate = _dot(f_in, w1_ref[:, c:c + _FFN_CHUNK])
            up = _dot(f_in, w3_ref[:, c:c + _FFN_CHUNK])
            hid_ref[:, c:c + _FFN_CHUNK] = (gate * jax.nn.sigmoid(gate) * up).astype(_BF16)

    def down_parts(acc, cuts):
        def part(lo, hi):
            def run():
                acc[0] = acc[0] + _dot(hid_ref[:, lo:hi], w2_ref[lo:hi, :])
            return run
        return [part(lo, hi) for lo, hi in zip(cuts[:-1], cuts[1:])]

    def single_stream_rows(mem, x):
        return jnp.concatenate([mem, _layernorm(x)], axis=0).astype(_BF16)

    def write_back(t):
        xt_ref[:, t:t + xc] = y_ref[t:t + xc, :].T
        copy = pltpu.make_async_copy(cols(xt_ref, t, xc), cols(out_hbm, t, xc), out_sems.at[t // xc])
        copy.start()
        return copy

    for copy in copies[:_DMA_DEPTH]:
        copy.start()
    arrive("x_head")
    x_ref[0:xc, :] = xt_ref[:, 0:xc].T

    for m, (name, raw_ref) in enumerate((("wq", rq_ref), ("wk", rk_ref), ("wv", rv_ref))):
        words = raw_ref.bitcast(jnp.uint32)
        arrive(name)
        for j in range(n_heads // 2):
            even_d = words[pl.ds(j, dm // 2, stride=n_heads), :]
            odd_d = words[pl.ds(j + n_heads // 2, dm // 2, stride=n_heads), :]
            lo = (even_d & jnp.uint32(0xFFFF)) | (odd_d << 16)
            hi = (even_d >> 16) | (odd_d & jnp.uint32(0xFFFF0000))
            for half, val in enumerate((lo, hi)):
                grp, hh = divmod(2 * j + half, hpd)
                col = (hh * 3 + m) * dh
                wqkv_ref[grp, :, col:col + dh] = pltpu.bitcast(val, _BF16)

    def stage_wo():
        arrive("wo")
        for head in range(n_heads):
            wo_ref[head * dh:(head + 1) * dh, :] = wot_ref[head].T

    def stage_gate_up(c):
        for start in range(0, ffn, wc):
            if c <= start < c + _FFN_CHUNK or start < c + _FFN_CHUNK <= start + wc:
                if ("w1", start) not in staged:
                    staged.add(("w1", start))
                    arrive(("w1", start))
                    arrive(("w3", start))

    staged = set()
    mem0 = mem0_ref[...].astype(_F32)
    x_s0 = x_ref[0:seg, :].astype(_F32)
    x_s1 = x_ref[seg:2 * seg, :].astype(_F32)
    a = attend(single_stream_rows(mem0, x_s0), 1, [stage_wo])
    x1_s0 = x_s0 + a[n_mem:]
    a = attend(single_stream_rows(a[:n_mem], x_s1), 1, [])
    x1 = jnp.concatenate([x_s1 + a[n_mem:], x1_s0], axis=0)
    x1_ref[...] = x1
    gate_up(_layernorm(x1).astype(_BF16), stage_gate_up)
    x2_s0 = x1_s0
    for c in range(0, ffn, wc):
        arrive(("w2", c))
        for t in range(c, c + wc, _W2_XPOSE_CHUNK):
            w2_ref[t:t + _W2_XPOSE_CHUNK, :] = w2t_ref[:, t:t + _W2_XPOSE_CHUNK].T
        x2_s0 = x2_s0 + _dot(hid_ref[seg:, c:c + wc], w2_ref[c:c + wc, :])
    xa = jnp.concatenate([x_ref[2 * seg:3 * seg, :].astype(_F32), x2_s0], axis=0)
    xa_ref[...] = xa
    h_ref[0:tok0, :] = jnp.concatenate([a[:n_mem], mem0], axis=0).astype(_BF16)
    h_ref[tok0:, :] = _layernorm(xa).astype(_BF16)
    arrive("x_tail")
    for t in range(xc, seq, xc):
        x_ref[t:t + xc, :] = xt_ref[:, t:t + xc].T

    def step(i, carry):
        y = [x1_ref[...]]
        parts = down_parts(y, _DOWN_CUTS + (ffn,))
        a = attend(h_ref[...], 2, parts[:-1])
        h_ref[0:tok0, :] = a[:tok0].astype(_BF16)
        x1 = xa_ref[...] + a[tok0:]
        x1_ref[...] = x1
        f_in = _layernorm(x1).astype(_BF16)

        parts[-1]()
        out_row = pl.multiple_of(jnp.maximum(i - 3, 0) * seg, seg)
        y_ref[pl.ds(out_row, seg), :] = y[0][seg:].astype(y_ref.dtype)
        nxt_row = pl.multiple_of(jnp.minimum(i + 1, n_seg - 1) * seg, seg)
        xa = jnp.concatenate([x_ref[pl.ds(nxt_row, seg), :].astype(_F32), y[0][:seg]], axis=0)
        xa_ref[...] = xa
        h_ref[tok0:, :] = _layernorm(xa).astype(_BF16)
        gate_up(f_in)
        return carry

    jax.lax.fori_loop(2, n_seg, step, 0)

    writes = []
    y = [x1_ref[...]]
    mem = h_ref[0:tok0, :].astype(_F32)[n_mem:]
    x_s0 = xa_ref[seg:, :]
    a = attend(single_stream_rows(mem, x_s0), 1, down_parts(y, _DOWN_CUTS + (ffn,)))
    y_ref[seq - 3 * seg:seq - 2 * seg, :] = y[0][seg:].astype(y_ref.dtype)
    x1_s0 = x_s0 + a[n_mem:]
    x_s1 = y[0][:seg]
    for t in range(0, seq - xc, xc):
        writes.append(write_back(t))
    a = attend(single_stream_rows(a[:n_mem], x_s1), 1, [])
    x1 = jnp.concatenate([x1_s0, x_s1 + a[n_mem:]], axis=0)
    gate_up(_layernorm(x1).astype(_BF16))
    y_ref[seq - 2 * seg:, :] = (x1 + _dot(hid_ref[...], w2_ref[...])).astype(y_ref.dtype)
    writes.append(write_back(seq - xc))
    for copy in writes:
        copy.wait()


@functools.partial(jax.jit, static_argnames=("A_seg_len",))
def pallas_interleave_layers__memory_aug_recurrent_mem_tr__glu_gated_swiglu__prompt_kernel(
    A_x: jax.Array,
    A_mem0: jax.Array,
    A_Wq: jax.Array,
    A_Wk: jax.Array,
    A_Wv: jax.Array,
    A_Wo: jax.Array,
    A_seg_len: int,
    B_x: jax.Array,
    B_w1: jax.Array,
    B_w3: jax.Array,
    B_w2: jax.Array,
):
    del B_x
    batch, seq, dm = A_x.shape
    _, n_heads, dh = A_Wq.shape
    n_mem = A_mem0.shape[1]
    ffn = B_w1.shape[1]
    seg = int(A_seg_len)
    assert batch == 1 and seq % _XPOSE_CHUNK == 0 and _XPOSE_CHUNK % seg == 0 and _XPOSE_CHUNK >= 3 * seg
    rows = 2 * (n_mem + seg)

    vmem = pl.BlockSpec(memory_space=pltpu.VMEM)
    hbm = pl.BlockSpec(memory_space=pltpu.HBM)
    out_t = pl.pallas_call(
        functools.partial(_kernel, seg=seg, n_heads=n_heads, dh=dh),
        out_shape=jax.ShapeDtypeStruct((dm, seq), A_x.dtype),
        in_specs=[hbm, vmem] + [hbm] * 7,
        out_specs=hbm,
        scratch_shapes=[
            pltpu.VMEM((dm, seq), _BF16),
            pltpu.VMEM((seq, dm), _BF16),
            pltpu.VMEM((dm * n_heads, dh), _BF16),
            pltpu.VMEM((dm * n_heads, dh), _BF16),
            pltpu.VMEM((dm * n_heads, dh), _BF16),
            pltpu.VMEM((n_heads // _HEADS_PER_DOT, dm, 3 * dh * _HEADS_PER_DOT), _BF16),
            pltpu.VMEM((n_heads, dm, dh), _BF16),
            pltpu.VMEM((n_heads * dh, dm), _BF16),
            pltpu.VMEM((dm, ffn), _BF16),
            pltpu.VMEM((dm, ffn), _BF16),
            pltpu.VMEM((dm, ffn), _BF16),
            pltpu.VMEM((ffn, dm), _BF16),
            pltpu.VMEM((rows, dm), _BF16),
            pltpu.VMEM((rows, n_heads * dh), _BF16),
            pltpu.VMEM((2 * seg, ffn), _BF16),
            pltpu.VMEM((2 * seg, dm), _F32),
            pltpu.VMEM((2 * seg, dm), _F32),
            pltpu.VMEM((seq, dm), _BF16),
            pltpu.SemaphoreType.DMA((6 + 3 * _FFN_DMA_CHUNKS,)),
            pltpu.SemaphoreType.DMA((seq // _XPOSE_CHUNK,)),
        ],
        compiler_params=pltpu.CompilerParams(vmem_limit_bytes=110 * 1024 * 1024),
    )(
        A_x.reshape(seq, dm).T,
        A_mem0.reshape(n_mem, dm),
        A_Wq.reshape(dm * n_heads, dh),
        A_Wk.reshape(dm * n_heads, dh),
        A_Wv.reshape(dm * n_heads, dh),
        A_Wo.transpose(0, 2, 1),
        B_w1,
        B_w3,
        B_w2.T,
    )
    return out_t.T.reshape(batch, seq, dm)
```

```python
import functools

import jax
import jax.numpy as jnp
import numpy as np
import jax.experimental.pallas as pl
import jax.experimental.pallas.tpu as pltpu

_EPS = 1e-5
_MASK_FILL = -1000000000.0
_HEADS_PER_DOT = 2
_QK_LAG = 1
_PV_LAG = 2
_FFN_CHUNK = 512
_XPOSE_CHUNK = 256
_W2_XPOSE_CHUNK = 384
_FFN_DMA_CHUNKS = 4
_QKV_DMA_CHUNKS = 2
_WORD_TILE = 4
_DOWN_CUTS = (0, 1152, 2304, 2816)

_F32 = jnp.float32
_BF16 = jnp.bfloat16


def _layernorm(x):
    mean = jnp.mean(x, axis=-1, keepdims=True)
    cen = x - mean
    var = jnp.mean(cen * cen, axis=-1, keepdims=True)
    return cen * jax.lax.rsqrt(var + _EPS)


def _dot(a, b):
    return jnp.dot(a, b, preferred_element_type=_F32)


def _dot_nt(a, b):
    return jax.lax.dot_general(a, b, (((1,), (1,)), ((), ())), preferred_element_type=_F32)


def _mask_tables(n_streams, n_mem, seg):
    tok0 = n_streams * n_mem
    rows = tok0 + n_streams * seg

    def split(axis):
        idx = jax.lax.broadcasted_iota(jnp.int32, (rows, rows), axis)
        is_mem = idx < tok0
        stream = jnp.where(is_mem, idx // n_mem, (idx - tok0) // seg)
        pos = jnp.where(is_mem, idx % n_mem, n_mem + (idx - tok0) % seg)
        return stream, pos

    q_stream, q_pos = split(0)
    k_stream, k_pos = split(1)
    same = q_stream == k_stream
    visible = same & ((q_pos < n_mem) | (q_pos >= k_pos))
    fill = jnp.where(same, _MASK_FILL, -jnp.inf).astype(_F32)
    return visible, fill


def _kernel(xt_hbm, mem0_ref, wq_hbm, wk_hbm, wv_hbm, wot_hbm, w1_hbm, w3_hbm, w2t_hbm,
            out_hbm,
            xt_ref, x_ref, rq_ref, rk_ref, rv_ref, wqkv_ref, wot_ref, wo_ref,
            w1_ref, w3_ref, w2t_ref, w2_ref,
            h_ref, o_ref, hid_ref, xa_ref, x1_ref, y_ref, in_sems, out_sems,
            *, seg, n_heads, dh):
    seq, dm = x_ref.shape
    n_mem = mem0_ref.shape[0]
    n_seg = seq // seg
    ffn = w1_ref.shape[1]
    scale = dh ** -0.5
    hpd = _HEADS_PER_DOT
    n_grp = n_heads // hpd
    tok0 = 2 * n_mem
    xc = _XPOSE_CHUNK
    wc = ffn // _FFN_DMA_CHUNKS

    def cols(ref, start, size):
        return ref.at[:, start:start + size]

    def rows_of(ref, start, size):
        return ref.at[start:start + size, :]

    raw_rows = dm * n_heads // _QKV_DMA_CHUNKS
    transfers = [("x_head", cols(xt_hbm, 0, xc), cols(xt_ref, 0, xc))]
    for name, src, dst in (("wq", wq_hbm, rq_ref), ("wk", wk_hbm, rk_ref), ("wv", wv_hbm, rv_ref)):
        for c in range(_QKV_DMA_CHUNKS):
            transfers.append(((name, c), rows_of(src, c * raw_rows, raw_rows),
                              rows_of(dst, c * raw_rows, raw_rows)))
    transfers.append(("wo", wot_hbm, wot_ref))
    for c in range(0, ffn, wc):
        transfers.append((("w1", c), cols(w1_hbm, c, wc), cols(w1_ref, c, wc)))
        transfers.append((("w3", c), cols(w3_hbm, c, wc), cols(w3_ref, c, wc)))
    transfers.append(("x_tail", cols(xt_hbm, xc, seq - xc), cols(xt_ref, xc, seq - xc)))
    for c in range(0, ffn, wc):
        transfers.append((("w2", c), cols(w2t_hbm, c, wc), cols(w2t_ref, c, wc)))
    copies = {name: pltpu.make_async_copy(src, dst, in_sems.at[n])
              for n, (name, src, dst) in enumerate(transfers)}

    def arrive(name):
        copies[name].wait()

    def project(h, grp):
        qkv = _dot(h, wqkv_ref[grp]).astype(_BF16)
        return [[qkv[:, (3 * hh + m) * dh:(3 * hh + m + 1) * dh] for m in range(3)]
                for hh in range(hpd)]

    def probabilities(qkv, visible, fill):
        probs = []
        for q, k, _ in qkv:
            s = jnp.where(visible, _dot_nt(q, k) * scale, fill)
            p = jnp.exp(s - jnp.max(s, axis=-1, keepdims=True))
            probs.append((p * (1.0 / jnp.sum(p, axis=-1, keepdims=True))).astype(_BF16))
        return probs

    def heads(h, n_streams, fillers):
        rows = h.shape[0]
        visible, fill = _mask_tables(n_streams, n_mem, seg)
        qkv, probs = {}, {}
        for t in range(n_grp + _PV_LAG):
            if t < n_grp:
                qkv[t] = project(h, t)
            elif t - n_grp < len(fillers):
                fillers[t - n_grp]()
            if 0 <= t - _QK_LAG < n_grp:
                probs[t - _QK_LAG] = probabilities(qkv[t - _QK_LAG], visible, fill)
            if 0 <= t - _PV_LAG:
                grp = t - _PV_LAG
                for hh, (p, (_, _, v)) in enumerate(zip(probs.pop(grp), qkv.pop(grp))):
                    head = grp * hpd + hh
                    o_ref[0:rows, head * dh:(head + 1) * dh] = _dot(p, v).astype(_BF16)
        for filler in fillers[_PV_LAG:]:
            filler()

    def attend(h, n_streams, fillers):
        heads(h, n_streams, fillers)
        return _dot(o_ref[0:h.shape[0], :], wo_ref[...])

    def gate_up(f_in, lo=0, hi=ffn):
        for c in range(lo, hi, _FFN_CHUNK):
            end = min(c + _FFN_CHUNK, hi)
            gate = _dot(f_in, w1_ref[:, c:end])
            up = _dot(f_in, w3_ref[:, c:end])
            hid_ref[:, c:end] = (gate * jax.nn.sigmoid(gate) * up).astype(_BF16)

    def down_parts(acc, cuts):
        def part(lo, hi):
            def run():
                acc[0] = acc[0] + _dot(hid_ref[:, lo:hi], w2_ref[lo:hi, :])
            return run
        return [part(lo, hi) for lo, hi in zip(cuts[:-1], cuts[1:])]

    def single_stream_rows(mem, x):
        return jnp.concatenate([mem, _layernorm(x)], axis=0).astype(_BF16)

    def write_back(t):
        xt_ref[:, t:t + xc] = y_ref[t:t + xc, :].T
        copy = pltpu.make_async_copy(cols(xt_ref, t, xc), cols(out_hbm, t, xc), out_sems.at[t // xc])
        copy.start()
        return copy

    for copy in copies.values():
        copy.start()
    arrive("x_head")
    x_ref[0:xc, :] = xt_ref[:, 0:xc].T

    pairs = n_heads // 2
    d_chunk = dm // _QKV_DMA_CHUNKS
    for m, (name, raw_ref) in enumerate((("wq", rq_ref), ("wk", rk_ref), ("wv", rv_ref))):
        words = raw_ref.bitcast(jnp.uint32)
        for c in range(_QKV_DMA_CHUNKS):
            arrive((name, c))

            def regroup(quad, carry, m=m, c=c, words=words):
                start = pl.multiple_of(c * d_chunk * pairs + quad * _WORD_TILE, _WORD_TILE)
                view = words.at[pl.ds(start, d_chunk * pairs - pairs + _WORD_TILE), :]
                for r in range(_WORD_TILE):
                    even_d = view[pl.ds(r, d_chunk // 2, stride=n_heads), :]
                    odd_d = view[pl.ds(r + pairs, d_chunk // 2, stride=n_heads), :]
                    lo = (even_d & jnp.uint32(0xFFFF)) | (odd_d << 16)
                    hi = (even_d >> 16) | (odd_d & jnp.uint32(0xFFFF0000))
                    for half, val in enumerate((lo, hi)):
                        grp, hh = divmod(2 * r + half, hpd)
                        col = (hh * 3 + m) * dh
                        wqkv_ref[quad * (2 * _WORD_TILE // hpd) + grp,
                                 c * d_chunk:(c + 1) * d_chunk, col:col + dh] = pltpu.bitcast(val, _BF16)
                return carry

            jax.lax.fori_loop(0, pairs // _WORD_TILE, regroup, 0)

    mem0 = mem0_ref[...].astype(_F32)
    xa_ref[0:n_mem, :] = mem0

    def first_segments(s, carry):
        x_s = x_ref[pl.ds(pl.multiple_of(s * seg, seg), seg), :].astype(_F32)
        heads(single_stream_rows(xa_ref[0:n_mem, :], x_s), 1, [])

        @pl.when(s == 0)
        def _():
            arrive("wo")

            def stage_wo(head, carry):
                wo_ref[pl.ds(pl.multiple_of(head * dh, dh), dh), :] = wot_ref[head].T
                return carry

            jax.lax.fori_loop(0, n_heads, stage_wo, 0, unroll=4)

        a = _dot(o_ref[0:n_mem + seg, :], wo_ref[...])
        xa_ref[0:n_mem, :] = a[:n_mem]
        x1_ref[pl.ds(pl.multiple_of((1 - s) * seg, seg), seg), :] = x_s + a[n_mem:]
        return carry

    jax.lax.fori_loop(0, 2, first_segments, 0)
    h_ref[0:tok0, :] = jnp.concatenate([xa_ref[0:n_mem, :], mem0], axis=0).astype(_BF16)
    f_in = _layernorm(x1_ref[...]).astype(_BF16)
    for c in range(0, ffn, wc):
        arrive(("w1", c))
        arrive(("w3", c))
        gate_up(f_in, c, c + wc)
    arrive("x_tail")
    for t in range(xc, seq, xc):
        x_ref[t:t + xc, :] = xt_ref[:, t:t + xc].T
    x2_s0 = x1_ref[seg:, :]
    for c in range(0, ffn, wc):
        arrive(("w2", c))
        for t in range(c, c + wc, _W2_XPOSE_CHUNK):
            w2_ref[t:t + _W2_XPOSE_CHUNK, :] = w2t_ref[:, t:t + _W2_XPOSE_CHUNK].T
        x2_s0 = x2_s0 + _dot(hid_ref[seg:, c:c + wc], w2_ref[c:c + wc, :])
    xa = jnp.concatenate([x_ref[2 * seg:3 * seg, :].astype(_F32), x2_s0], axis=0)
    xa_ref[...] = xa
    h_ref[tok0:, :] = _layernorm(xa).astype(_BF16)

    def step(i, carry):
        y = [x1_ref[...]]
        parts = down_parts(y, _DOWN_CUTS + (ffn,))
        a = attend(h_ref[...], 2, parts[:-1])
        h_ref[0:tok0, :] = a[:tok0].astype(_BF16)
        x1 = xa_ref[...] + a[tok0:]
        x1_ref[...] = x1
        f_in = _layernorm(x1).astype(_BF16)

        parts[-1]()
        out_row = pl.multiple_of(jnp.maximum(i - 3, 0) * seg, seg)
        y_ref[pl.ds(out_row, seg), :] = y[0][seg:].astype(y_ref.dtype)
        nxt_row = pl.multiple_of(jnp.minimum(i + 1, n_seg - 1) * seg, seg)
        xa = jnp.concatenate([x_ref[pl.ds(nxt_row, seg), :].astype(_F32), y[0][:seg]], axis=0)
        xa_ref[...] = xa
        h_ref[tok0:, :] = _layernorm(xa).astype(_BF16)
        gate_up(f_in)
        return carry

    jax.lax.fori_loop(2, n_seg, step, 0)

    writes = []
    y = [x1_ref[...]]
    mem = h_ref[0:tok0, :].astype(_F32)[n_mem:]
    x_s0 = xa_ref[seg:, :]
    a = attend(single_stream_rows(mem, x_s0), 1, down_parts(y, _DOWN_CUTS + (ffn,)))
    y_ref[seq - 3 * seg:seq - 2 * seg, :] = y[0][seg:].astype(y_ref.dtype)
    x1_s0 = x_s0 + a[n_mem:]
    x_s1 = y[0][:seg]
    for t in range(0, seq - xc, xc):
        writes.append(write_back(t))
    a = attend(single_stream_rows(a[:n_mem], x_s1), 1, [])
    x1 = jnp.concatenate([x1_s0, x_s1 + a[n_mem:]], axis=0)
    gate_up(_layernorm(x1).astype(_BF16))
    y_ref[seq - 2 * seg:, :] = (x1 + _dot(hid_ref[...], w2_ref[...])).astype(y_ref.dtype)
    writes.append(write_back(seq - xc))
    for copy in writes:
        copy.wait()


@functools.partial(jax.jit, static_argnames=("A_seg_len",))
def pallas_interleave_layers__memory_aug_recurrent_mem_tr__glu_gated_swiglu__prompt_kernel(
    A_x: jax.Array,
    A_mem0: jax.Array,
    A_Wq: jax.Array,
    A_Wk: jax.Array,
    A_Wv: jax.Array,
    A_Wo: jax.Array,
    A_seg_len: int,
    B_x: jax.Array,
    B_w1: jax.Array,
    B_w3: jax.Array,
    B_w2: jax.Array,
):
    del B_x
    batch, seq, dm = A_x.shape
    _, n_heads, dh = A_Wq.shape
    n_mem = A_mem0.shape[1]
    ffn = B_w1.shape[1]
    seg = int(A_seg_len)
    assert batch == 1 and seq % _XPOSE_CHUNK == 0 and _XPOSE_CHUNK % seg == 0 and _XPOSE_CHUNK >= 3 * seg
    rows = 2 * (n_mem + seg)

    vmem = pl.BlockSpec(memory_space=pltpu.VMEM)
    hbm = pl.BlockSpec(memory_space=pltpu.HBM)
    out_t = pl.pallas_call(
        functools.partial(_kernel, seg=seg, n_heads=n_heads, dh=dh),
        out_shape=jax.ShapeDtypeStruct((dm, seq), A_x.dtype),
        in_specs=[hbm, vmem] + [hbm] * 7,
        out_specs=hbm,
        scratch_shapes=[
            pltpu.VMEM((dm, seq), _BF16),
            pltpu.VMEM((seq, dm), _BF16),
            pltpu.VMEM((dm * n_heads, dh), _BF16),
            pltpu.VMEM((dm * n_heads, dh), _BF16),
            pltpu.VMEM((dm * n_heads, dh), _BF16),
            pltpu.VMEM((n_heads // _HEADS_PER_DOT, dm, 3 * dh * _HEADS_PER_DOT), _BF16),
            pltpu.VMEM((n_heads, dm, dh), _BF16),
            pltpu.VMEM((n_heads * dh, dm), _BF16),
            pltpu.VMEM((dm, ffn), _BF16),
            pltpu.VMEM((dm, ffn), _BF16),
            pltpu.VMEM((dm, ffn), _BF16),
            pltpu.VMEM((ffn, dm), _BF16),
            pltpu.VMEM((rows, dm), _BF16),
            pltpu.VMEM((rows, n_heads * dh), _BF16),
            pltpu.VMEM((2 * seg, ffn), _BF16),
            pltpu.VMEM((2 * seg, dm), _F32),
            pltpu.VMEM((2 * seg, dm), _F32),
            pltpu.VMEM((seq, dm), _BF16),
            pltpu.SemaphoreType.DMA((3 + 3 * _QKV_DMA_CHUNKS + 3 * _FFN_DMA_CHUNKS,)),
            pltpu.SemaphoreType.DMA((seq // _XPOSE_CHUNK,)),
        ],
        compiler_params=pltpu.CompilerParams(vmem_limit_bytes=110 * 1024 * 1024),
    )(
        A_x.reshape(seq, dm).T,
        A_mem0.reshape(n_mem, dm),
        A_Wq.reshape(dm * n_heads, dh),
        A_Wk.reshape(dm * n_heads, dh),
        A_Wv.reshape(dm * n_heads, dh),
        A_Wo.transpose(0, 2, 1),
        B_w1,
        B_w3,
        B_w2.T,
    )
    return out_t.T.reshape(batch, seq, dm)
```

```python
import functools

import jax
import jax.numpy as jnp
import numpy as np
import jax.experimental.pallas as pl
import jax.experimental.pallas.tpu as pltpu

_EPS = 1e-5
_MASK_FILL = -1000000000.0
_HEADS_PER_DOT = 2
_QK_LAG = 1
_PV_LAG = 2
_FFN_CHUNK = 512
_XPOSE_CHUNK = 256
_W2_XPOSE_CHUNK = 384
_FFN_DMA_CHUNKS = 3
_QKV_DMA_CHUNKS = 2
_WORD_TILE = 4
_DOWN_CUTS = (0, 1152, 2304, 2816)

_LANES = 128
_HALF = _LANES // 2
_F32 = jnp.float32
_BF16 = jnp.bfloat16


def _layernorm(x):
    mean = jnp.mean(x, axis=-1, keepdims=True)
    cen = x - mean
    var = jnp.mean(cen * cen, axis=-1, keepdims=True)
    return cen * jax.lax.rsqrt(var + _EPS)


def _dot(a, b):
    return jnp.dot(a, b, preferred_element_type=_F32)


def _dot_nt(a, b):
    return jax.lax.dot_general(a, b, (((1,), (1,)), ((), ())), preferred_element_type=_F32)


def _split_lhs(x):
    full = x.shape[1] - _HALF
    first, rest = x[:, :_LANES], x[:, _LANES:full]
    tail = x[:, full:]
    lhs_b0 = jnp.concatenate([first[:, :_HALF], tail], axis=1)
    lhs_s = jnp.concatenate([tail, first[:, _HALF:]], axis=1)
    return jnp.concatenate([first, rest, lhs_b0, lhs_s], axis=1).astype(_BF16)


def _paired_dot(lhs, w_a, w_b, w_s):
    full = w_a.shape[0]
    shared = _dot(lhs[:, full + _LANES:], w_s)
    lhs_b = jnp.concatenate([lhs[:, full:full + _LANES], lhs[:, _LANES:full]], axis=1)
    return _dot(lhs[:, :full], w_a) + shared, _dot(lhs_b, w_b) + shared


def _pair_weights(a_mid, a_tail, b_mid, b_tail):
    a_new = (a_mid.astype(_F32) - b_mid.astype(_F32)).astype(_BF16)
    b_new = (b_tail.astype(_F32) - a_tail.astype(_F32)).astype(_BF16)
    return a_new, b_new, jnp.concatenate([a_tail, b_mid], axis=0)


def _mask_tables(n_streams, n_mem, seg):
    tok0 = n_streams * n_mem
    rows = tok0 + n_streams * seg

    def split(axis):
        idx = jax.lax.broadcasted_iota(jnp.int32, (rows, rows), axis)
        is_mem = idx < tok0
        stream = jnp.where(is_mem, idx // n_mem, (idx - tok0) // seg)
        pos = jnp.where(is_mem, idx % n_mem, n_mem + (idx - tok0) % seg)
        return stream, pos

    q_stream, q_pos = split(0)
    k_stream, k_pos = split(1)
    same = q_stream == k_stream
    visible = same & ((q_pos < n_mem) | (q_pos >= k_pos))
    fill = jnp.where(same, _MASK_FILL, -jnp.inf).astype(_F32)
    return visible, fill


def _kernel(xt_hbm, mem0_ref, wq_hbm, wk_hbm, wv_hbm, wot_hbm, w1_hbm, w3_hbm, w2t_hbm,
            out_hbm,
            xt_ref, x_ref, rq_ref, rk_ref, rv_ref, wqkv_ref, wot_ref, wo_ref,
            w1_ref, w3_ref, w2t_ref, w2_ref, sqkv_ref, s1_ref, s3_ref,
            h_ref, o_ref, hid_ref, xa_ref, x1_ref, y_ref, in_sems, out_sems,
            *, seg, n_heads, dh):
    seq, dm = x_ref.shape
    n_mem = mem0_ref.shape[0]
    n_seg = seq // seg
    ffn = w1_ref.shape[1]
    scale = dh ** -0.5
    hpd = _HEADS_PER_DOT
    n_grp = n_heads // hpd
    tok0 = 2 * n_mem
    full = dm - _HALF
    mid = slice(_HALF, _LANES)
    fc = _FFN_CHUNK
    xc = _XPOSE_CHUNK
    wc = ffn // _FFN_DMA_CHUNKS

    def cols(ref, start, size):
        return ref.at[:, start:start + size]

    def rows_of(ref, start, size):
        return ref.at[start:start + size, :]

    raw_rows = dm * n_heads // _QKV_DMA_CHUNKS
    transfers = [("x_head", cols(xt_hbm, 0, xc), cols(xt_ref, 0, xc))]
    for name, src, dst in (("wq", wq_hbm, rq_ref), ("wk", wk_hbm, rk_ref), ("wv", wv_hbm, rv_ref)):
        for c in range(_QKV_DMA_CHUNKS):
            transfers.append(((name, c), rows_of(src, c * raw_rows, raw_rows),
                              rows_of(dst, c * raw_rows, raw_rows)))
    transfers.append(("wo", wot_hbm, wot_ref))
    for c in range(0, ffn, wc):
        transfers.append((("w1", c), cols(w1_hbm, c, wc), cols(w1_ref, c, wc)))
        transfers.append((("w3", c), cols(w3_hbm, c, wc), cols(w3_ref, c, wc)))
    transfers.append(("x_tail", cols(xt_hbm, xc, seq - xc), cols(xt_ref, xc, seq - xc)))
    for c in range(0, ffn, wc):
        transfers.append((("w2", c), cols(w2t_hbm, c, wc), cols(w2t_ref, c, wc)))
    copies = {name: pltpu.make_async_copy(src, dst, in_sems.at[n])
              for n, (name, src, dst) in enumerate(transfers)}

    def arrive(name):
        copies[name].wait()

    def project(h, grp):
        both = _paired_dot(h, wqkv_ref[grp, 0:full, 0:3 * dh], wqkv_ref[grp, 0:full, 3 * dh:],
                           sqkv_ref[grp])
        return [[qkv[:, m * dh:(m + 1) * dh].astype(_BF16) for m in range(3)] for qkv in both]

    def probabilities(qkv, visible, fill):
        probs = []
        for q, k, _ in qkv:
            s = jnp.where(visible, _dot_nt(q, k) * scale, fill)
            p = jnp.exp(s - jnp.max(s, axis=-1, keepdims=True))
            probs.append((p * (1.0 / jnp.sum(p, axis=-1, keepdims=True))).astype(_BF16))
        return probs

    def heads(h, n_streams, fillers):
        rows = h.shape[0]
        visible, fill = _mask_tables(n_streams, n_mem, seg)
        qkv, probs = {}, {}
        for t in range(n_grp + _PV_LAG):
            if t < n_grp:
                qkv[t] = project(h, t)
            elif t - n_grp < len(fillers):
                fillers[t - n_grp]()
            if 0 <= t - _QK_LAG < n_grp:
                probs[t - _QK_LAG] = probabilities(qkv[t - _QK_LAG], visible, fill)
            if 0 <= t - _PV_LAG:
                grp = t - _PV_LAG
                for hh, (p, (_, _, v)) in enumerate(zip(probs.pop(grp), qkv.pop(grp))):
                    head = grp * hpd + hh
                    o_ref[0:rows, head * dh:(head + 1) * dh] = _dot(p, v).astype(_BF16)
        for filler in fillers[_PV_LAG:]:
            filler()

    def attend(h, n_streams, fillers):
        heads(h, n_streams, fillers)
        return _dot(o_ref[0:h.shape[0], :], wo_ref[...])

    def pair_gate_up(lo, hi):
        for w_ref, s_ref in ((w1_ref, s1_ref), (w3_ref, s3_ref)):
            for c in range(lo, hi, fc):
                ca, cb = slice(c, c + fc // 2), slice(c + fc // 2, c + fc)
                w_ref[mid, ca], w_ref[mid, cb], s_ref[:, c // 2:(c + fc) // 2] = _pair_weights(
                    w_ref[mid, ca], w_ref[full:, ca], w_ref[mid, cb], w_ref[full:, cb])

    def gate_up(f_in, lo=0, hi=ffn):
        for c in range(lo, hi, fc):
            ca, cb = slice(c, c + fc // 2), slice(c + fc // 2, c + fc)
            cs = slice(c // 2, (c + fc) // 2)
            gates = _paired_dot(f_in, w1_ref[0:full, ca], w1_ref[0:full, cb], s1_ref[:, cs])
            ups = _paired_dot(f_in, w3_ref[0:full, ca], w3_ref[0:full, cb], s3_ref[:, cs])
            for cols_, gate, up in zip((ca, cb), gates, ups):
                hid_ref[:, cols_] = (gate * jax.nn.sigmoid(gate) * up).astype(_BF16)

    def down_parts(acc, cuts):
        def part(lo, hi):
            def run():
                acc[0] = acc[0] + _dot(hid_ref[:, lo:hi], w2_ref[lo:hi, :])
            return run
        return [part(lo, hi) for lo, hi in zip(cuts[:-1], cuts[1:])]

    def single_stream_rows(mem, x):
        return _split_lhs(jnp.concatenate([mem, _layernorm(x)], axis=0))

    def write_back(t):
        xt_ref[:, t:t + xc] = y_ref[t:t + xc, :].T
        copy = pltpu.make_async_copy(cols(xt_ref, t, xc), cols(out_hbm, t, xc), out_sems.at[t // xc])
        copy.start()
        return copy

    for copy in copies.values():
        copy.start()
    arrive("x_head")
    x_ref[0:xc, :] = xt_ref[:, 0:xc].T

    pairs = n_heads // 2
    d_chunk = dm // _QKV_DMA_CHUNKS
    for m, (name, raw_ref) in enumerate((("wq", rq_ref), ("wk", rk_ref), ("wv", rv_ref))):
        words = raw_ref.bitcast(jnp.uint32)
        for c in range(_QKV_DMA_CHUNKS):
            arrive((name, c))

            def regroup(quad, carry, m=m, c=c, words=words):
                start = pl.multiple_of(c * d_chunk * pairs + quad * _WORD_TILE, _WORD_TILE)
                view = words.at[pl.ds(start, d_chunk * pairs - pairs + _WORD_TILE), :]
                for r in range(_WORD_TILE):
                    even_d = view[pl.ds(r, d_chunk // 2, stride=n_heads), :]
                    odd_d = view[pl.ds(r + pairs, d_chunk // 2, stride=n_heads), :]
                    lo = (even_d & jnp.uint32(0xFFFF)) | (odd_d << 16)
                    hi = (even_d >> 16) | (odd_d & jnp.uint32(0xFFFF0000))
                    for half, val in enumerate((lo, hi)):
                        grp, hh = divmod(2 * r + half, hpd)
                        col = (hh * 3 + m) * dh
                        wqkv_ref[quad * (2 * _WORD_TILE // hpd) + grp,
                                 c * d_chunk:(c + 1) * d_chunk, col:col + dh] = pltpu.bitcast(val, _BF16)
                return carry

            jax.lax.fori_loop(0, pairs // _WORD_TILE, regroup, 0)

    def pair_heads(grp, carry):
        ca, cb = slice(0, 3 * dh), slice(3 * dh, 6 * dh)
        wqkv_ref[grp, mid, ca], wqkv_ref[grp, mid, cb], sqkv_ref[grp] = _pair_weights(
            wqkv_ref[grp, mid, ca], wqkv_ref[grp, full:, ca],
            wqkv_ref[grp, mid, cb], wqkv_ref[grp, full:, cb])
        return carry

    jax.lax.fori_loop(0, n_grp, pair_heads, 0)

    mem0 = mem0_ref[...].astype(_F32)
    xa_ref[0:n_mem, :] = mem0

    def first_segments(s, carry):
        x_s = x_ref[pl.ds(pl.multiple_of(s * seg, seg), seg), :].astype(_F32)
        heads(single_stream_rows(xa_ref[0:n_mem, :], x_s), 1, [])

        @pl.when(s == 0)
        def _():
            arrive("wo")

            def stage_wo(head, carry):
                wo_ref[pl.ds(pl.multiple_of(head * dh, dh), dh), :] = wot_ref[head].T
                return carry

            jax.lax.fori_loop(0, n_heads, stage_wo, 0, unroll=4)

        a = _dot(o_ref[0:n_mem + seg, :], wo_ref[...])
        xa_ref[0:n_mem, :] = a[:n_mem]
        x1_ref[pl.ds(pl.multiple_of((1 - s) * seg, seg), seg), :] = x_s + a[n_mem:]
        return carry

    jax.lax.fori_loop(0, 2, first_segments, 0)
    h_ref[0:tok0, :] = _split_lhs(jnp.concatenate([xa_ref[0:n_mem, :], mem0], axis=0))
    f_in = _split_lhs(_layernorm(x1_ref[...]))
    for c in range(0, ffn, wc):
        arrive(("w1", c))
        arrive(("w3", c))
        pair_gate_up(c, c + wc)
        gate_up(f_in, c, c + wc)
    arrive("x_tail")
    for t in range(xc, seq, xc):
        x_ref[t:t + xc, :] = xt_ref[:, t:t + xc].T
    x2_s0 = x1_ref[seg:, :]
    for c in range(0, ffn, wc):
        arrive(("w2", c))
        for t in range(c, c + wc, _W2_XPOSE_CHUNK):
            w2_ref[t:t + _W2_XPOSE_CHUNK, :] = w2t_ref[:, t:t + _W2_XPOSE_CHUNK].T
        x2_s0 = x2_s0 + _dot(hid_ref[seg:, c:c + wc], w2_ref[c:c + wc, :])
    xa = jnp.concatenate([x_ref[2 * seg:3 * seg, :].astype(_F32), x2_s0], axis=0)
    xa_ref[...] = xa
    h_ref[tok0:, :] = _split_lhs(_layernorm(xa))

    def step(i, carry):
        y = [x1_ref[...]]
        parts = down_parts(y, _DOWN_CUTS + (ffn,))
        a = attend(h_ref[...], 2, parts[:-1])
        h_ref[0:tok0, :] = _split_lhs(a[:tok0])
        x1 = xa_ref[...] + a[tok0:]
        x1_ref[...] = x1
        f_in = _split_lhs(_layernorm(x1))

        parts[-1]()
        out_row = pl.multiple_of(jnp.maximum(i - 3, 0) * seg, seg)
        y_ref[pl.ds(out_row, seg), :] = y[0][seg:].astype(y_ref.dtype)
        nxt_row = pl.multiple_of(jnp.minimum(i + 1, n_seg - 1) * seg, seg)
        xa = jnp.concatenate([x_ref[pl.ds(nxt_row, seg), :].astype(_F32), y[0][:seg]], axis=0)
        xa_ref[...] = xa
        h_ref[tok0:, :] = _split_lhs(_layernorm(xa))
        gate_up(f_in)
        return carry

    jax.lax.fori_loop(2, n_seg, step, 0)

    writes = []
    y = [x1_ref[...]]
    h = h_ref[...].astype(_F32)
    h = jnp.concatenate([h[n_mem:tok0], h[tok0 + seg:]], axis=0).astype(_BF16)
    x_s0 = xa_ref[seg:, :]
    a = attend(h, 1, down_parts(y, _DOWN_CUTS + (ffn,)))
    y_ref[seq - 3 * seg:seq - 2 * seg, :] = y[0][seg:].astype(y_ref.dtype)
    x1_s0 = x_s0 + a[n_mem:]
    x_s1 = y[0][:seg]
    for t in range(0, seq - xc, xc):
        writes.append(write_back(t))
    a = attend(single_stream_rows(a[:n_mem], x_s1), 1, [])
    x1 = jnp.concatenate([x1_s0, x_s1 + a[n_mem:]], axis=0)
    gate_up(_split_lhs(_layernorm(x1)))
    y_ref[seq - 2 * seg:, :] = (x1 + _dot(hid_ref[...], w2_ref[...])).astype(y_ref.dtype)
    writes.append(write_back(seq - xc))
    for copy in writes:
        copy.wait()


@functools.partial(jax.jit, static_argnames=("A_seg_len",))
def pallas_interleave_layers__memory_aug_recurrent_mem_tr__glu_gated_swiglu__prompt_kernel(
    A_x: jax.Array,
    A_mem0: jax.Array,
    A_Wq: jax.Array,
    A_Wk: jax.Array,
    A_Wv: jax.Array,
    A_Wo: jax.Array,
    A_seg_len: int,
    B_x: jax.Array,
    B_w1: jax.Array,
    B_w3: jax.Array,
    B_w2: jax.Array,
):
    del B_x
    batch, seq, dm = A_x.shape
    _, n_heads, dh = A_Wq.shape
    n_mem = A_mem0.shape[1]
    ffn = B_w1.shape[1]
    seg = int(A_seg_len)
    assert batch == 1 and seq % _XPOSE_CHUNK == 0 and _XPOSE_CHUNK % seg == 0 and _XPOSE_CHUNK >= 3 * seg
    rows = 2 * (n_mem + seg)

    vmem = pl.BlockSpec(memory_space=pltpu.VMEM)
    hbm = pl.BlockSpec(memory_space=pltpu.HBM)
    out_t = pl.pallas_call(
        functools.partial(_kernel, seg=seg, n_heads=n_heads, dh=dh),
        out_shape=jax.ShapeDtypeStruct((dm, seq), A_x.dtype),
        in_specs=[hbm, vmem] + [hbm] * 7,
        out_specs=hbm,
        scratch_shapes=[
            pltpu.VMEM((dm, seq), _BF16),
            pltpu.VMEM((seq, dm), _BF16),
            pltpu.VMEM((dm * n_heads, dh), _BF16),
            pltpu.VMEM((dm * n_heads, dh), _BF16),
            pltpu.VMEM((dm * n_heads, dh), _BF16),
            pltpu.VMEM((n_heads // _HEADS_PER_DOT, dm, 3 * dh * _HEADS_PER_DOT), _BF16),
            pltpu.VMEM((n_heads, dm, dh), _BF16),
            pltpu.VMEM((n_heads * dh, dm), _BF16),
            pltpu.VMEM((dm, ffn), _BF16),
            pltpu.VMEM((dm, ffn), _BF16),
            pltpu.VMEM((dm, ffn), _BF16),
            pltpu.VMEM((ffn, dm), _BF16),
            pltpu.VMEM((n_heads // 2, _LANES, 3 * dh), _BF16),
            pltpu.VMEM((_LANES, ffn // 2), _BF16),
            pltpu.VMEM((_LANES, ffn // 2), _BF16),
            pltpu.VMEM((rows, dm - _HALF + 2 * _LANES), _BF16),
            pltpu.VMEM((rows, n_heads * dh), _BF16),
            pltpu.VMEM((2 * seg, ffn), _BF16),
            pltpu.VMEM((2 * seg, dm), _F32),
            pltpu.VMEM((2 * seg, dm), _F32),
            pltpu.VMEM((seq, dm), _BF16),
            pltpu.SemaphoreType.DMA((3 + 3 * _QKV_DMA_CHUNKS + 3 * _FFN_DMA_CHUNKS,)),
            pltpu.SemaphoreType.DMA((seq // _XPOSE_CHUNK,)),
        ],
        compiler_params=pltpu.CompilerParams(vmem_limit_bytes=110 * 1024 * 1024),
    )(
        A_x.reshape(seq, dm).T,
        A_mem0.reshape(n_mem, dm),
        A_Wq.reshape(dm * n_heads, dh),
        A_Wk.reshape(dm * n_heads, dh),
        A_Wv.reshape(dm * n_heads, dh),
        A_Wo.transpose(0, 2, 1),
        B_w1,
        B_w3,
        B_w2.T,
    )
    return out_t.T.reshape(batch, seq, dm)
```

```python
import functools

import jax
import jax.numpy as jnp
import numpy as np
import jax.experimental.pallas as pl
import jax.experimental.pallas.tpu as pltpu

_EPS = 1e-5
_MASK_FILL = -1000000000.0
_HEADS_PER_DOT = 2
_QK_LAG = 1
_PV_LAG = 2
_FFN_CHUNK = 512
_XPOSE_CHUNK = 256
_FFN_DMA_CHUNKS = 3
_QKV_DMA_CHUNKS = 2
_WORD_TILE = 4

_LANES = 128
_HALF = _LANES // 2
_F32 = jnp.float32
_BF16 = jnp.bfloat16


def _layernorm(x):
    mean = jnp.mean(x, axis=-1, keepdims=True)
    cen = x - mean
    var = jnp.mean(cen * cen, axis=-1, keepdims=True)
    return cen * jax.lax.rsqrt(var + _EPS)


def _dot(a, b):
    return jnp.dot(a, b, preferred_element_type=_F32)


def _dot_nt(a, b):
    return jax.lax.dot_general(a, b, (((1,), (1,)), ((), ())), preferred_element_type=_F32)


def _split_lhs(x):
    full = x.shape[1] - _HALF
    first, rest = x[:, :_LANES], x[:, _LANES:full]
    tail = x[:, full:]
    lhs_b0 = jnp.concatenate([first[:, :_HALF], tail], axis=1)
    lhs_s = jnp.concatenate([tail, first[:, _HALF:]], axis=1)
    return jnp.concatenate([first, rest, lhs_b0, lhs_s], axis=1).astype(_BF16)


def _paired_dot(lhs, w_a, w_b, w_s):
    full = w_a.shape[0]
    shared = _dot(lhs[:, full + _LANES:], w_s)
    lhs_b = jnp.concatenate([lhs[:, full:full + _LANES], lhs[:, _LANES:full]], axis=1)
    return _dot(lhs[:, :full], w_a) + shared, _dot(lhs_b, w_b) + shared


def _pair_weights(a_mid, a_tail, b_mid, b_tail):
    a_new = (a_mid.astype(_F32) - b_mid.astype(_F32)).astype(_BF16)
    b_new = (b_tail.astype(_F32) - a_tail.astype(_F32)).astype(_BF16)
    return a_new, b_new, jnp.concatenate([a_tail, b_mid], axis=0)


def _pair_output_weights(ut, vt):
    full = ut.shape[0] - _HALF
    mid = slice(_HALF, _LANES)
    u_new, v_new, shared = _pair_weights(ut[mid], ut[full:], vt[mid], vt[full:])
    u = jnp.concatenate([ut[:_HALF], u_new, ut[_LANES:full]], axis=0)
    v = jnp.concatenate([vt[:_HALF], v_new, vt[_LANES:full]], axis=0)
    return u.T, v.T, shared.T


def _output_passes(lhs_ref, rows, w_ref, s_ref):
    half = s_ref.shape[0]
    u, v, uv = slice(0, half), slice(half, 2 * half), slice(2 * half, 3 * half)
    got = {}

    def wide(name, part):
        return lambda: got.__setitem__(name, _dot(lhs_ref[rows, part], w_ref[part, _LANES:]))

    def narrow():
        got["u0"] = _dot(lhs_ref[rows, u], w_ref[u, 0:_LANES])
        got["v0"] = _dot(lhs_ref[rows, v], w_ref[v, 0:_LANES])
        got["shared"] = _dot(lhs_ref[rows, uv], s_ref[...])

    def combine():
        u0, v0, shared = got["u0"], got["v0"], got["shared"]
        is_low = jax.lax.broadcasted_iota(jnp.int32, u0.shape, 1) < _HALF
        first = u0 + jnp.where(is_low, v0, shared)
        last = v0[:, _HALF:] + shared[:, :_HALF]
        return jnp.concatenate([first, got["u"] + got["v"], last], axis=1)

    return [wide("u", u), wide("v", v), narrow], combine


def _output_dot(lhs_ref, rows, w_ref, s_ref):
    passes, combine = _output_passes(lhs_ref, rows, w_ref, s_ref)
    for run in passes:
        run()
    return combine()


def _mask_tables(n_streams, n_mem, seg):
    tok0 = n_streams * n_mem
    rows = tok0 + n_streams * seg

    def split(axis):
        idx = jax.lax.broadcasted_iota(jnp.int32, (rows, rows), axis)
        is_mem = idx < tok0
        stream = jnp.where(is_mem, idx // n_mem, (idx - tok0) // seg)
        pos = jnp.where(is_mem, idx % n_mem, n_mem + (idx - tok0) % seg)
        return stream, pos

    q_stream, q_pos = split(0)
    k_stream, k_pos = split(1)
    same = q_stream == k_stream
    visible = same & ((q_pos < n_mem) | (q_pos >= k_pos))
    fill = jnp.where(same, _MASK_FILL, -jnp.inf).astype(_F32)
    return visible, fill


def _kernel(xt_hbm, mem0_ref, wq_hbm, wk_hbm, wv_hbm, wot_hbm, w1_hbm, w3_hbm, w2t_hbm,
            out_hbm,
            xt_ref, x_ref, rq_ref, rk_ref, rv_ref, wqkv_ref, wot_ref, wo_ref,
            w1_ref, w3_ref, w2t_ref, w2_ref, sqkv_ref, s1_ref, s3_ref, so_ref, s2_ref,
            h_ref, o_ref, hid_ref, xa_ref, x1_ref, y_ref, in_sems, out_sems,
            *, seg, n_heads, dh):
    seq, dm = x_ref.shape
    n_mem = mem0_ref.shape[0]
    n_seg = seq // seg
    ffn = w1_ref.shape[1]
    scale = dh ** -0.5
    hpd = _HEADS_PER_DOT
    n_grp = n_heads // hpd
    tok0 = 2 * n_mem
    full = dm - _HALF
    mid = slice(_HALF, _LANES)
    fc = _FFN_CHUNK
    xc = _XPOSE_CHUNK
    wc = ffn // _FFN_DMA_CHUNKS

    def cols(ref, start, size):
        return ref.at[:, start:start + size]

    def rows_of(ref, start, size):
        return ref.at[start:start + size, :]

    raw_rows = dm * n_heads // _QKV_DMA_CHUNKS
    transfers = [("x_head", cols(xt_hbm, 0, xc), cols(xt_ref, 0, xc))]
    for name, src, dst in (("wq", wq_hbm, rq_ref), ("wk", wk_hbm, rk_ref), ("wv", wv_hbm, rv_ref)):
        for c in range(_QKV_DMA_CHUNKS):
            transfers.append(((name, c), rows_of(src, c * raw_rows, raw_rows),
                              rows_of(dst, c * raw_rows, raw_rows)))
    transfers.append(("wo", wot_hbm, wot_ref))
    for c in range(0, ffn, wc):
        transfers.append((("w1", c), cols(w1_hbm, c, wc), cols(w1_ref, c, wc)))
        transfers.append((("w3", c), cols(w3_hbm, c, wc), cols(w3_ref, c, wc)))
    transfers.append(("x_tail", cols(xt_hbm, xc, seq - xc), cols(xt_ref, xc, seq - xc)))
    for c in range(0, ffn, wc):
        transfers.append((("w2", c), cols(w2t_hbm, c, wc), cols(w2t_ref, c, wc)))
    copies = {name: pltpu.make_async_copy(src, dst, in_sems.at[n])
              for n, (name, src, dst) in enumerate(transfers)}

    def arrive(name):
        copies[name].wait()

    def project(h, grp):
        both = _paired_dot(h, wqkv_ref[grp, 0:full, 0:3 * dh], wqkv_ref[grp, 0:full, 3 * dh:],
                           sqkv_ref[grp])
        return [[qkv[:, m * dh:(m + 1) * dh].astype(_BF16) for m in range(3)] for qkv in both]

    def probabilities(qkv, visible, fill):
        probs = []
        for q, k, _ in qkv:
            s = jnp.where(visible, _dot_nt(q, k) * scale, fill)
            p = jnp.exp(s - jnp.max(s, axis=-1, keepdims=True))
            probs.append((p * (1.0 / jnp.sum(p, axis=-1, keepdims=True))).astype(_BF16))
        return probs

    def heads(h, n_streams, fillers):
        rows = h.shape[0]
        visible, fill = _mask_tables(n_streams, n_mem, seg)
        qkv, probs = {}, {}
        for t in range(n_grp + _PV_LAG):
            if t < n_grp:
                qkv[t] = project(h, t)
            elif t - n_grp < len(fillers):
                fillers[t - n_grp]()
            if 0 <= t - _QK_LAG < n_grp:
                probs[t - _QK_LAG] = probabilities(qkv[t - _QK_LAG], visible, fill)
            if 0 <= t - _PV_LAG:
                grp = t - _PV_LAG
                outs = [_dot(p, v) for p, (_, _, v) in zip(probs.pop(grp), qkv.pop(grp))]
                for part, out in enumerate(outs + [outs[0] + outs[1]]):
                    col = (part * n_grp + grp) * dh
                    o_ref[0:rows, col:col + dh] = out.astype(_BF16)
        for filler in fillers[_PV_LAG:]:
            filler()

    def attend(h, n_streams, fillers):
        heads(h, n_streams, fillers)
        return _output_dot(o_ref, slice(0, h.shape[0]), wo_ref, so_ref)

    def pair_gate_up(lo, hi):
        for w_ref, s_ref in ((w1_ref, s1_ref), (w3_ref, s3_ref)):
            for c in range(lo, hi, fc):
                ca, cb = slice(c, c + fc // 2), slice(c + fc // 2, c + fc)
                w_ref[mid, ca], w_ref[mid, cb], s_ref[:, c // 2:(c + fc) // 2] = _pair_weights(
                    w_ref[mid, ca], w_ref[full:, ca], w_ref[mid, cb], w_ref[full:, cb])

    def gate_up(f_in, lo=0, hi=ffn):
        for c in range(lo, hi, fc):
            ca, cb = slice(c, c + fc // 2), slice(c + fc // 2, c + fc)
            cs = slice(c // 2, (c + fc) // 2)
            gates = _paired_dot(f_in, w1_ref[0:full, ca], w1_ref[0:full, cb], s1_ref[:, cs])
            ups = _paired_dot(f_in, w3_ref[0:full, ca], w3_ref[0:full, cb], s3_ref[:, cs])
            hids = [gate * jax.nn.sigmoid(gate) * up for gate, up in zip(gates, ups)]
            for part, hid in enumerate(hids + [hids[0] + hids[1]]):
                col = (part * ffn + c) // 2
                hid_ref[:, col:col + fc // 2] = hid.astype(_BF16)

    def stage_down(lo, hi):
        for c in range(lo, hi, fc):
            rows_u, rows_v = pl.ds(c // 2, fc // 2), pl.ds((ffn + c) // 2, fc // 2)
            w2_ref[rows_u, :], w2_ref[rows_v, :], s2_ref[rows_u, :] = _pair_output_weights(
                w2t_ref[:, c:c + fc // 2], w2t_ref[:, c + fc // 2:c + fc])

    def single_stream_rows(mem, x):
        return _split_lhs(jnp.concatenate([mem, _layernorm(x)], axis=0))

    def write_back(t):
        xt_ref[:, t:t + xc] = y_ref[t:t + xc, :].T
        copy = pltpu.make_async_copy(cols(xt_ref, t, xc), cols(out_hbm, t, xc), out_sems.at[t // xc])
        copy.start()
        return copy

    for copy in copies.values():
        copy.start()
    arrive("x_head")
    x_ref[0:xc, :] = xt_ref[:, 0:xc].T

    pairs = n_heads // 2
    d_chunk = dm // _QKV_DMA_CHUNKS
    for m, (name, raw_ref) in enumerate((("wq", rq_ref), ("wk", rk_ref), ("wv", rv_ref))):
        words = raw_ref.bitcast(jnp.uint32)
        for c in range(_QKV_DMA_CHUNKS):
            arrive((name, c))

            def regroup(quad, carry, m=m, c=c, words=words):
                start = pl.multiple_of(c * d_chunk * pairs + quad * _WORD_TILE, _WORD_TILE)
                view = words.at[pl.ds(start, d_chunk * pairs - pairs + _WORD_TILE), :]
                for r in range(_WORD_TILE):
                    even_d = view[pl.ds(r, d_chunk // 2, stride=n_heads), :]
                    odd_d = view[pl.ds(r + pairs, d_chunk // 2, stride=n_heads), :]
                    lo = (even_d & jnp.uint32(0xFFFF)) | (odd_d << 16)
                    hi = (even_d >> 16) | (odd_d & jnp.uint32(0xFFFF0000))
                    for half, val in enumerate((lo, hi)):
                        grp, hh = divmod(2 * r + half, hpd)
                        col = (hh * 3 + m) * dh
                        wqkv_ref[quad * (2 * _WORD_TILE // hpd) + grp,
                                 c * d_chunk:(c + 1) * d_chunk, col:col + dh] = pltpu.bitcast(val, _BF16)
                return carry

            jax.lax.fori_loop(0, pairs // _WORD_TILE, regroup, 0)

    def pair_heads(grp, carry):
        ca, cb = slice(0, 3 * dh), slice(3 * dh, 6 * dh)
        wqkv_ref[grp, mid, ca], wqkv_ref[grp, mid, cb], sqkv_ref[grp] = _pair_weights(
            wqkv_ref[grp, mid, ca], wqkv_ref[grp, full:, ca],
            wqkv_ref[grp, mid, cb], wqkv_ref[grp, full:, cb])
        return carry

    jax.lax.fori_loop(0, n_grp, pair_heads, 0)

    mem0 = mem0_ref[...].astype(_F32)
    xa_ref[0:n_mem, :] = mem0

    def first_segments(s, carry):
        x_s = x_ref[pl.ds(pl.multiple_of(s * seg, seg), seg), :].astype(_F32)
        heads(single_stream_rows(xa_ref[0:n_mem, :], x_s), 1, [])

        @pl.when(s == 0)
        def _():
            arrive("wo")

            def stage_wo(grp, carry):
                rows_u = pl.ds(pl.multiple_of(grp * dh, dh), dh)
                rows_v = pl.ds(pl.multiple_of((n_grp + grp) * dh, dh), dh)
                wo_ref[rows_u, :], wo_ref[rows_v, :], so_ref[rows_u, :] = _pair_output_weights(
                    wot_ref[2 * grp], wot_ref[2 * grp + 1])
                return carry

            jax.lax.fori_loop(0, n_grp, stage_wo, 0, unroll=2)

        a = _output_dot(o_ref, slice(0, n_mem + seg), wo_ref, so_ref)
        xa_ref[0:n_mem, :] = a[:n_mem]
        x1_ref[pl.ds(pl.multiple_of((1 - s) * seg, seg), seg), :] = x_s + a[n_mem:]
        return carry

    jax.lax.fori_loop(0, 2, first_segments, 0)
    h_ref[0:tok0, :] = _split_lhs(jnp.concatenate([xa_ref[0:n_mem, :], mem0], axis=0))
    f_in = _split_lhs(_layernorm(x1_ref[...]))
    for c in range(0, ffn, wc):
        arrive(("w1", c))
        arrive(("w3", c))
        pair_gate_up(c, c + wc)
        gate_up(f_in, c, c + wc)
    arrive("x_tail")
    for t in range(xc, seq, xc):
        x_ref[t:t + xc, :] = xt_ref[:, t:t + xc].T
    for c in range(0, ffn, wc):
        arrive(("w2", c))
        stage_down(c, c + wc)
    x2_s0 = x1_ref[seg:, :] + _output_dot(hid_ref, slice(seg, 2 * seg), w2_ref, s2_ref)
    xa = jnp.concatenate([x_ref[2 * seg:3 * seg, :].astype(_F32), x2_s0], axis=0)
    xa_ref[...] = xa
    h_ref[tok0:, :] = _split_lhs(_layernorm(xa))

    def step(i, carry):
        x1_prev = x1_ref[...]
        passes, combine = _output_passes(hid_ref, slice(0, 2 * seg), w2_ref, s2_ref)
        a = attend(h_ref[...], 2, passes[:-1])
        h_ref[0:tok0, :] = _split_lhs(a[:tok0])
        x1 = xa_ref[...] + a[tok0:]
        x1_ref[...] = x1
        f_in = _split_lhs(_layernorm(x1))

        passes[-1]()
        y = x1_prev + combine()
        out_row = pl.multiple_of(jnp.maximum(i - 3, 0) * seg, seg)
        y_ref[pl.ds(out_row, seg), :] = y[seg:].astype(y_ref.dtype)
        nxt_row = pl.multiple_of(jnp.minimum(i + 1, n_seg - 1) * seg, seg)
        xa = jnp.concatenate([x_ref[pl.ds(nxt_row, seg), :].astype(_F32), y[:seg]], axis=0)
        xa_ref[...] = xa
        h_ref[tok0:, :] = _split_lhs(_layernorm(xa))
        gate_up(f_in)
        return carry

    jax.lax.fori_loop(2, n_seg, step, 0)

    writes = []
    passes, combine = _output_passes(hid_ref, slice(0, 2 * seg), w2_ref, s2_ref)
    h = h_ref[...].astype(_F32)
    h = jnp.concatenate([h[n_mem:tok0], h[tok0 + seg:]], axis=0).astype(_BF16)
    x_s0 = xa_ref[seg:, :]
    a = attend(h, 1, passes[:-1])
    passes[-1]()
    y = x1_ref[...] + combine()
    y_ref[seq - 3 * seg:seq - 2 * seg, :] = y[seg:].astype(y_ref.dtype)
    x1_s0 = x_s0 + a[n_mem:]
    x_s1 = y[:seg]
    for t in range(0, seq - xc, xc):
        writes.append(write_back(t))
    a = attend(single_stream_rows(a[:n_mem], x_s1), 1, [])
    x1 = jnp.concatenate([x1_s0, x_s1 + a[n_mem:]], axis=0)
    gate_up(_split_lhs(_layernorm(x1)))
    y_ref[seq - 2 * seg:, :] = (
        x1 + _output_dot(hid_ref, slice(0, 2 * seg), w2_ref, s2_ref)).astype(y_ref.dtype)
    writes.append(write_back(seq - xc))
    for copy in writes:
        copy.wait()


@functools.partial(jax.jit, static_argnames=("A_seg_len",))
def pallas_interleave_layers__memory_aug_recurrent_mem_tr__glu_gated_swiglu__prompt_kernel(
    A_x: jax.Array,
    A_mem0: jax.Array,
    A_Wq: jax.Array,
    A_Wk: jax.Array,
    A_Wv: jax.Array,
    A_Wo: jax.Array,
    A_seg_len: int,
    B_x: jax.Array,
    B_w1: jax.Array,
    B_w3: jax.Array,
    B_w2: jax.Array,
):
    del B_x
    batch, seq, dm = A_x.shape
    _, n_heads, dh = A_Wq.shape
    n_mem = A_mem0.shape[1]
    ffn = B_w1.shape[1]
    seg = int(A_seg_len)
    assert batch == 1 and seq % _XPOSE_CHUNK == 0 and _XPOSE_CHUNK % seg == 0 and _XPOSE_CHUNK >= 3 * seg
    rows = 2 * (n_mem + seg)

    vmem = pl.BlockSpec(memory_space=pltpu.VMEM)
    hbm = pl.BlockSpec(memory_space=pltpu.HBM)
    out_t = pl.pallas_call(
        functools.partial(_kernel, seg=seg, n_heads=n_heads, dh=dh),
        out_shape=jax.ShapeDtypeStruct((dm, seq), A_x.dtype),
        in_specs=[hbm, vmem] + [hbm] * 7,
        out_specs=hbm,
        scratch_shapes=[
            pltpu.VMEM((dm, seq), _BF16),
            pltpu.VMEM((seq, dm), _BF16),
            pltpu.VMEM((dm * n_heads, dh), _BF16),
            pltpu.VMEM((dm * n_heads, dh), _BF16),
            pltpu.VMEM((dm * n_heads, dh), _BF16),
            pltpu.VMEM((n_heads // _HEADS_PER_DOT, dm, 3 * dh * _HEADS_PER_DOT), _BF16),
            pltpu.VMEM((n_heads, dm, dh), _BF16),
            pltpu.VMEM((n_heads * dh, dm - _HALF), _BF16),
            pltpu.VMEM((dm, ffn), _BF16),
            pltpu.VMEM((dm, ffn), _BF16),
            pltpu.VMEM((dm, ffn), _BF16),
            pltpu.VMEM((ffn, dm - _HALF), _BF16),
            pltpu.VMEM((n_heads // 2, _LANES, 3 * dh), _BF16),
            pltpu.VMEM((_LANES, ffn // 2), _BF16),
            pltpu.VMEM((_LANES, ffn // 2), _BF16),
            pltpu.VMEM((n_heads * dh // 2, _LANES), _BF16),
            pltpu.VMEM((ffn // 2, _LANES), _BF16),
            pltpu.VMEM((rows, dm - _HALF + 2 * _LANES), _BF16),
            pltpu.VMEM((rows, n_heads * dh * 3 // 2), _BF16),
            pltpu.VMEM((2 * seg, ffn * 3 // 2), _BF16),
            pltpu.VMEM((2 * seg, dm), _F32),
            pltpu.VMEM((2 * seg, dm), _F32),
            pltpu.VMEM((seq, dm), _BF16),
            pltpu.SemaphoreType.DMA((3 + 3 * _QKV_DMA_CHUNKS + 3 * _FFN_DMA_CHUNKS,)),
            pltpu.SemaphoreType.DMA((seq // _XPOSE_CHUNK,)),
        ],
        compiler_params=pltpu.CompilerParams(vmem_limit_bytes=110 * 1024 * 1024),
    )(
        A_x.reshape(seq, dm).T,
        A_mem0.reshape(n_mem, dm),
        A_Wq.reshape(dm * n_heads, dh),
        A_Wk.reshape(dm * n_heads, dh),
        A_Wv.reshape(dm * n_heads, dh),
        A_Wo.transpose(0, 2, 1),
        B_w1,
        B_w3,
        B_w2.T,
    )
    return out_t.T.reshape(batch, seq, dm)
```

```python
import functools

import jax
import jax.numpy as jnp
import numpy as np
import jax.experimental.pallas as pl
import jax.experimental.pallas.tpu as pltpu

_EPS = 1e-5
_MASK_FILL = -1000000000.0
_HEADS_PER_DOT = 2
_QK_LAG = 1
_PV_LAG = 4
_FFN_CHUNK = 512
_XPOSE_CHUNK = 256
_FFN_DMA_CHUNKS = 3
_QKV_DMA_CHUNKS = 2
_WORD_TILE = 4

_LANES = 128
_HALF = _LANES // 2
_F32 = jnp.float32
_BF16 = jnp.bfloat16


def _layernorm(x):
    mean = jnp.mean(x, axis=-1, keepdims=True)
    cen = x - mean
    var = jnp.mean(cen * cen, axis=-1, keepdims=True)
    return cen * jax.lax.rsqrt(var + _EPS)


def _dot(a, b):
    return jnp.dot(a, b, preferred_element_type=_F32)


def _dot_nt(a, b):
    return jax.lax.dot_general(a, b, (((1,), (1,)), ((), ())), preferred_element_type=_F32)


def _split_lhs(x):
    full = x.shape[1] - _HALF
    first, rest = x[:, :_LANES], x[:, _LANES:full]
    tail = x[:, full:]
    lhs_b0 = jnp.concatenate([first[:, :_HALF], tail], axis=1)
    lhs_s = jnp.concatenate([tail, first[:, _HALF:]], axis=1)
    return jnp.concatenate([first, rest, lhs_b0, lhs_s], axis=1).astype(_BF16)


def _paired_dot(lhs, w_a, w_b, w_s):
    full = w_a.shape[0]
    shared = _dot(lhs[:, full + _LANES:], w_s)
    lhs_b = jnp.concatenate([lhs[:, full:full + _LANES], lhs[:, _LANES:full]], axis=1)
    return _dot(lhs[:, :full], w_a) + shared, _dot(lhs_b, w_b) + shared


def _pair_weights(a_mid, a_tail, b_mid, b_tail):
    a_new = (a_mid.astype(_F32) - b_mid.astype(_F32)).astype(_BF16)
    b_new = (b_tail.astype(_F32) - a_tail.astype(_F32)).astype(_BF16)
    return a_new, b_new, jnp.concatenate([a_tail, b_mid], axis=0)


def _pair_output_weights(ut, vt):
    full = ut.shape[0] - _HALF
    mid = slice(_HALF, _LANES)
    u_new, v_new, shared = _pair_weights(ut[mid], ut[full:], vt[mid], vt[full:])
    u = jnp.concatenate([ut[:_HALF], u_new, ut[_LANES:full]], axis=0)
    v = jnp.concatenate([vt[:_HALF], v_new, vt[_LANES:full]], axis=0)
    return u.T, v.T, shared.T


def _output_wide(lhs_ref, rows, w_ref, lo=0, hi=None):
    hi = w_ref.shape[0] if hi is None else hi
    return _dot(lhs_ref[rows, lo:hi], w_ref[lo:hi, _LANES:])


def _output_finish(lhs_ref, rows, w_ref, s_ref, wide):
    half = s_ref.shape[0]
    u0 = _dot(lhs_ref[rows, 0:half], w_ref[0:half, 0:_LANES])
    v0 = _dot(lhs_ref[rows, half:2 * half], w_ref[half:, 0:_LANES])
    shared = _dot(lhs_ref[rows, 2 * half:], s_ref[...])
    is_low = jax.lax.broadcasted_iota(jnp.int32, u0.shape, 1) < _HALF
    first = u0 + jnp.where(is_low, v0, shared)
    last = v0[:, _HALF:] + shared[:, :_HALF]
    return jnp.concatenate([first, wide, last], axis=1)


def _output_dot(lhs_ref, rows, w_ref, s_ref):
    return _output_finish(lhs_ref, rows, w_ref, s_ref, _output_wide(lhs_ref, rows, w_ref))


def _mask_tables(n_streams, n_mem, seg):
    tok0 = n_streams * n_mem
    rows = tok0 + n_streams * seg

    def split(axis):
        idx = jax.lax.broadcasted_iota(jnp.int32, (rows, rows), axis)
        is_mem = idx < tok0
        stream = jnp.where(is_mem, idx // n_mem, (idx - tok0) // seg)
        pos = jnp.where(is_mem, idx % n_mem, n_mem + (idx - tok0) % seg)
        return stream, pos

    q_stream, q_pos = split(0)
    k_stream, k_pos = split(1)
    same = q_stream == k_stream
    visible = same & ((q_pos < n_mem) | (q_pos >= k_pos))
    fill = jnp.where(same, _MASK_FILL, -jnp.inf).astype(_F32)
    return visible, fill


def _kernel(xt_hbm, mem0_ref, wq_hbm, wk_hbm, wv_hbm, wot_hbm, w1_hbm, w3_hbm, w2t_hbm,
            out_hbm,
            xt_ref, x_ref, rq_ref, rk_ref, rv_ref, wqkv_ref, wot_ref, wo_ref,
            w1_ref, w3_ref, w2t_ref, w2_ref, sqkv_ref, s1_ref, s3_ref, so_ref, s2_ref,
            o_ref, hid_ref, a_ref, xa_ref, x1_ref, wide_ref, y_ref, in_sems, out_sems,
            *, seg, n_heads, dh):
    seq, dm = x_ref.shape
    n_mem = mem0_ref.shape[0]
    n_seg = seq // seg
    ffn = w1_ref.shape[1]
    scale = dh ** -0.5
    hpd = _HEADS_PER_DOT
    n_grp = n_heads // hpd
    tok0 = 2 * n_mem
    full = dm - _HALF
    mid = slice(_HALF, _LANES)
    fc = _FFN_CHUNK
    xc = _XPOSE_CHUNK
    wc = ffn // _FFN_DMA_CHUNKS

    def cols(ref, start, size):
        return ref.at[:, start:start + size]

    def rows_of(ref, start, size):
        return ref.at[start:start + size, :]

    raw_rows = dm * n_heads // _QKV_DMA_CHUNKS
    transfers = [("x_head", cols(xt_hbm, 0, xc), cols(xt_ref, 0, xc))]
    for name, src, dst in (("wq", wq_hbm, rq_ref), ("wk", wk_hbm, rk_ref), ("wv", wv_hbm, rv_ref)):
        for c in range(_QKV_DMA_CHUNKS):
            transfers.append(((name, c), rows_of(src, c * raw_rows, raw_rows),
                              rows_of(dst, c * raw_rows, raw_rows)))
    transfers.append(("wo", wot_hbm, wot_ref))
    for c in range(0, ffn, wc):
        transfers.append((("w1", c), cols(w1_hbm, c, wc), cols(w1_ref, c, wc)))
        transfers.append((("w3", c), cols(w3_hbm, c, wc), cols(w3_ref, c, wc)))
    transfers.append(("x_tail", cols(xt_hbm, xc, seq - xc), cols(xt_ref, xc, seq - xc)))
    for c in range(0, ffn, wc):
        transfers.append((("w2", c), cols(w2t_hbm, c, wc), cols(w2t_ref, c, wc)))
    copies = {name: pltpu.make_async_copy(src, dst, in_sems.at[n])
              for n, (name, src, dst) in enumerate(transfers)}

    def arrive(name):
        copies[name].wait()

    def project(h, grp):
        both = _paired_dot(h, wqkv_ref[grp, 0:full, 0:3 * dh], wqkv_ref[grp, 0:full, 3 * dh:],
                           sqkv_ref[grp])
        return [[qkv[:, m * dh:(m + 1) * dh].astype(_BF16) for m in range(3)] for qkv in both]

    def probabilities(qkv, visible, fill):
        probs = []
        for q, k, _ in qkv:
            s = jnp.where(visible, _dot_nt(q, k) * scale, fill)
            p = jnp.exp(s - jnp.max(s, axis=-1, keepdims=True))
            probs.append((p * (1.0 / jnp.sum(p, axis=-1, keepdims=True))).astype(_BF16))
        return probs

    def heads(h, n_streams, fillers=()):
        rows = h.shape[0]
        visible, fill = _mask_tables(n_streams, n_mem, seg)
        qkv, probs = {}, {}
        for t in range(n_grp + _PV_LAG):
            if t < n_grp:
                qkv[t] = project(h, t)
            elif t - n_grp < len(fillers):
                fillers[t - n_grp]()
            if 0 <= t - _QK_LAG < n_grp:
                probs[t - _QK_LAG] = probabilities(qkv[t - _QK_LAG], visible, fill)
            if 0 <= t - _PV_LAG:
                grp = t - _PV_LAG
                outs = [_dot(p, v) for p, (_, _, v) in zip(probs.pop(grp), qkv.pop(grp))]
                for part, out in enumerate(outs + [outs[0] + outs[1]]):
                    col = (part * n_grp + grp) * dh
                    o_ref[0:rows, col:col + dh] = out.astype(_BF16)

    def attend(h, n_streams):
        rows, half, wide = slice(0, h.shape[0]), n_grp * dh, []
        cut_u, cut_v = (n_grp - _PV_LAG) * dh, half + (n_grp - _PV_LAG + 1) * dh

        def part(lo, hi):
            return lambda: wide.append(_output_wide(o_ref, rows, wo_ref, lo, hi))

        heads(h, n_streams, (part(0, cut_u), part(half, cut_v)))
        part(cut_u, half)()
        part(cut_v, 2 * half)()
        wide = (wide[0] + wide[1]) + (wide[2] + wide[3])
        return _output_finish(o_ref, rows, wo_ref, so_ref, wide)

    def pair_gate_up(lo, hi):
        for w_ref, s_ref in ((w1_ref, s1_ref), (w3_ref, s3_ref)):
            for c in range(lo, hi, fc):
                ca, cb = slice(c, c + fc // 2), slice(c + fc // 2, c + fc)
                w_ref[mid, ca], w_ref[mid, cb], s_ref[:, c // 2:(c + fc) // 2] = _pair_weights(
                    w_ref[mid, ca], w_ref[full:, ca], w_ref[mid, cb], w_ref[full:, cb])

    def gate_up(f_in, lo=0, hi=ffn):
        for c in range(lo, hi, fc):
            ca, cb = slice(c, c + fc // 2), slice(c + fc // 2, c + fc)
            cs = slice(c // 2, (c + fc) // 2)
            gates = _paired_dot(f_in, w1_ref[0:full, ca], w1_ref[0:full, cb], s1_ref[:, cs])
            ups = _paired_dot(f_in, w3_ref[0:full, ca], w3_ref[0:full, cb], s3_ref[:, cs])
            hids = [gate * jax.nn.sigmoid(gate) * up for gate, up in zip(gates, ups)]
            for part, hid in enumerate(hids + [hids[0] + hids[1]]):
                col = (part * ffn + c) // 2
                hid_ref[0:hid.shape[0], col:col + fc // 2] = hid.astype(_BF16)

    def stage_down(lo, hi):
        for c in range(lo, hi, fc):
            rows_u, rows_v = pl.ds(c // 2, fc // 2), pl.ds((ffn + c) // 2, fc // 2)
            w2_ref[rows_u, :], w2_ref[rows_v, :], s2_ref[rows_u, :] = _pair_output_weights(
                w2t_ref[:, c:c + fc // 2], w2t_ref[:, c + fc // 2:c + fc])

    def single_stream_rows(mem, x):
        return _split_lhs(jnp.concatenate([mem, _layernorm(x)], axis=0))

    def write_back(t, size):
        xt_ref[:, t:t + size] = y_ref[t:t + size, :].T
        copy = pltpu.make_async_copy(
            cols(xt_ref, t, size), cols(out_hbm, t, size), out_sems.at[pl.cdiv(t, xc)])
        copy.start()
        return copy

    for copy in copies.values():
        copy.start()
    arrive("x_head")
    x_ref[0:xc, :] = xt_ref[:, 0:xc].T

    pairs = n_heads // 2
    d_chunk = dm // _QKV_DMA_CHUNKS
    for m, (name, raw_ref) in enumerate((("wq", rq_ref), ("wk", rk_ref), ("wv", rv_ref))):
        words = raw_ref.bitcast(jnp.uint32)
        for c in range(_QKV_DMA_CHUNKS):
            arrive((name, c))

            def regroup(quad, carry, m=m, c=c, words=words):
                start = pl.multiple_of(c * d_chunk * pairs + quad * _WORD_TILE, _WORD_TILE)
                view = words.at[pl.ds(start, d_chunk * pairs - pairs + _WORD_TILE), :]
                for r in range(_WORD_TILE):
                    even_d = view[pl.ds(r, d_chunk // 2, stride=n_heads), :]
                    odd_d = view[pl.ds(r + pairs, d_chunk // 2, stride=n_heads), :]
                    lo = (even_d & jnp.uint32(0xFFFF)) | (odd_d << 16)
                    hi = (even_d >> 16) | (odd_d & jnp.uint32(0xFFFF0000))
                    for half, val in enumerate((lo, hi)):
                        grp, hh = divmod(2 * r + half, hpd)
                        col = (hh * 3 + m) * dh
                        wqkv_ref[quad * (2 * _WORD_TILE // hpd) + grp,
                                 c * d_chunk:(c + 1) * d_chunk, col:col + dh] = pltpu.bitcast(val, _BF16)
                return carry

            jax.lax.fori_loop(0, pairs // _WORD_TILE, regroup, 0)

    def pair_heads(grp, carry):
        ca, cb = slice(0, 3 * dh), slice(3 * dh, 6 * dh)
        wqkv_ref[grp, mid, ca], wqkv_ref[grp, mid, cb], sqkv_ref[grp] = _pair_weights(
            wqkv_ref[grp, mid, ca], wqkv_ref[grp, full:, ca],
            wqkv_ref[grp, mid, cb], wqkv_ref[grp, full:, cb])
        return carry

    jax.lax.fori_loop(0, n_grp, pair_heads, 0)

    mem0 = mem0_ref[...].astype(_F32)
    a_ref[0:n_mem, :] = mem0

    def first_segments(s, carry):
        x_s = x_ref[pl.ds(pl.multiple_of(s * seg, seg), seg), :].astype(_F32)
        heads(single_stream_rows(a_ref[0:n_mem, :], x_s), 1)

        @pl.when(s == 0)
        def _():
            arrive("wo")

            def stage_wo(grp, carry):
                rows_u = pl.ds(pl.multiple_of(grp * dh, dh), dh)
                rows_v = pl.ds(pl.multiple_of((n_grp + grp) * dh, dh), dh)
                wo_ref[rows_u, :], wo_ref[rows_v, :], so_ref[rows_u, :] = _pair_output_weights(
                    wot_ref[2 * grp], wot_ref[2 * grp + 1])
                return carry

            jax.lax.fori_loop(0, n_grp, stage_wo, 0, unroll=2)

        a = _output_dot(o_ref, slice(0, n_mem + seg), wo_ref, so_ref)
        a_ref[0:n_mem, :] = a[:n_mem]
        a_ref[pl.ds(pl.multiple_of(tok0 + (1 - s) * seg, n_mem), seg), :] = a[n_mem:]
        return carry

    jax.lax.fori_loop(0, 2, first_segments, 0)
    zeros = jnp.zeros((seg, dm), _F32)
    x1_s0 = x_ref[0:seg, :].astype(_F32) + a_ref[tok0 + seg:, :]
    a_ref[n_mem:tok0, :] = mem0
    a_ref[tok0 + seg:, :] = zeros
    xa_ref[...] = jnp.concatenate([x_ref[seg:2 * seg, :].astype(_F32), zeros], axis=0)
    x1_ref[...] = jnp.concatenate([x1_s0, zeros], axis=0)
    hid_ref[seg:, :] = jnp.zeros((seg, hid_ref.shape[1]), _BF16)
    f_in = _split_lhs(_layernorm(x1_s0))
    for c in range(0, ffn, wc):
        arrive(("w1", c))
        arrive(("w3", c))
        pair_gate_up(c, c + wc)
        gate_up(f_in, c, c + wc)
    arrive("x_tail")
    for t in range(xc, seq, xc):
        x_ref[t:t + xc, :] = xt_ref[:, t:t + xc].T
    for c in range(0, ffn, wc):
        arrive(("w2", c))
        stage_down(c, c + wc)
    wide_ref[0:seg, :] = _output_wide(hid_ref, slice(0, seg), w2_ref)
    wide_ref[seg:, :] = jnp.zeros((seg, wide_ref.shape[1]), _F32)

    both = slice(0, 2 * seg)

    def feed_forward(out_row):
        y = x1_ref[...] + _output_finish(hid_ref, both, w2_ref, s2_ref, wide_ref[...])
        y_ref[pl.ds(out_row, seg), :] = y[seg:].astype(y_ref.dtype)
        x1 = xa_ref[...] + a_ref[tok0:, :]
        x1_ref[...] = x1
        gate_up(_split_lhs(_layernorm(x1)))
        return y[:seg]

    def step(i, carry):
        x2 = feed_forward(pl.multiple_of(jnp.maximum(i - 3, 0) * seg, seg))
        nxt_row = pl.multiple_of((i + 1) * seg, seg)
        xa = jnp.concatenate([x_ref[pl.ds(nxt_row, seg), :].astype(_F32), x2], axis=0)
        xa_ref[...] = xa
        wide_ref[...] = _output_wide(hid_ref, both, w2_ref)
        a_ref[...] = attend(
            _split_lhs(jnp.concatenate([a_ref[0:tok0, :], _layernorm(xa)], axis=0)), 2)
        return carry

    jax.lax.fori_loop(1, n_seg - 1, step, 0)

    x_s0 = feed_forward(seq - 4 * seg)
    a = attend(single_stream_rows(a_ref[n_mem:tok0, :], x_s0), 1)
    y = x1_ref[...] + _output_dot(hid_ref, both, w2_ref, s2_ref)
    y_ref[seq - 3 * seg:seq - 2 * seg, :] = y[seg:].astype(y_ref.dtype)
    x1_s0 = x_s0 + a[n_mem:]
    last = seq - _LANES
    writes = [write_back(t, min(xc, last - t)) for t in range(0, last, xc)]
    a = attend(single_stream_rows(a[:n_mem], y[:seg]), 1)
    x1 = jnp.concatenate([x1_s0, y[:seg] + a[n_mem:]], axis=0)
    gate_up(_split_lhs(_layernorm(x1)))
    y_ref[seq - 2 * seg:, :] = (x1 + _output_dot(hid_ref, both, w2_ref, s2_ref)).astype(y_ref.dtype)
    writes.append(write_back(last, _LANES))
    for copy in writes:
        copy.wait()


@functools.partial(jax.jit, static_argnames=("A_seg_len",))
def pallas_interleave_layers__memory_aug_recurrent_mem_tr__glu_gated_swiglu__prompt_kernel(
    A_x: jax.Array,
    A_mem0: jax.Array,
    A_Wq: jax.Array,
    A_Wk: jax.Array,
    A_Wv: jax.Array,
    A_Wo: jax.Array,
    A_seg_len: int,
    B_x: jax.Array,
    B_w1: jax.Array,
    B_w3: jax.Array,
    B_w2: jax.Array,
):
    del B_x
    batch, seq, dm = A_x.shape
    _, n_heads, dh = A_Wq.shape
    n_mem = A_mem0.shape[1]
    ffn = B_w1.shape[1]
    seg = int(A_seg_len)
    assert batch == 1 and seq % _XPOSE_CHUNK == 0 and _XPOSE_CHUNK % seg == 0 and _XPOSE_CHUNK >= 3 * seg
    rows = 2 * (n_mem + seg)

    vmem = pl.BlockSpec(memory_space=pltpu.VMEM)
    hbm = pl.BlockSpec(memory_space=pltpu.HBM)
    out_t = pl.pallas_call(
        functools.partial(_kernel, seg=seg, n_heads=n_heads, dh=dh),
        out_shape=jax.ShapeDtypeStruct((dm, seq), A_x.dtype),
        in_specs=[hbm, vmem] + [hbm] * 7,
        out_specs=hbm,
        scratch_shapes=[
            pltpu.VMEM((dm, seq), _BF16),
            pltpu.VMEM((seq, dm), _BF16),
            pltpu.VMEM((dm * n_heads, dh), _BF16),
            pltpu.VMEM((dm * n_heads, dh), _BF16),
            pltpu.VMEM((dm * n_heads, dh), _BF16),
            pltpu.VMEM((n_heads // _HEADS_PER_DOT, dm, 3 * dh * _HEADS_PER_DOT), _BF16),
            pltpu.VMEM((n_heads, dm, dh), _BF16),
            pltpu.VMEM((n_heads * dh, dm - _HALF), _BF16),
            pltpu.VMEM((dm, ffn), _BF16),
            pltpu.VMEM((dm, ffn), _BF16),
            pltpu.VMEM((dm, ffn), _BF16),
            pltpu.VMEM((ffn, dm - _HALF), _BF16),
            pltpu.VMEM((n_heads // 2, _LANES, 3 * dh), _BF16),
            pltpu.VMEM((_LANES, ffn // 2), _BF16),
            pltpu.VMEM((_LANES, ffn // 2), _BF16),
            pltpu.VMEM((n_heads * dh // 2, _LANES), _BF16),
            pltpu.VMEM((ffn // 2, _LANES), _BF16),
            pltpu.VMEM((rows, n_heads * dh * 3 // 2), _BF16),
            pltpu.VMEM((2 * seg, ffn * 3 // 2), _BF16),
            pltpu.VMEM((rows, dm), _F32),
            pltpu.VMEM((2 * seg, dm), _F32),
            pltpu.VMEM((2 * seg, dm), _F32),
            pltpu.VMEM((2 * seg, dm - _HALF - _LANES), _F32),
            pltpu.VMEM((seq, dm), _BF16),
            pltpu.SemaphoreType.DMA((3 + 3 * _QKV_DMA_CHUNKS + 3 * _FFN_DMA_CHUNKS,)),
            pltpu.SemaphoreType.DMA((seq // _XPOSE_CHUNK + 1,)),
        ],
        compiler_params=pltpu.CompilerParams(vmem_limit_bytes=110 * 1024 * 1024),
    )(
        A_x.reshape(seq, dm).T,
        A_mem0.reshape(n_mem, dm),
        A_Wq.reshape(dm * n_heads, dh),
        A_Wk.reshape(dm * n_heads, dh),
        A_Wv.reshape(dm * n_heads, dh),
        A_Wo.transpose(0, 2, 1),
        B_w1,
        B_w3,
        B_w2.T,
    )
    return out_t.T.reshape(batch, seq, dm)
```

```python
import functools

import jax
import jax.numpy as jnp
import numpy as np
import jax.experimental.pallas as pl
import jax.experimental.pallas.tpu as pltpu

_EPS = 1e-5
_MASK_FILL = -1000000000.0
_QK_LAG = 1
_PV_LAG = 4
_FFN_CHUNK = 512
_XPOSE_CHUNK = 256
_FFN_DMA_CHUNKS = 3
_QKV_DMA_CHUNKS = 2
_WORD_TILE = 4

_LANES = 128
_HALF = _LANES // 2
_F32 = jnp.float32
_BF16 = jnp.bfloat16


def _layernorm(x):
    mean = jnp.mean(x, axis=-1, keepdims=True)
    cen = x - mean
    var = jnp.mean(cen * cen, axis=-1, keepdims=True)
    return cen * jax.lax.rsqrt(var + _EPS)


def _dot(a, b):
    return jnp.dot(a, b, preferred_element_type=_F32)


def _dot_nt(a, b):
    return jax.lax.dot_general(a, b, (((1,), (1,)), ((), ())), preferred_element_type=_F32)


class _Packed:
    def __init__(self, ref):
        self.ref = ref
        self.shape = (2 * ref.shape[0], ref.shape[1])

    def _index(self, idx):
        rows, cols = idx
        if isinstance(rows, slice):
            lo, hi, _ = rows.indices(self.shape[0])
            return slice(lo // 2, hi // 2), cols
        start, size = rows
        return pl.ds(pl.multiple_of(start // 2, size // 2), size // 2), cols

    def __getitem__(self, idx):
        return pltpu.bitcast(self.ref[self._index(idx)], _BF16)

    def __setitem__(self, idx, value):
        self.ref[self._index(idx)] = pltpu.bitcast(value, jnp.uint32)


def _packed_scratch(rows, cols):
    return pltpu.VMEM((rows // 2, cols), jnp.uint32)


def _split_lhs(x):
    full = x.shape[1] - _HALF
    first, rest = x[:, :_LANES], x[:, _LANES:full]
    tail = x[:, full:]
    lhs_b0 = jnp.concatenate([first[:, :_HALF], tail], axis=1)
    lhs_s = jnp.concatenate([tail, first[:, _HALF:]], axis=1)
    return jnp.concatenate([first, rest, lhs_b0, lhs_s], axis=1).astype(_BF16)


def _paired_dot(lhs, w_a, w_b, w_s):
    full = w_a.shape[0]
    shared = _dot(lhs[:, full + _LANES:], w_s)
    lhs_b = jnp.concatenate([lhs[:, full:full + _LANES], lhs[:, _LANES:full]], axis=1)
    return _dot(lhs[:, :full], w_a) + shared, _dot(lhs_b, w_b) + shared


def _pair_weights(a_mid, a_tail, b_mid, b_tail):
    a_new = (a_mid.astype(_F32) - b_mid.astype(_F32)).astype(_BF16)
    b_new = (b_tail.astype(_F32) - a_tail.astype(_F32)).astype(_BF16)
    return a_new, b_new, jnp.concatenate([a_tail, b_mid], axis=0)


def _pair_output_weights(ut, vt):
    full = ut.shape[0] - _HALF
    mid = slice(_HALF, _LANES)
    u_new, v_new, shared = _pair_weights(ut[mid], ut[full:], vt[mid], vt[full:])
    u = jnp.concatenate([ut[:_HALF], u_new, ut[_LANES:full]], axis=0)
    v = jnp.concatenate([vt[:_HALF], v_new, vt[_LANES:full]], axis=0)
    return u.T, v.T, shared.T


def _output_wide(lhs_ref, rows, w_ref, lo=0, hi=None):
    hi = w_ref.shape[0] if hi is None else hi
    return _dot(lhs_ref[rows, lo:hi], w_ref[lo:hi, _LANES:])


def _output_finish(lhs_ref, rows, w_ref, s_ref, wide):
    half = s_ref.shape[0]
    u0 = _dot(lhs_ref[rows, 0:half], w_ref[0:half, 0:_LANES])
    v0 = _dot(lhs_ref[rows, half:2 * half], w_ref[half:, 0:_LANES])
    shared = _dot(lhs_ref[rows, 2 * half:], s_ref[:, :])
    is_low = jax.lax.broadcasted_iota(jnp.int32, u0.shape, 1) < _HALF
    first = u0 + jnp.where(is_low, v0, shared)
    last = v0[:, _HALF:] + shared[:, :_HALF]
    return jnp.concatenate([first, wide, last], axis=1)


def _output_dot(lhs_ref, rows, w_ref, s_ref):
    return _output_finish(lhs_ref, rows, w_ref, s_ref, _output_wide(lhs_ref, rows, w_ref))


def _mask_tables(n_streams, n_mem, seg):
    tok0 = n_streams * n_mem
    rows = tok0 + n_streams * seg

    def split(axis):
        idx = jax.lax.broadcasted_iota(jnp.int32, (rows, rows), axis)
        is_mem = idx < tok0
        stream = jnp.where(is_mem, idx // n_mem, (idx - tok0) // seg)
        pos = jnp.where(is_mem, idx % n_mem, n_mem + (idx - tok0) % seg)
        return stream, pos

    q_stream, q_pos = split(0)
    k_stream, k_pos = split(1)
    same = q_stream == k_stream
    visible = same & ((q_pos < n_mem) | (q_pos >= k_pos))
    fill = jnp.where(same, _MASK_FILL, -jnp.inf).astype(_F32)
    return visible, fill


def _kernel(xt_hbm, mem0_ref, wq_hbm, wk_hbm, wv_hbm, wot_hbm, w1_hbm, w3_hbm, w2t_hbm,
            out_hbm,
            xt_ref, x_ref, rq_ref, rk_ref, rv_ref, wqkv_ref, wot_ref, wo_ref,
            r1_ref, r3_ref, w1_ref, w3_ref, w2t_ref, w2_ref, sqkv_ref, s1_ref, s3_ref, so_ref, s2_ref,
            o_ref, hid_ref, a_ref, xa_ref, x1_ref, wide_ref, y_ref, in_sems, out_sems,
            *, seg, n_heads, dh):
    seq, dm = x_ref.shape
    n_mem = mem0_ref.shape[0]
    n_seg = seq // seg
    ffn = w1_ref.shape[1]
    wqkv_ref, wo_ref, w1_ref, w3_ref, w2_ref = map(
        _Packed, (wqkv_ref, wo_ref, w1_ref, w3_ref, w2_ref))
    sqkv_ref, s1_ref, s3_ref, so_ref, s2_ref = map(
        _Packed, (sqkv_ref, s1_ref, s3_ref, so_ref, s2_ref))
    o_ref, hid_ref = _Packed(o_ref), _Packed(hid_ref)
    scale = dh ** -0.5
    n_grp = n_heads // 2
    tok0 = 2 * n_mem
    full = dm - _HALF
    mid = slice(_HALF, _LANES)
    fc = _FFN_CHUNK
    xc = _XPOSE_CHUNK
    wc = ffn // _FFN_DMA_CHUNKS

    def cols(ref, start, size):
        return ref.at[:, start:start + size]

    def rows_of(ref, start, size):
        return ref.at[start:start + size, :]

    raw_rows = dm * n_heads // _QKV_DMA_CHUNKS
    transfers = [("x_head", cols(xt_hbm, 0, xc), cols(xt_ref, 0, xc))]
    for name, src, dst in (("wq", wq_hbm, rq_ref), ("wk", wk_hbm, rk_ref), ("wv", wv_hbm, rv_ref)):
        for c in range(_QKV_DMA_CHUNKS):
            transfers.append(((name, c), rows_of(src, c * raw_rows, raw_rows),
                              rows_of(dst, c * raw_rows, raw_rows)))
    transfers.append(("wo", wot_hbm, wot_ref))
    for c in range(0, ffn, wc):
        transfers.append((("w1", c), cols(w1_hbm, c, wc), cols(r1_ref, c, wc)))
        transfers.append((("w3", c), cols(w3_hbm, c, wc), cols(r3_ref, c, wc)))
    transfers.append(("x_tail", cols(xt_hbm, xc, seq - xc), cols(xt_ref, xc, seq - xc)))
    for c in range(0, ffn, wc):
        transfers.append((("w2", c), cols(w2t_hbm, c, wc), cols(w2t_ref, c, wc)))
    copies = {name: pltpu.make_async_copy(src, dst, in_sems.at[n])
              for n, (name, src, dst) in enumerate(transfers)}

    def arrive(name):
        copies[name].wait()

    def project(h, grp):
        rows = slice(grp * dm, grp * dm + full)
        both = _paired_dot(h, wqkv_ref[rows, 0:3 * dh], wqkv_ref[rows, 3 * dh:],
                           sqkv_ref[grp * _LANES:(grp + 1) * _LANES, :])
        return [[qkv[:, m * dh:(m + 1) * dh].astype(_BF16) for m in range(3)] for qkv in both]

    def probabilities(qkv, visible, fill):
        probs = []
        for q, k, _ in qkv:
            s = jnp.where(visible, _dot_nt(q, k) * scale, fill)
            p = jnp.exp(s - jnp.max(s, axis=-1, keepdims=True))
            probs.append((p * (1.0 / jnp.sum(p, axis=-1, keepdims=True))).astype(_BF16))
        return probs

    def heads(h, n_streams, fillers=()):
        rows = h.shape[0]
        visible, fill = _mask_tables(n_streams, n_mem, seg)
        qkv, probs = {}, {}
        for t in range(n_grp + _PV_LAG):
            if t < n_grp:
                qkv[t] = project(h, t)
            elif t - n_grp < len(fillers):
                fillers[t - n_grp]()
            if 0 <= t - _QK_LAG < n_grp:
                probs[t - _QK_LAG] = probabilities(qkv[t - _QK_LAG], visible, fill)
            if 0 <= t - _PV_LAG:
                grp = t - _PV_LAG
                outs = [_dot(p, v) for p, (_, _, v) in zip(probs.pop(grp), qkv.pop(grp))]
                for part, out in enumerate(outs + [outs[0] + outs[1]]):
                    col = (part * n_grp + grp) * dh
                    o_ref[0:rows, col:col + dh] = out.astype(_BF16)

    def attend(h, n_streams):
        rows, half, wide = slice(0, h.shape[0]), n_grp * dh, []
        cut_u, cut_v = (n_grp - _PV_LAG) * dh, half + (n_grp - _PV_LAG + 1) * dh

        def part(lo, hi):
            return lambda: wide.append(_output_wide(o_ref, rows, wo_ref, lo, hi))

        heads(h, n_streams, (part(0, cut_u), part(half, cut_v)))
        part(cut_u, half)()
        part(cut_v, 2 * half)()
        wide = (wide[0] + wide[1]) + (wide[2] + wide[3])
        return _output_finish(o_ref, rows, wo_ref, so_ref, wide)

    def pair_gate_up(lo, hi):
        for raw, w_ref, s_ref in ((r1_ref, w1_ref, s1_ref), (r3_ref, w3_ref, s3_ref)):
            w_ref[0:_HALF, lo:hi] = raw[0:_HALF, lo:hi]
            w_ref[_LANES:, lo:hi] = raw[_LANES:full, lo:hi]
            for c in range(lo, hi, fc):
                ca, cb = slice(c, c + fc // 2), slice(c + fc // 2, c + fc)
                w_ref[mid, ca], w_ref[mid, cb], s_ref[:, c // 2:(c + fc) // 2] = _pair_weights(
                    raw[mid, ca], raw[full:, ca], raw[mid, cb], raw[full:, cb])

    def gate_up(f_in, lo=0, hi=ffn):
        for c in range(lo, hi, fc):
            ca, cb = slice(c, c + fc // 2), slice(c + fc // 2, c + fc)
            cs = slice(c // 2, (c + fc) // 2)
            gates = _paired_dot(f_in, w1_ref[0:full, ca], w1_ref[0:full, cb], s1_ref[:, cs])
            ups = _paired_dot(f_in, w3_ref[0:full, ca], w3_ref[0:full, cb], s3_ref[:, cs])
            hids = [gate * jax.nn.sigmoid(gate) * up for gate, up in zip(gates, ups)]
            for part, hid in enumerate(hids + [hids[0] + hids[1]]):
                col = (part * ffn + c) // 2
                hid_ref[0:hid.shape[0], col:col + fc // 2] = hid.astype(_BF16)

    def stage_down(lo, hi):
        for c in range(lo, hi, fc):
            rows_u = slice(c // 2, (c + fc) // 2)
            rows_v = slice((ffn + c) // 2, (ffn + c + fc) // 2)
            w2_ref[rows_u, :], w2_ref[rows_v, :], s2_ref[rows_u, :] = _pair_output_weights(
                w2t_ref[:, c:c + fc // 2], w2t_ref[:, c + fc // 2:c + fc])

    def single_stream_rows(mem, x):
        return _split_lhs(jnp.concatenate([mem, _layernorm(x)], axis=0))

    def write_back(t, size):
        xt_ref[:, t:t + size] = y_ref[t:t + size, :].T
        copy = pltpu.make_async_copy(
            cols(xt_ref, t, size), cols(out_hbm, t, size), out_sems.at[pl.cdiv(t, xc)])
        copy.start()
        return copy

    for copy in copies.values():
        copy.start()
    arrive("x_head")
    x_ref[0:xc, :] = xt_ref[:, 0:xc].T

    pairs = n_heads // 2
    d_chunk = dm // _QKV_DMA_CHUNKS
    for m, (name, raw_ref) in enumerate((("wq", rq_ref), ("wk", rk_ref), ("wv", rv_ref))):
        words = raw_ref.bitcast(jnp.uint32)
        for c in range(_QKV_DMA_CHUNKS):
            arrive((name, c))

            def regroup(quad, carry, m=m, c=c, words=words):
                start = pl.multiple_of(c * d_chunk * pairs + quad * _WORD_TILE, _WORD_TILE)
                view = words.at[pl.ds(start, d_chunk * pairs - pairs + _WORD_TILE), :]
                for r in range(_WORD_TILE):
                    even_d = view[pl.ds(r, d_chunk // 2, stride=n_heads), :]
                    odd_d = view[pl.ds(r + pairs, d_chunk // 2, stride=n_heads), :]
                    lo = (even_d & jnp.uint32(0xFFFF)) | (odd_d << 16)
                    hi = (even_d >> 16) | (odd_d & jnp.uint32(0xFFFF0000))
                    row = (quad * _WORD_TILE + r) * (dm // 2) + c * (d_chunk // 2)
                    for half, val in enumerate((lo, hi)):
                        col = (half * 3 + m) * dh
                        wqkv_ref.ref[pl.ds(pl.multiple_of(row, 8), d_chunk // 2), col:col + dh] = val
                return carry

            jax.lax.fori_loop(0, pairs // _WORD_TILE, regroup, 0)

    def pair_heads(grp, carry):
        ca, cb = slice(0, 3 * dh), slice(3 * dh, 6 * dh)
        mid_rows, tail_rows = (grp * dm + _HALF, _HALF), (grp * dm + full, _HALF)
        (wqkv_ref[mid_rows, ca], wqkv_ref[mid_rows, cb],
         sqkv_ref[(grp * _LANES, _LANES), :]) = _pair_weights(
             wqkv_ref[mid_rows, ca], wqkv_ref[tail_rows, ca],
             wqkv_ref[mid_rows, cb], wqkv_ref[tail_rows, cb])
        return carry

    jax.lax.fori_loop(0, n_grp, pair_heads, 0)

    mem0 = mem0_ref[...].astype(_F32)
    a_ref[0:n_mem, :] = mem0

    def first_segments(s, carry):
        x_s = x_ref[pl.ds(pl.multiple_of(s * seg, seg), seg), :].astype(_F32)
        heads(single_stream_rows(a_ref[0:n_mem, :], x_s), 1)

        @pl.when(s == 0)
        def _():
            arrive("wo")

            def stage_wo(grp, carry):
                rows_u, rows_v = (grp * dh, dh), ((n_grp + grp) * dh, dh)
                wo_ref[rows_u, :], wo_ref[rows_v, :], so_ref[rows_u, :] = _pair_output_weights(
                    wot_ref[2 * grp], wot_ref[2 * grp + 1])
                return carry

            jax.lax.fori_loop(0, n_grp, stage_wo, 0, unroll=2)

        a = _output_dot(o_ref, slice(0, n_mem + seg), wo_ref, so_ref)
        a_ref[0:n_mem, :] = a[:n_mem]
        a_ref[pl.ds(pl.multiple_of(tok0 + (1 - s) * seg, n_mem), seg), :] = a[n_mem:]
        return carry

    jax.lax.fori_loop(0, 2, first_segments, 0)
    zeros = jnp.zeros((seg, dm), _F32)
    x1_s0 = x_ref[0:seg, :].astype(_F32) + a_ref[tok0 + seg:, :]
    a_ref[n_mem:tok0, :] = mem0
    a_ref[tok0 + seg:, :] = zeros
    xa_ref[...] = jnp.concatenate([x_ref[seg:2 * seg, :].astype(_F32), zeros], axis=0)
    x1_ref[...] = jnp.concatenate([x1_s0, zeros], axis=0)
    hid_ref[seg:, :] = jnp.zeros((seg, hid_ref.shape[1]), _BF16)
    f_in = _split_lhs(_layernorm(x1_s0))
    for c in range(0, ffn, wc):
        arrive(("w1", c))
        arrive(("w3", c))
        pair_gate_up(c, c + wc)
        gate_up(f_in, c, c + wc)
    arrive("x_tail")
    for t in range(xc, seq, xc):
        x_ref[t:t + xc, :] = xt_ref[:, t:t + xc].T
    for c in range(0, ffn, wc):
        arrive(("w2", c))
        stage_down(c, c + wc)
    wide_ref[0:seg, :] = _output_wide(hid_ref, slice(0, seg), w2_ref)
    wide_ref[seg:, :] = jnp.zeros((seg, wide_ref.shape[1]), _F32)

    both = slice(0, 2 * seg)

    def feed_forward(out_row):
        y = x1_ref[...] + _output_finish(hid_ref, both, w2_ref, s2_ref, wide_ref[...])
        y_ref[pl.ds(out_row, seg), :] = y[seg:].astype(y_ref.dtype)
        x1 = xa_ref[...] + a_ref[tok0:, :]
        x1_ref[...] = x1
        gate_up(_split_lhs(_layernorm(x1)))
        return y[:seg]

    def step(i, carry):
        x2 = feed_forward(pl.multiple_of(jnp.maximum(i - 3, 0) * seg, seg))
        nxt_row = pl.multiple_of((i + 1) * seg, seg)
        xa = jnp.concatenate([x_ref[pl.ds(nxt_row, seg), :].astype(_F32), x2], axis=0)
        xa_ref[...] = xa
        wide_ref[...] = _output_wide(hid_ref, both, w2_ref)
        a_ref[...] = attend(
            _split_lhs(jnp.concatenate([a_ref[0:tok0, :], _layernorm(xa)], axis=0)), 2)
        return carry

    jax.lax.fori_loop(1, n_seg - 1, step, 0)

    x_s0 = feed_forward(seq - 4 * seg)
    a = attend(single_stream_rows(a_ref[n_mem:tok0, :], x_s0), 1)
    y = x1_ref[...] + _output_dot(hid_ref, both, w2_ref, s2_ref)
    y_ref[seq - 3 * seg:seq - 2 * seg, :] = y[seg:].astype(y_ref.dtype)
    x1_s0 = x_s0 + a[n_mem:]
    last = seq - _LANES
    writes = [write_back(t, min(xc, last - t)) for t in range(0, last, xc)]
    a = attend(single_stream_rows(a[:n_mem], y[:seg]), 1)
    x1 = jnp.concatenate([x1_s0, y[:seg] + a[n_mem:]], axis=0)
    gate_up(_split_lhs(_layernorm(x1)))
    y_ref[seq - 2 * seg:, :] = (x1 + _output_dot(hid_ref, both, w2_ref, s2_ref)).astype(y_ref.dtype)
    writes.append(write_back(last, _LANES))
    for copy in writes:
        copy.wait()


@functools.partial(jax.jit, static_argnames=("A_seg_len",))
def pallas_interleave_layers__memory_aug_recurrent_mem_tr__glu_gated_swiglu__prompt_kernel(
    A_x: jax.Array,
    A_mem0: jax.Array,
    A_Wq: jax.Array,
    A_Wk: jax.Array,
    A_Wv: jax.Array,
    A_Wo: jax.Array,
    A_seg_len: int,
    B_x: jax.Array,
    B_w1: jax.Array,
    B_w3: jax.Array,
    B_w2: jax.Array,
):
    del B_x
    batch, seq, dm = A_x.shape
    _, n_heads, dh = A_Wq.shape
    n_mem = A_mem0.shape[1]
    ffn = B_w1.shape[1]
    seg = int(A_seg_len)
    assert batch == 1 and seq % _XPOSE_CHUNK == 0 and _XPOSE_CHUNK % seg == 0 and _XPOSE_CHUNK >= 3 * seg
    rows = 2 * (n_mem + seg)
    full = dm - _HALF

    vmem = pl.BlockSpec(memory_space=pltpu.VMEM)
    hbm = pl.BlockSpec(memory_space=pltpu.HBM)
    out_t = pl.pallas_call(
        functools.partial(_kernel, seg=seg, n_heads=n_heads, dh=dh),
        out_shape=jax.ShapeDtypeStruct((dm, seq), A_x.dtype),
        in_specs=[hbm, vmem] + [hbm] * 7,
        out_specs=hbm,
        scratch_shapes=[
            pltpu.VMEM((dm, seq), _BF16),
            pltpu.VMEM((seq, dm), _BF16),
            pltpu.VMEM((dm * n_heads, dh), _BF16),
            pltpu.VMEM((dm * n_heads, dh), _BF16),
            pltpu.VMEM((dm * n_heads, dh), _BF16),
            _packed_scratch(n_heads // 2 * dm, 6 * dh),
            pltpu.VMEM((n_heads, dm, dh), _BF16),
            _packed_scratch(n_heads * dh, full),
            pltpu.VMEM((dm, ffn), _BF16),
            pltpu.VMEM((dm, ffn), _BF16),
            _packed_scratch(full, ffn),
            _packed_scratch(full, ffn),
            pltpu.VMEM((dm, ffn), _BF16),
            _packed_scratch(ffn, full),
            _packed_scratch(n_heads // 2 * _LANES, 3 * dh),
            _packed_scratch(_LANES, ffn // 2),
            _packed_scratch(_LANES, ffn // 2),
            _packed_scratch(n_heads * dh // 2, _LANES),
            _packed_scratch(ffn // 2, _LANES),
            _packed_scratch(rows, n_heads * dh * 3 // 2),
            _packed_scratch(2 * seg, ffn * 3 // 2),
            pltpu.VMEM((rows, dm), _F32),
            pltpu.VMEM((2 * seg, dm), _F32),
            pltpu.VMEM((2 * seg, dm), _F32),
            pltpu.VMEM((2 * seg, dm - _HALF - _LANES), _F32),
            pltpu.VMEM((seq, dm), _BF16),
            pltpu.SemaphoreType.DMA((3 + 3 * _QKV_DMA_CHUNKS + 3 * _FFN_DMA_CHUNKS,)),
            pltpu.SemaphoreType.DMA((seq // _XPOSE_CHUNK + 1,)),
        ],
        compiler_params=pltpu.CompilerParams(vmem_limit_bytes=110 * 1024 * 1024),
    )(
        A_x.reshape(seq, dm).T,
        A_mem0.reshape(n_mem, dm),
        A_Wq.reshape(dm * n_heads, dh),
        A_Wk.reshape(dm * n_heads, dh),
        A_Wv.reshape(dm * n_heads, dh),
        A_Wo.transpose(0, 2, 1),
        B_w1,
        B_w3,
        B_w2.T,
    )
    return out_t.T.reshape(batch, seq, dm)
```

```python
import functools

import jax
import jax.numpy as jnp
import numpy as np
import jax.experimental.pallas as pl
import jax.experimental.pallas.tpu as pltpu

_EPS = 1e-5
_MASK_FILL = -1000000000.0
_QK_LAG = 1
_PV_LAG = 4
_FFN_CHUNK = 512
_XPOSE_CHUNK = 256
_FFN_DMA_CHUNKS = 3
_QKV_DMA_CHUNKS = 2
_WORD_TILE = 4

_LANES = 128
_HALF = _LANES // 2
_F32 = jnp.float32
_BF16 = jnp.bfloat16


def _layernorm(x):
    mean = jnp.mean(x, axis=-1, keepdims=True)
    cen = x - mean
    var = jnp.mean(cen * cen, axis=-1, keepdims=True)
    return cen * jax.lax.rsqrt(var + _EPS)


def _dot(a, b):
    return jnp.dot(a, b, preferred_element_type=_F32)


def _dot_nt(a, b):
    return jax.lax.dot_general(a, b, (((1,), (1,)), ((), ())), preferred_element_type=_F32)


class _Packed:
    def __init__(self, ref):
        self.ref = ref
        self.shape = (2 * ref.shape[0], ref.shape[1])

    def _index(self, idx):
        rows, cols = idx
        if isinstance(rows, slice):
            lo, hi, _ = rows.indices(self.shape[0])
            return slice(lo // 2, hi // 2), cols
        start, size = rows
        return pl.ds(pl.multiple_of(start // 2, size // 2), size // 2), cols

    def __getitem__(self, idx):
        return pltpu.bitcast(self.ref[self._index(idx)], _BF16)

    def __setitem__(self, idx, value):
        self.ref[self._index(idx)] = pltpu.bitcast(value, jnp.uint32)


def _packed_scratch(rows, cols):
    return pltpu.VMEM((rows // 2, cols), jnp.uint32)


def _split_lhs(x):
    full = x.shape[1] - _HALF
    first, rest = x[:, :_LANES], x[:, _LANES:full]
    tail = x[:, full:]
    lhs_b0 = jnp.concatenate([first[:, :_HALF], tail], axis=1)
    lhs_s = jnp.concatenate([tail, first[:, _HALF:]], axis=1)
    return jnp.concatenate([first, rest, lhs_b0, lhs_s], axis=1).astype(_BF16)


def _paired_dot(lhs, w_a, w_b, w_s):
    full = w_a.shape[0]
    shared = _dot(lhs[:, full + _LANES:], w_s)
    lhs_b = jnp.concatenate([lhs[:, full:full + _LANES], lhs[:, _LANES:full]], axis=1)
    return _dot(lhs[:, :full], w_a) + shared, _dot(lhs_b, w_b) + shared


def _pair_weights(a_mid, a_tail, b_mid, b_tail):
    a_new = (a_mid.astype(_F32) - b_mid.astype(_F32)).astype(_BF16)
    b_new = (b_tail.astype(_F32) - a_tail.astype(_F32)).astype(_BF16)
    return a_new, b_new, jnp.concatenate([a_tail, b_mid], axis=0)


def _pair_output_weights(ut, vt):
    full = ut.shape[0] - _HALF
    mid = slice(_HALF, _LANES)
    u_new, v_new, shared = _pair_weights(ut[mid], ut[full:], vt[mid], vt[full:])
    u = jnp.concatenate([ut[:_HALF], u_new, ut[_LANES:full]], axis=0)
    v = jnp.concatenate([vt[:_HALF], v_new, vt[_LANES:full]], axis=0)
    return u.T, v.T, shared.T


def _output_wide(lhs_ref, rows, w_ref, lo=0, hi=None):
    hi = w_ref.shape[0] if hi is None else hi
    return _dot(lhs_ref[rows, lo:hi], w_ref[lo:hi, _LANES:])


def _output_finish(lhs_ref, rows, w_ref, s_ref, wide):
    half = s_ref.shape[0]
    u0 = _dot(lhs_ref[rows, 0:half], w_ref[0:half, 0:_LANES])
    v0 = _dot(lhs_ref[rows, half:2 * half], w_ref[half:, 0:_LANES])
    shared = _dot(lhs_ref[rows, 2 * half:], s_ref[:, :])
    is_low = jax.lax.broadcasted_iota(jnp.int32, u0.shape, 1) < _HALF
    first = u0 + jnp.where(is_low, v0, shared)
    last = v0[:, _HALF:] + shared[:, :_HALF]
    return jnp.concatenate([first, wide, last], axis=1)


def _output_dot(lhs_ref, rows, w_ref, s_ref):
    return _output_finish(lhs_ref, rows, w_ref, s_ref, _output_wide(lhs_ref, rows, w_ref))


def _mask_tables(n_streams, n_mem, seg):
    tok0 = n_streams * n_mem
    rows = tok0 + n_streams * seg

    def split(axis):
        idx = jax.lax.broadcasted_iota(jnp.int32, (rows, rows), axis)
        is_mem = idx < tok0
        stream = jnp.where(is_mem, idx // n_mem, (idx - tok0) // seg)
        pos = jnp.where(is_mem, idx % n_mem, n_mem + (idx - tok0) % seg)
        return stream, pos

    q_stream, q_pos = split(0)
    k_stream, k_pos = split(1)
    same = q_stream == k_stream
    visible = same & ((q_pos < n_mem) | (q_pos >= k_pos))
    fill = jnp.where(same, _MASK_FILL, -jnp.inf).astype(_F32)
    return visible, fill


def _kernel(xt_hbm, mem0_ref, wq_hbm, wk_hbm, wv_hbm, wot_hbm, w1_hbm, w3_hbm, w2t_hbm,
            out_hbm,
            xt_ref, x_ref, rq_ref, rk_ref, rv_ref, wqkv_ref, wot_ref, wo_ref,
            r1_ref, r3_ref, w1_ref, w3_ref, w2t_ref, w2_ref, sqkv_ref, s1_ref, s3_ref, so_ref, s2_ref,
            o_ref, hid_ref, a_ref, xa_ref, x1_ref, wide_ref, y_ref, in_sems, out_sems,
            *, seg, n_heads, dh):
    seq, dm = x_ref.shape
    n_mem = mem0_ref.shape[0]
    n_seg = seq // seg
    ffn = w1_ref.shape[1]
    wqkv_ref, wo_ref, w1_ref, w3_ref, w2_ref = map(
        _Packed, (wqkv_ref, wo_ref, w1_ref, w3_ref, w2_ref))
    sqkv_ref, s1_ref, s3_ref, so_ref, s2_ref = map(
        _Packed, (sqkv_ref, s1_ref, s3_ref, so_ref, s2_ref))
    o_ref, hid_ref = _Packed(o_ref), _Packed(hid_ref)
    scale = dh ** -0.5
    n_grp = n_heads // 2
    tok0 = 2 * n_mem
    full = dm - _HALF
    mid = slice(_HALF, _LANES)
    fc = _FFN_CHUNK
    xc = _XPOSE_CHUNK
    wc = ffn // _FFN_DMA_CHUNKS

    def cols(ref, start, size):
        return ref.at[:, start:start + size]

    def rows_of(ref, start, size):
        return ref.at[start:start + size, :]

    raw_rows = dm * n_heads // _QKV_DMA_CHUNKS
    transfers = [("x_head", cols(xt_hbm, 0, xc), cols(xt_ref, 0, xc))]
    for name, src, dst in (("wq", wq_hbm, rq_ref), ("wk", wk_hbm, rk_ref), ("wv", wv_hbm, rv_ref)):
        for c in range(_QKV_DMA_CHUNKS):
            transfers.append(((name, c), rows_of(src, c * raw_rows, raw_rows),
                              rows_of(dst, c * raw_rows, raw_rows)))
    transfers.append(("wo", wot_hbm, wot_ref))
    for c in range(0, ffn, wc):
        transfers.append((("w1", c), cols(w1_hbm, c, wc), cols(r1_ref, c, wc)))
        transfers.append((("w3", c), cols(w3_hbm, c, wc), cols(r3_ref, c, wc)))
    for c in range(0, ffn, wc):
        transfers.append((("w2", c), cols(w2t_hbm, c, wc), cols(w2t_ref, c, wc)))
    transfers.append(("x_tail", cols(xt_hbm, xc, seq - xc), cols(xt_ref, xc, seq - xc)))
    copies = {name: pltpu.make_async_copy(src, dst, in_sems.at[n])
              for n, (name, src, dst) in enumerate(transfers)}

    def arrive(name):
        copies[name].wait()

    def project(h, grp):
        rows = slice(grp * dm, grp * dm + full)
        both = _paired_dot(h, wqkv_ref[rows, 0:3 * dh], wqkv_ref[rows, 3 * dh:],
                           sqkv_ref[grp * _LANES:(grp + 1) * _LANES, :])
        return [[qkv[:, m * dh:(m + 1) * dh].astype(_BF16) for m in range(3)] for qkv in both]

    def probabilities(qkv, visible, fill):
        probs = []
        for q, k, _ in qkv:
            s = jnp.where(visible, _dot_nt(q, k) * scale, fill)
            p = jnp.exp(s - jnp.max(s, axis=-1, keepdims=True))
            probs.append((p * (1.0 / jnp.sum(p, axis=-1, keepdims=True))).astype(_BF16))
        return probs

    def heads(h, n_streams, fillers=()):
        rows = h.shape[0]
        visible, fill = _mask_tables(n_streams, n_mem, seg)
        qkv, probs = {}, {}
        for t in range(n_grp + _PV_LAG):
            if t < n_grp:
                qkv[t] = project(h, t)
            elif t - n_grp < len(fillers):
                fillers[t - n_grp]()
            if 0 <= t - _QK_LAG < n_grp:
                probs[t - _QK_LAG] = probabilities(qkv[t - _QK_LAG], visible, fill)
            if 0 <= t - _PV_LAG:
                grp = t - _PV_LAG
                outs = [_dot(p, v) for p, (_, _, v) in zip(probs.pop(grp), qkv.pop(grp))]
                for part, out in enumerate(outs + [outs[0] + outs[1]]):
                    col = (part * n_grp + grp) * dh
                    o_ref[0:rows, col:col + dh] = out.astype(_BF16)

    def attend(h, n_streams):
        rows, half, wide = slice(0, h.shape[0]), n_grp * dh, []
        cut_u, cut_v = (n_grp - _PV_LAG) * dh, half + (n_grp - _PV_LAG + 1) * dh

        def part(lo, hi):
            return lambda: wide.append(_output_wide(o_ref, rows, wo_ref, lo, hi))

        heads(h, n_streams, (part(0, cut_u), part(half, cut_v)))
        part(cut_u, half)()
        part(cut_v, 2 * half)()
        wide = (wide[0] + wide[1]) + (wide[2] + wide[3])
        return _output_finish(o_ref, rows, wo_ref, so_ref, wide)

    def pair_gate_up(lo, hi):
        for raw, w_ref, s_ref in ((r1_ref, w1_ref, s1_ref), (r3_ref, w3_ref, s3_ref)):
            w_ref[0:_HALF, lo:hi] = raw[0:_HALF, lo:hi]
            w_ref[_LANES:, lo:hi] = raw[_LANES:full, lo:hi]
            for c in range(lo, hi, fc):
                ca, cb = slice(c, c + fc // 2), slice(c + fc // 2, c + fc)
                w_ref[mid, ca], w_ref[mid, cb], s_ref[:, c // 2:(c + fc) // 2] = _pair_weights(
                    raw[mid, ca], raw[full:, ca], raw[mid, cb], raw[full:, cb])

    def gate_up(f_in, lo=0, hi=ffn):
        for c in range(lo, hi, fc):
            ca, cb = slice(c, c + fc // 2), slice(c + fc // 2, c + fc)
            cs = slice(c // 2, (c + fc) // 2)
            gates = _paired_dot(f_in, w1_ref[0:full, ca], w1_ref[0:full, cb], s1_ref[:, cs])
            ups = _paired_dot(f_in, w3_ref[0:full, ca], w3_ref[0:full, cb], s3_ref[:, cs])
            hids = [gate * jax.nn.sigmoid(gate) * up for gate, up in zip(gates, ups)]
            for part, hid in enumerate(hids + [hids[0] + hids[1]]):
                col = (part * ffn + c) // 2
                hid_ref[0:hid.shape[0], col:col + fc // 2] = hid.astype(_BF16)

    def stage_down(lo, hi):
        for c in range(lo, hi, fc):
            rows_u = slice(c // 2, (c + fc) // 2)
            rows_v = slice((ffn + c) // 2, (ffn + c + fc) // 2)
            w2_ref[rows_u, :], w2_ref[rows_v, :], s2_ref[rows_u, :] = _pair_output_weights(
                w2t_ref[:, c:c + fc // 2], w2t_ref[:, c + fc // 2:c + fc])

    def single_stream_rows(mem, x):
        return _split_lhs(jnp.concatenate([mem, _layernorm(x)], axis=0))

    def write_back(t, size):
        xt_ref[:, t:t + size] = y_ref[t:t + size, :].T
        copy = pltpu.make_async_copy(
            cols(xt_ref, t, size), cols(out_hbm, t, size), out_sems.at[pl.cdiv(t, xc)])
        copy.start()
        return copy

    for copy in copies.values():
        copy.start()
    arrive("x_head")
    x_ref[0:xc, :] = xt_ref[:, 0:xc].T

    pairs = n_heads // 2
    d_chunk = dm // _QKV_DMA_CHUNKS
    for m, (name, raw_ref) in enumerate((("wq", rq_ref), ("wk", rk_ref), ("wv", rv_ref))):
        words = raw_ref.bitcast(jnp.uint32)
        for c in range(_QKV_DMA_CHUNKS):
            arrive((name, c))

            def regroup(quad, carry, m=m, c=c, words=words):
                start = pl.multiple_of(c * d_chunk * pairs + quad * _WORD_TILE, _WORD_TILE)
                view = words.at[pl.ds(start, d_chunk * pairs - pairs + _WORD_TILE), :]
                for r in range(_WORD_TILE):
                    even_d = view[pl.ds(r, d_chunk // 2, stride=n_heads), :]
                    odd_d = view[pl.ds(r + pairs, d_chunk // 2, stride=n_heads), :]
                    lo = (even_d & jnp.uint32(0xFFFF)) | (odd_d << 16)
                    hi = (even_d >> 16) | (odd_d & jnp.uint32(0xFFFF0000))
                    row = (quad * _WORD_TILE + r) * (dm // 2) + c * (d_chunk // 2)
                    for half, val in enumerate((lo, hi)):
                        col = (half * 3 + m) * dh
                        wqkv_ref.ref[pl.ds(pl.multiple_of(row, 8), d_chunk // 2), col:col + dh] = val
                return carry

            jax.lax.fori_loop(0, pairs // _WORD_TILE, regroup, 0)

    def pair_heads(grp, carry):
        ca, cb = slice(0, 3 * dh), slice(3 * dh, 6 * dh)
        mid_rows, tail_rows = (grp * dm + _HALF, _HALF), (grp * dm + full, _HALF)
        (wqkv_ref[mid_rows, ca], wqkv_ref[mid_rows, cb],
         sqkv_ref[(grp * _LANES, _LANES), :]) = _pair_weights(
             wqkv_ref[mid_rows, ca], wqkv_ref[tail_rows, ca],
             wqkv_ref[mid_rows, cb], wqkv_ref[tail_rows, cb])
        return carry

    jax.lax.fori_loop(0, n_grp, pair_heads, 0)

    mem0 = mem0_ref[...].astype(_F32)
    a_ref[0:n_mem, :] = mem0

    def first_segments(s, carry):
        x_s = x_ref[pl.ds(pl.multiple_of(s * seg, seg), seg), :].astype(_F32)
        heads(single_stream_rows(a_ref[0:n_mem, :], x_s), 1)

        @pl.when(s == 0)
        def _():
            arrive("wo")

            def stage_wo(grp, carry):
                rows_u, rows_v = (grp * dh, dh), ((n_grp + grp) * dh, dh)
                wo_ref[rows_u, :], wo_ref[rows_v, :], so_ref[rows_u, :] = _pair_output_weights(
                    wot_ref[2 * grp], wot_ref[2 * grp + 1])
                return carry

            jax.lax.fori_loop(0, n_grp, stage_wo, 0, unroll=2)

        a = _output_dot(o_ref, slice(0, n_mem + seg), wo_ref, so_ref)
        a_ref[0:n_mem, :] = a[:n_mem]
        a_ref[pl.ds(pl.multiple_of(tok0 + (1 - s) * seg, n_mem), seg), :] = a[n_mem:]
        return carry

    jax.lax.fori_loop(0, 2, first_segments, 0)
    zeros = jnp.zeros((seg, dm), _F32)
    x1_s0 = x_ref[0:seg, :].astype(_F32) + a_ref[tok0 + seg:, :]
    a_ref[n_mem:tok0, :] = mem0
    a_ref[tok0 + seg:, :] = zeros
    xa_ref[...] = jnp.concatenate([x_ref[seg:2 * seg, :].astype(_F32), zeros], axis=0)
    x1_ref[...] = jnp.concatenate([x1_s0, zeros], axis=0)
    hid_ref[seg:, :] = jnp.zeros((seg, hid_ref.shape[1]), _BF16)
    f_in = _split_lhs(_layernorm(x1_s0))
    for c in range(0, ffn, wc):
        arrive(("w1", c))
        arrive(("w3", c))
        pair_gate_up(c, c + wc)
        gate_up(f_in, c, c + wc)
    for c in range(0, ffn, wc):
        arrive(("w2", c))
        stage_down(c, c + wc)
    wide_ref[0:seg, :] = _output_wide(hid_ref, slice(0, seg), w2_ref)
    wide_ref[seg:, :] = jnp.zeros((seg, wide_ref.shape[1]), _F32)

    both = slice(0, 2 * seg)

    def feed_forward(out_row):
        y = x1_ref[...] + _output_finish(hid_ref, both, w2_ref, s2_ref, wide_ref[...])
        y_ref[pl.ds(out_row, seg), :] = y[seg:].astype(y_ref.dtype)
        x1 = xa_ref[...] + a_ref[tok0:, :]
        x1_ref[...] = x1
        gate_up(_split_lhs(_layernorm(x1)))
        return y[:seg]

    def step(i, carry):
        @pl.when(i == xc // seg - 1)
        def _():
            arrive("x_tail")
            for t in range(xc, seq, xc):
                x_ref[t:t + xc, :] = xt_ref[:, t:t + xc].T

        x2 = feed_forward(pl.multiple_of(jnp.maximum(i - 3, 0) * seg, seg))
        nxt_row = pl.multiple_of((i + 1) * seg, seg)
        xa = jnp.concatenate([x_ref[pl.ds(nxt_row, seg), :].astype(_F32), x2], axis=0)
        xa_ref[...] = xa
        wide_ref[...] = _output_wide(hid_ref, both, w2_ref)
        a_ref[...] = attend(
            _split_lhs(jnp.concatenate([a_ref[0:tok0, :], _layernorm(xa)], axis=0)), 2)
        return carry

    jax.lax.fori_loop(1, n_seg - 1, step, 0)

    x_s0 = feed_forward(seq - 4 * seg)
    a = attend(single_stream_rows(a_ref[n_mem:tok0, :], x_s0), 1)
    y = x1_ref[...] + _output_dot(hid_ref, both, w2_ref, s2_ref)
    y_ref[seq - 3 * seg:seq - 2 * seg, :] = y[seg:].astype(y_ref.dtype)
    x1_s0 = x_s0 + a[n_mem:]
    last = seq - _LANES
    writes = [write_back(t, min(xc, last - t)) for t in range(0, last, xc)]
    a = attend(single_stream_rows(a[:n_mem], y[:seg]), 1)
    x1 = jnp.concatenate([x1_s0, y[:seg] + a[n_mem:]], axis=0)
    gate_up(_split_lhs(_layernorm(x1)))
    y_ref[seq - 2 * seg:, :] = (x1 + _output_dot(hid_ref, both, w2_ref, s2_ref)).astype(y_ref.dtype)
    writes.append(write_back(last, _LANES))
    for copy in writes:
        copy.wait()


@functools.partial(jax.jit, static_argnames=("A_seg_len",))
def pallas_interleave_layers__memory_aug_recurrent_mem_tr__glu_gated_swiglu__prompt_kernel(
    A_x: jax.Array,
    A_mem0: jax.Array,
    A_Wq: jax.Array,
    A_Wk: jax.Array,
    A_Wv: jax.Array,
    A_Wo: jax.Array,
    A_seg_len: int,
    B_x: jax.Array,
    B_w1: jax.Array,
    B_w3: jax.Array,
    B_w2: jax.Array,
):
    del B_x
    batch, seq, dm = A_x.shape
    _, n_heads, dh = A_Wq.shape
    n_mem = A_mem0.shape[1]
    ffn = B_w1.shape[1]
    seg = int(A_seg_len)
    assert batch == 1 and seq % _XPOSE_CHUNK == 0 and _XPOSE_CHUNK % seg == 0 and _XPOSE_CHUNK >= 3 * seg
    rows = 2 * (n_mem + seg)
    full = dm - _HALF

    vmem = pl.BlockSpec(memory_space=pltpu.VMEM)
    hbm = pl.BlockSpec(memory_space=pltpu.HBM)
    out_t = pl.pallas_call(
        functools.partial(_kernel, seg=seg, n_heads=n_heads, dh=dh),
        out_shape=jax.ShapeDtypeStruct((dm, seq), A_x.dtype),
        in_specs=[hbm, vmem] + [hbm] * 7,
        out_specs=hbm,
        scratch_shapes=[
            pltpu.VMEM((dm, seq), _BF16),
            pltpu.VMEM((seq, dm), _BF16),
            pltpu.VMEM((dm * n_heads, dh), _BF16),
            pltpu.VMEM((dm * n_heads, dh), _BF16),
            pltpu.VMEM((dm * n_heads, dh), _BF16),
            _packed_scratch(n_heads // 2 * dm, 6 * dh),
            pltpu.VMEM((n_heads, dm, dh), _BF16),
            _packed_scratch(n_heads * dh, full),
            pltpu.VMEM((dm, ffn), _BF16),
            pltpu.VMEM((dm, ffn), _BF16),
            _packed_scratch(full, ffn),
            _packed_scratch(full, ffn),
            pltpu.VMEM((dm, ffn), _BF16),
            _packed_scratch(ffn, full),
            _packed_scratch(n_heads // 2 * _LANES, 3 * dh),
            _packed_scratch(_LANES, ffn // 2),
            _packed_scratch(_LANES, ffn // 2),
            _packed_scratch(n_heads * dh // 2, _LANES),
            _packed_scratch(ffn // 2, _LANES),
            _packed_scratch(rows, n_heads * dh * 3 // 2),
            _packed_scratch(2 * seg, ffn * 3 // 2),
            pltpu.VMEM((rows, dm), _F32),
            pltpu.VMEM((2 * seg, dm), _F32),
            pltpu.VMEM((2 * seg, dm), _F32),
            pltpu.VMEM((2 * seg, dm - _HALF - _LANES), _F32),
            pltpu.VMEM((seq, dm), _BF16),
            pltpu.SemaphoreType.DMA((3 + 3 * _QKV_DMA_CHUNKS + 3 * _FFN_DMA_CHUNKS,)),
            pltpu.SemaphoreType.DMA((seq // _XPOSE_CHUNK + 1,)),
        ],
        compiler_params=pltpu.CompilerParams(vmem_limit_bytes=110 * 1024 * 1024),
    )(
        A_x.reshape(seq, dm).T,
        A_mem0.reshape(n_mem, dm),
        A_Wq.reshape(dm * n_heads, dh),
        A_Wk.reshape(dm * n_heads, dh),
        A_Wv.reshape(dm * n_heads, dh),
        A_Wo.transpose(0, 2, 1),
        B_w1,
        B_w3,
        B_w2.T,
    )
    return out_t.T.reshape(batch, seq, dm)
```

```python
import functools

import jax
import jax.numpy as jnp
import numpy as np
import jax.experimental.pallas as pl
import jax.experimental.pallas.tpu as pltpu

_EPS = 1e-5
_MASK_FILL = -1000000000.0
_QK_LAG = 1
_PV_LAG = 4
_FFN_CHUNK = 512
_XPOSE_CHUNK = 256
_FFN_DMA_CHUNKS = 3
_QKV_DMA_CHUNKS = 2
_WORD_TILE = 4

_LANES = 128
_HALF = _LANES // 2
_F32 = jnp.float32
_BF16 = jnp.bfloat16


def _layernorm(x):
    mean = jnp.mean(x, axis=-1, keepdims=True)
    cen = x - mean
    var = jnp.mean(cen * cen, axis=-1, keepdims=True)
    return cen * jax.lax.rsqrt(var + _EPS)


def _dot(a, b):
    return jnp.dot(a, b, preferred_element_type=_F32)


def _dot_nt(a, b):
    return jax.lax.dot_general(a, b, (((1,), (1,)), ((), ())), preferred_element_type=_F32)


class _Packed:
    def __init__(self, ref):
        self.ref = ref
        self.shape = (2 * ref.shape[0], ref.shape[1])

    def _index(self, idx):
        rows, cols = idx
        if isinstance(rows, slice):
            lo, hi, _ = rows.indices(self.shape[0])
            return slice(lo // 2, hi // 2), cols
        start, size = rows
        return pl.ds(pl.multiple_of(start // 2, size // 2), size // 2), cols

    def __getitem__(self, idx):
        return pltpu.bitcast(self.ref[self._index(idx)], _BF16)

    def __setitem__(self, idx, value):
        self.ref[self._index(idx)] = pltpu.bitcast(value, jnp.uint32)


def _packed_scratch(rows, cols):
    return pltpu.VMEM((rows // 2, cols), jnp.uint32)


def _split_lhs(x):
    full = x.shape[1] - _HALF
    first, rest = x[:, :_LANES], x[:, _LANES:full]
    tail = x[:, full:]
    lhs_b0 = jnp.concatenate([first[:, :_HALF], tail], axis=1)
    lhs_s = jnp.concatenate([tail, first[:, _HALF:]], axis=1)
    return jnp.concatenate([first, rest, lhs_b0, lhs_s], axis=1).astype(_BF16)


def _paired_dot(lhs, w_a, w_b, w_s):
    full = w_a.shape[0]
    shared = _dot(lhs[:, full + _LANES:], w_s)
    lhs_b = jnp.concatenate([lhs[:, full:full + _LANES], lhs[:, _LANES:full]], axis=1)
    return _dot(lhs[:, :full], w_a) + shared, _dot(lhs_b, w_b) + shared


def _pair_weights(a_mid, a_tail, b_mid, b_tail):
    a_new = (a_mid.astype(_F32) - b_mid.astype(_F32)).astype(_BF16)
    b_new = (b_tail.astype(_F32) - a_tail.astype(_F32)).astype(_BF16)
    return a_new, b_new, jnp.concatenate([a_tail, b_mid], axis=0)


def _pair_output_weights(ut, vt):
    full = ut.shape[0] - _HALF
    mid = slice(_HALF, _LANES)
    u_new, v_new, shared = _pair_weights(ut[mid], ut[full:], vt[mid], vt[full:])
    u = jnp.concatenate([ut[:_HALF], u_new, ut[_LANES:full]], axis=0)
    v = jnp.concatenate([vt[:_HALF], v_new, vt[_LANES:full]], axis=0)
    return u.T, v.T, shared.T


def _output_wide(lhs_ref, rows, w_ref, lo=0, hi=None):
    hi = w_ref.shape[0] if hi is None else hi
    return _dot(lhs_ref[rows, lo:hi], w_ref[lo:hi, _LANES:])


def _output_finish(lhs_ref, rows, w_ref, s_ref, wide):
    half = s_ref.shape[0]
    u0 = _dot(lhs_ref[rows, 0:half], w_ref[0:half, 0:_LANES])
    v0 = _dot(lhs_ref[rows, half:2 * half], w_ref[half:, 0:_LANES])
    shared = _dot(lhs_ref[rows, 2 * half:], s_ref[:, :])
    is_low = jax.lax.broadcasted_iota(jnp.int32, u0.shape, 1) < _HALF
    first = u0 + jnp.where(is_low, v0, shared)
    last = v0[:, _HALF:] + shared[:, :_HALF]
    return jnp.concatenate([first, wide, last], axis=1)


def _output_dot(lhs_ref, rows, w_ref, s_ref):
    return _output_finish(lhs_ref, rows, w_ref, s_ref, _output_wide(lhs_ref, rows, w_ref))


def _mask_tables(n_streams, n_mem, seg):
    tok0 = n_streams * n_mem
    rows = tok0 + n_streams * seg

    def split(axis):
        idx = jax.lax.broadcasted_iota(jnp.int32, (rows, rows), axis)
        is_mem = idx < tok0
        stream = jnp.where(is_mem, idx // n_mem, (idx - tok0) // seg)
        pos = jnp.where(is_mem, idx % n_mem, n_mem + (idx - tok0) % seg)
        return stream, pos

    q_stream, q_pos = split(0)
    k_stream, k_pos = split(1)
    same = q_stream == k_stream
    visible = same & ((q_pos < n_mem) | (q_pos >= k_pos))
    fill = jnp.where(same, _MASK_FILL, -jnp.inf).astype(_F32)
    return visible, fill


def _kernel(xt_hbm, mem0_ref, wq_hbm, wk_hbm, wv_hbm, wot_hbm, w1_hbm, w3_hbm, w2t_hbm,
            out_hbm,
            xt_ref, x_ref, rq_ref, rk_ref, rv_ref, wqkv_ref, wot_ref, wo_ref,
            r1_ref, r3_ref, w1_ref, w3_ref, w2t_ref, w2_ref, sqkv_ref, s1_ref, s3_ref, so_ref, s2_ref,
            o_ref, hid_ref, a_ref, xa_ref, x1_ref, wide_ref, y_ref, in_sems, out_sems,
            *, seg, n_heads, dh):
    seq, dm = x_ref.shape
    n_mem = mem0_ref.shape[0]
    n_seg = seq // seg
    ffn = w1_ref.shape[1]
    wqkv_ref, wo_ref, w1_ref, w3_ref, w2_ref = map(
        _Packed, (wqkv_ref, wo_ref, w1_ref, w3_ref, w2_ref))
    sqkv_ref, s1_ref, s3_ref, so_ref, s2_ref = map(
        _Packed, (sqkv_ref, s1_ref, s3_ref, so_ref, s2_ref))
    o_ref, hid_ref = _Packed(o_ref), _Packed(hid_ref)
    scale = dh ** -0.5
    n_grp = n_heads // 2
    tok0 = 2 * n_mem
    full = dm - _HALF
    mid = slice(_HALF, _LANES)
    fc = _FFN_CHUNK
    xc = _XPOSE_CHUNK
    wc = ffn // _FFN_DMA_CHUNKS

    def cols(ref, start, size):
        return ref.at[:, start:start + size]

    def rows_of(ref, start, size):
        return ref.at[start:start + size, :]

    raw_rows = dm * n_heads // _QKV_DMA_CHUNKS
    transfers = [("x_head", cols(xt_hbm, 0, xc), cols(xt_ref, 0, xc))]
    for name, src, dst in (("wq", wq_hbm, rq_ref), ("wk", wk_hbm, rk_ref), ("wv", wv_hbm, rv_ref)):
        for c in range(_QKV_DMA_CHUNKS):
            transfers.append(((name, c), rows_of(src, c * raw_rows, raw_rows),
                              rows_of(dst, c * raw_rows, raw_rows)))
    transfers.append(("wo", wot_hbm, wot_ref))
    for c in range(0, ffn, wc):
        transfers.append((("w1", c), cols(w1_hbm, c, wc), cols(r1_ref, c, wc)))
        transfers.append((("w3", c), cols(w3_hbm, c, wc), cols(r3_ref, c, wc)))
    for c in range(0, ffn, wc):
        transfers.append((("w2", c), cols(w2t_hbm, c, wc), cols(w2t_ref, c, wc)))
    transfers.append(("x_tail", cols(xt_hbm, xc, seq - xc), cols(xt_ref, xc, seq - xc)))
    copies = {name: pltpu.make_async_copy(src, dst, in_sems.at[n])
              for n, (name, src, dst) in enumerate(transfers)}

    def arrive(name):
        copies[name].wait()

    def project(h, grp):
        rows = slice(grp * dm, grp * dm + full)
        both = _paired_dot(h, wqkv_ref[rows, 0:3 * dh], wqkv_ref[rows, 3 * dh:],
                           sqkv_ref[grp * _LANES:(grp + 1) * _LANES, :])
        return [[qkv[:, m * dh:(m + 1) * dh].astype(_BF16) for m in range(3)] for qkv in both]

    def probabilities(qkv, visible, fill):
        probs = []
        for q, k, _ in qkv:
            s = jnp.where(visible, _dot_nt(q, k) * scale, fill)
            p = jnp.exp(s - jnp.max(s, axis=-1, keepdims=True))
            probs.append((p * (1.0 / jnp.sum(p, axis=-1, keepdims=True))).astype(_BF16))
        return probs

    def heads(h, n_streams, fillers=()):
        rows = h.shape[0]
        visible, fill = _mask_tables(n_streams, n_mem, seg)
        qkv, probs = {}, {}
        for t in range(n_grp + _PV_LAG):
            if t < n_grp:
                qkv[t] = project(h, t)
            elif t - n_grp < len(fillers):
                fillers[t - n_grp]()
            if 0 <= t - _QK_LAG < n_grp:
                probs[t - _QK_LAG] = probabilities(qkv[t - _QK_LAG], visible, fill)
            if 0 <= t - _PV_LAG:
                grp = t - _PV_LAG
                outs = [_dot(p, v) for p, (_, _, v) in zip(probs.pop(grp), qkv.pop(grp))]
                for part, out in enumerate(outs + [outs[0] + outs[1]]):
                    col = (part * n_grp + grp) * dh
                    o_ref[0:rows, col:col + dh] = out.astype(_BF16)

    def attend(h, n_streams):
        rows, half, wide = slice(0, h.shape[0]), n_grp * dh, []
        cut_u, cut_v = (n_grp - _PV_LAG) * dh, half + (n_grp - _PV_LAG + 1) * dh

        def part(lo, hi):
            return lambda: wide.append(_output_wide(o_ref, rows, wo_ref, lo, hi))

        heads(h, n_streams, (part(0, cut_u), part(half, cut_v)))
        part(cut_u, half)()
        part(cut_v, 2 * half)()
        wide = (wide[0] + wide[1]) + (wide[2] + wide[3])
        return _output_finish(o_ref, rows, wo_ref, so_ref, wide)

    def pair_gate_up(lo, hi):
        for raw, w_ref, s_ref in ((r1_ref, w1_ref, s1_ref), (r3_ref, w3_ref, s3_ref)):
            w_ref[0:_HALF, lo:hi] = raw[0:_HALF, lo:hi]
            w_ref[_LANES:, lo:hi] = raw[_LANES:full, lo:hi]
            for c in range(lo, hi, fc):
                ca, cb = slice(c, c + fc // 2), slice(c + fc // 2, c + fc)
                w_ref[mid, ca], w_ref[mid, cb], s_ref[:, c // 2:(c + fc) // 2] = _pair_weights(
                    raw[mid, ca], raw[full:, ca], raw[mid, cb], raw[full:, cb])

    def gate_up(f_in, lo=0, hi=ffn):
        for c in range(lo, hi, fc):
            ca, cb = slice(c, c + fc // 2), slice(c + fc // 2, c + fc)
            cs = slice(c // 2, (c + fc) // 2)
            gates = _paired_dot(f_in, w1_ref[0:full, ca], w1_ref[0:full, cb], s1_ref[:, cs])
            ups = _paired_dot(f_in, w3_ref[0:full, ca], w3_ref[0:full, cb], s3_ref[:, cs])
            hids = [gate * jax.nn.sigmoid(gate) * up for gate, up in zip(gates, ups)]
            for part, hid in enumerate(hids + [hids[0] + hids[1]]):
                col = (part * ffn + c) // 2
                hid_ref[0:hid.shape[0], col:col + fc // 2] = hid.astype(_BF16)

    def stage_down(lo, hi):
        for c in range(lo, hi, fc):
            rows_u = slice(c // 2, (c + fc) // 2)
            rows_v = slice((ffn + c) // 2, (ffn + c + fc) // 2)
            w2_ref[rows_u, :], w2_ref[rows_v, :], s2_ref[rows_u, :] = _pair_output_weights(
                w2t_ref[:, c:c + fc // 2], w2t_ref[:, c + fc // 2:c + fc])

    def single_stream_rows(mem, x):
        return _split_lhs(jnp.concatenate([mem, _layernorm(x)], axis=0))

    def write_back(t, size):
        xt_ref[:, t:t + size] = y_ref[t:t + size, :].T
        copy = pltpu.make_async_copy(
            cols(xt_ref, t, size), cols(out_hbm, t, size), out_sems.at[pl.cdiv(t, xc)])
        copy.start()
        return copy

    for copy in copies.values():
        copy.start()
    arrive("x_head")
    x_ref[0:xc, :] = xt_ref[:, 0:xc].T

    pairs = n_heads // 2
    d_chunk = dm // _QKV_DMA_CHUNKS
    for m, (name, raw_ref) in enumerate((("wq", rq_ref), ("wk", rk_ref), ("wv", rv_ref))):
        words = raw_ref.bitcast(jnp.uint32)
        for c in range(_QKV_DMA_CHUNKS):
            arrive((name, c))

            def regroup(quad, carry, m=m, c=c, words=words):
                start = pl.multiple_of(c * d_chunk * pairs + quad * _WORD_TILE, _WORD_TILE)
                view = words.at[pl.ds(start, d_chunk * pairs - pairs + _WORD_TILE), :]
                for r in range(_WORD_TILE):
                    even_d = view[pl.ds(r, d_chunk // 2, stride=n_heads), :]
                    odd_d = view[pl.ds(r + pairs, d_chunk // 2, stride=n_heads), :]
                    lo = (even_d & jnp.uint32(0xFFFF)) | (odd_d << 16)
                    hi = (even_d >> 16) | (odd_d & jnp.uint32(0xFFFF0000))
                    row = (quad * _WORD_TILE + r) * (dm // 2) + c * (d_chunk // 2)
                    for half, val in enumerate((lo, hi)):
                        col = (half * 3 + m) * dh
                        wqkv_ref.ref[pl.ds(pl.multiple_of(row, 8), d_chunk // 2), col:col + dh] = val
                return carry

            jax.lax.fori_loop(0, pairs // _WORD_TILE, regroup, 0)

    def pair_heads(grp, carry):
        ca, cb = slice(0, 3 * dh), slice(3 * dh, 6 * dh)
        mid_rows, tail_rows = (grp * dm + _HALF, _HALF), (grp * dm + full, _HALF)
        (wqkv_ref[mid_rows, ca], wqkv_ref[mid_rows, cb],
         sqkv_ref[(grp * _LANES, _LANES), :]) = _pair_weights(
             wqkv_ref[mid_rows, ca], wqkv_ref[tail_rows, ca],
             wqkv_ref[mid_rows, cb], wqkv_ref[tail_rows, cb])
        return carry

    jax.lax.fori_loop(0, n_grp, pair_heads, 0)

    mem0 = mem0_ref[...].astype(_F32)
    a_ref[0:n_mem, :] = mem0

    def first_segments(s, carry):
        x_s = x_ref[pl.ds(pl.multiple_of(s * seg, seg), seg), :].astype(_F32)
        heads(single_stream_rows(a_ref[0:n_mem, :], x_s), 1)

        @pl.when(s == 0)
        def _():
            arrive("wo")

            def stage_wo(grp, carry):
                rows_u, rows_v = (grp * dh, dh), ((n_grp + grp) * dh, dh)
                wo_ref[rows_u, :], wo_ref[rows_v, :], so_ref[rows_u, :] = _pair_output_weights(
                    wot_ref[2 * grp], wot_ref[2 * grp + 1])
                return carry

            jax.lax.fori_loop(0, n_grp, stage_wo, 0, unroll=2)

        a = _output_dot(o_ref, slice(0, n_mem + seg), wo_ref, so_ref)
        a_ref[0:n_mem, :] = a[:n_mem]
        a_ref[pl.ds(pl.multiple_of(tok0 + (1 - s) * seg, n_mem), seg), :] = a[n_mem:]
        return carry

    jax.lax.fori_loop(0, 2, first_segments, 0)
    a_ref[n_mem:tok0, :] = mem0
    x1 = jnp.concatenate([x_ref[seg:2 * seg, :], x_ref[0:seg, :]], axis=0).astype(_F32)
    x1 = x1 + a_ref[tok0:, :]
    x1_ref[...] = x1
    f_in = _split_lhs(_layernorm(x1))
    for c in range(0, ffn, wc):
        arrive(("w1", c))
        arrive(("w3", c))
        pair_gate_up(c, c + wc)
        gate_up(f_in, c, c + wc)
    for c in range(0, ffn, wc):
        arrive(("w2", c))
        stage_down(c, c + wc)

    both = slice(0, 2 * seg)

    def feed_forward(out_row):
        y = x1_ref[...] + _output_finish(hid_ref, both, w2_ref, s2_ref, wide_ref[...])
        y_ref[pl.ds(out_row, seg), :] = y[seg:].astype(y_ref.dtype)
        x1 = xa_ref[...] + a_ref[tok0:, :]
        x1_ref[...] = x1
        gate_up(_split_lhs(_layernorm(x1)))
        return y[:seg]

    def attend_both(x_row, x2):
        xa = jnp.concatenate([x_ref[pl.ds(x_row, seg), :].astype(_F32), x2], axis=0)
        xa_ref[...] = xa
        a_ref[...] = attend(
            _split_lhs(jnp.concatenate([a_ref[0:tok0, :], _layernorm(xa)], axis=0)), 2)

    def step(i, carry):
        @pl.when(i == xc // seg - 1)
        def _():
            arrive("x_tail")
            for t in range(xc, seq, xc):
                x_ref[t:t + xc, :] = xt_ref[:, t:t + xc].T

        x2 = feed_forward(pl.multiple_of(jnp.maximum(i - 3, 0) * seg, seg))
        wide_ref[...] = _output_wide(hid_ref, both, w2_ref)
        attend_both(pl.multiple_of((i + 1) * seg, seg), x2)
        return carry

    wide_ref[...] = _output_wide(hid_ref, both, w2_ref)
    attend_both(2 * seg, x1_ref[seg:, :] + _output_finish(
        hid_ref, slice(seg, 2 * seg), w2_ref, s2_ref, wide_ref[seg:, :]))
    jax.lax.fori_loop(2, n_seg - 1, step, 0)

    x_s0 = feed_forward(seq - 4 * seg)
    a = attend(single_stream_rows(a_ref[n_mem:tok0, :], x_s0), 1)
    y = x1_ref[...] + _output_dot(hid_ref, both, w2_ref, s2_ref)
    y_ref[seq - 3 * seg:seq - 2 * seg, :] = y[seg:].astype(y_ref.dtype)
    x1_s0 = x_s0 + a[n_mem:]
    last = seq - _LANES
    writes = [write_back(t, min(xc, last - t)) for t in range(0, last, xc)]
    a = attend(single_stream_rows(a[:n_mem], y[:seg]), 1)
    x1 = jnp.concatenate([x1_s0, y[:seg] + a[n_mem:]], axis=0)
    gate_up(_split_lhs(_layernorm(x1)))
    y_ref[seq - 2 * seg:, :] = (x1 + _output_dot(hid_ref, both, w2_ref, s2_ref)).astype(y_ref.dtype)
    writes.append(write_back(last, _LANES))
    for copy in writes:
        copy.wait()


@functools.partial(jax.jit, static_argnames=("A_seg_len",))
def pallas_interleave_layers__memory_aug_recurrent_mem_tr__glu_gated_swiglu__prompt_kernel(
    A_x: jax.Array,
    A_mem0: jax.Array,
    A_Wq: jax.Array,
    A_Wk: jax.Array,
    A_Wv: jax.Array,
    A_Wo: jax.Array,
    A_seg_len: int,
    B_x: jax.Array,
    B_w1: jax.Array,
    B_w3: jax.Array,
    B_w2: jax.Array,
):
    del B_x
    batch, seq, dm = A_x.shape
    _, n_heads, dh = A_Wq.shape
    n_mem = A_mem0.shape[1]
    ffn = B_w1.shape[1]
    seg = int(A_seg_len)
    assert batch == 1 and seq % _XPOSE_CHUNK == 0 and _XPOSE_CHUNK % seg == 0 and _XPOSE_CHUNK >= 3 * seg
    rows = 2 * (n_mem + seg)
    full = dm - _HALF

    vmem = pl.BlockSpec(memory_space=pltpu.VMEM)
    hbm = pl.BlockSpec(memory_space=pltpu.HBM)
    out_t = pl.pallas_call(
        functools.partial(_kernel, seg=seg, n_heads=n_heads, dh=dh),
        out_shape=jax.ShapeDtypeStruct((dm, seq), A_x.dtype),
        in_specs=[hbm, vmem] + [hbm] * 7,
        out_specs=hbm,
        scratch_shapes=[
            pltpu.VMEM((dm, seq), _BF16),
            pltpu.VMEM((seq, dm), _BF16),
            pltpu.VMEM((dm * n_heads, dh), _BF16),
            pltpu.VMEM((dm * n_heads, dh), _BF16),
            pltpu.VMEM((dm * n_heads, dh), _BF16),
            _packed_scratch(n_heads // 2 * dm, 6 * dh),
            pltpu.VMEM((n_heads, dm, dh), _BF16),
            _packed_scratch(n_heads * dh, full),
            pltpu.VMEM((dm, ffn), _BF16),
            pltpu.VMEM((dm, ffn), _BF16),
            _packed_scratch(full, ffn),
            _packed_scratch(full, ffn),
            pltpu.VMEM((dm, ffn), _BF16),
            _packed_scratch(ffn, full),
            _packed_scratch(n_heads // 2 * _LANES, 3 * dh),
            _packed_scratch(_LANES, ffn // 2),
            _packed_scratch(_LANES, ffn // 2),
            _packed_scratch(n_heads * dh // 2, _LANES),
            _packed_scratch(ffn // 2, _LANES),
            _packed_scratch(rows, n_heads * dh * 3 // 2),
            _packed_scratch(2 * seg, ffn * 3 // 2),
            pltpu.VMEM((rows, dm), _F32),
            pltpu.VMEM((2 * seg, dm), _F32),
            pltpu.VMEM((2 * seg, dm), _F32),
            pltpu.VMEM((2 * seg, dm - _HALF - _LANES), _F32),
            pltpu.VMEM((seq, dm), _BF16),
            pltpu.SemaphoreType.DMA((3 + 3 * _QKV_DMA_CHUNKS + 3 * _FFN_DMA_CHUNKS,)),
            pltpu.SemaphoreType.DMA((seq // _XPOSE_CHUNK + 1,)),
        ],
        compiler_params=pltpu.CompilerParams(vmem_limit_bytes=110 * 1024 * 1024),
    )(
        A_x.reshape(seq, dm).T,
        A_mem0.reshape(n_mem, dm),
        A_Wq.reshape(dm * n_heads, dh),
        A_Wk.reshape(dm * n_heads, dh),
        A_Wv.reshape(dm * n_heads, dh),
        A_Wo.transpose(0, 2, 1),
        B_w1,
        B_w3,
        B_w2.T,
    )
    return out_t.T.reshape(batch, seq, dm)
```

```python
import functools

import jax
import jax.numpy as jnp
import numpy as np
import jax.experimental.pallas as pl
import jax.experimental.pallas.tpu as pltpu

_EPS = 1e-5
_MASK_FILL = -1000000000.0
_QK_LAG = 1
_PV_LAG = 4
_FFN_CHUNK = 512
_XPOSE_CHUNK = 256
_FFN_DMA_CHUNKS = 3
_QKV_DMA_CHUNKS = 2
_WORD_TILE = 4

_LANES = 128
_HALF = _LANES // 2
_F32 = jnp.float32
_BF16 = jnp.bfloat16


def _layernorm(x):
    mean = jnp.mean(x, axis=-1, keepdims=True)
    cen = x - mean
    var = jnp.mean(cen * cen, axis=-1, keepdims=True)
    return cen * jax.lax.rsqrt(var + _EPS)


def _dot(a, b):
    return jnp.dot(a, b, preferred_element_type=_F32)


def _dot_nt(a, b):
    return jax.lax.dot_general(a, b, (((1,), (1,)), ((), ())), preferred_element_type=_F32)


class _Packed:
    def __init__(self, ref):
        self.ref = ref
        self.shape = (2 * ref.shape[0], ref.shape[1])

    def _index(self, idx):
        rows, cols = idx
        if isinstance(rows, slice):
            lo, hi, _ = rows.indices(self.shape[0])
            return slice(lo // 2, hi // 2), cols
        start, size = rows
        return pl.ds(pl.multiple_of(start // 2, size // 2), size // 2), cols

    def __getitem__(self, idx):
        return pltpu.bitcast(self.ref[self._index(idx)], _BF16)

    def __setitem__(self, idx, value):
        self.ref[self._index(idx)] = pltpu.bitcast(value, jnp.uint32)


def _packed_scratch(rows, cols):
    return pltpu.VMEM((rows // 2, cols), jnp.uint32)


def _split_lhs(x):
    full = x.shape[1] - _HALF
    first, rest = x[:, :_LANES], x[:, _LANES:full]
    tail = x[:, full:]
    lhs_b0 = jnp.concatenate([first[:, :_HALF], tail], axis=1)
    lhs_s = jnp.concatenate([tail, first[:, _HALF:]], axis=1)
    return jnp.concatenate([first, rest, lhs_b0, lhs_s], axis=1).astype(_BF16)


def _paired_dot(lhs, w_a, w_b, w_s):
    full = w_a.shape[0]
    shared = _dot(lhs[:, full + _LANES:], w_s)
    lhs_b = jnp.concatenate([lhs[:, full:full + _LANES], lhs[:, _LANES:full]], axis=1)
    return _dot(lhs[:, :full], w_a) + shared, _dot(lhs_b, w_b) + shared


def _pair_weights(a_mid, a_tail, b_mid, b_tail):
    a_new = (a_mid.astype(_F32) - b_mid.astype(_F32)).astype(_BF16)
    b_new = (b_tail.astype(_F32) - a_tail.astype(_F32)).astype(_BF16)
    return a_new, b_new, jnp.concatenate([a_tail, b_mid], axis=0)


def _pair_output_weights(ut, vt):
    full = ut.shape[0] - _HALF
    mid = slice(_HALF, _LANES)
    u_new, v_new, shared = _pair_weights(ut[mid], ut[full:], vt[mid], vt[full:])
    u = jnp.concatenate([ut[:_HALF], u_new, ut[_LANES:full]], axis=0)
    v = jnp.concatenate([vt[:_HALF], v_new, vt[_LANES:full]], axis=0)
    return u.T, v.T, shared.T


def _output_wide(lhs_ref, rows, w_ref, lo=0, hi=None):
    hi = w_ref.shape[0] if hi is None else hi
    return _dot(lhs_ref[rows, lo:hi], w_ref[lo:hi, _LANES:])


def _output_finish(lhs_ref, rows, w_ref, s_ref, wide):
    half = s_ref.shape[0]
    u0 = _dot(lhs_ref[rows, 0:half], w_ref[0:half, 0:_LANES])
    v0 = _dot(lhs_ref[rows, half:2 * half], w_ref[half:, 0:_LANES])
    shared = _dot(lhs_ref[rows, 2 * half:], s_ref[:, :])
    is_low = jax.lax.broadcasted_iota(jnp.int32, u0.shape, 1) < _HALF
    first = u0 + jnp.where(is_low, v0, shared)
    last = v0[:, _HALF:] + shared[:, :_HALF]
    return jnp.concatenate([first, wide, last], axis=1)


def _output_dot(lhs_ref, rows, w_ref, s_ref):
    return _output_finish(lhs_ref, rows, w_ref, s_ref, _output_wide(lhs_ref, rows, w_ref))


def _mask_tables(n_streams, n_mem, seg):
    tok0 = n_streams * n_mem
    rows = tok0 + n_streams * seg

    def split(axis):
        idx = jax.lax.broadcasted_iota(jnp.int32, (rows, rows), axis)
        is_mem = idx < tok0
        stream = jnp.where(is_mem, idx // n_mem, (idx - tok0) // seg)
        pos = jnp.where(is_mem, idx % n_mem, n_mem + (idx - tok0) % seg)
        return stream, pos

    q_stream, q_pos = split(0)
    k_stream, k_pos = split(1)
    same = q_stream == k_stream
    visible = same & ((q_pos < n_mem) | (q_pos >= k_pos))
    fill = jnp.where(same, _MASK_FILL, -jnp.inf).astype(_F32)
    return visible, fill


def _kernel(xt_hbm, mem0_ref, wq_hbm, wk_hbm, wv_hbm, wot_hbm, w1_hbm, w3_hbm, w2t_hbm,
            out_hbm,
            xt_ref, x_ref, rq_ref, rk_ref, rv_ref, wqkv_ref, wot_ref, wo_ref,
            r1_ref, r3_ref, w1_ref, w3_ref, w2t_ref, w2_ref, sqkv_ref, s1_ref, s3_ref, so_ref, s2_ref,
            o_ref, hid_ref, a_ref, xa_ref, x1_ref, wide_ref, y_ref, in_sems, out_sems,
            *, seg, n_heads, dh):
    seq, dm = x_ref.shape
    n_mem = mem0_ref.shape[0]
    n_seg = seq // seg
    ffn = w1_ref.shape[1]
    wqkv_ref, wo_ref, w1_ref, w3_ref, w2_ref = map(
        _Packed, (wqkv_ref, wo_ref, w1_ref, w3_ref, w2_ref))
    sqkv_ref, s1_ref, s3_ref, so_ref, s2_ref = map(
        _Packed, (sqkv_ref, s1_ref, s3_ref, so_ref, s2_ref))
    o_ref, hid_ref = _Packed(o_ref), _Packed(hid_ref)
    scale = dh ** -0.5
    n_grp = n_heads // 2
    tok0 = 2 * n_mem
    full = dm - _HALF
    mid = slice(_HALF, _LANES)
    fc = _FFN_CHUNK
    xc = _XPOSE_CHUNK
    wc = ffn // _FFN_DMA_CHUNKS

    def cols(ref, start, size):
        return ref.at[:, start:start + size]

    def rows_of(ref, start, size):
        return ref.at[start:start + size, :]

    raw_rows = dm * n_heads // _QKV_DMA_CHUNKS
    transfers = [("x_head", cols(xt_hbm, 0, xc), cols(xt_ref, 0, xc))]
    for name, src, dst in (("wq", wq_hbm, rq_ref), ("wk", wk_hbm, rk_ref), ("wv", wv_hbm, rv_ref)):
        for c in range(_QKV_DMA_CHUNKS):
            transfers.append(((name, c), rows_of(src, c * raw_rows, raw_rows),
                              rows_of(dst, c * raw_rows, raw_rows)))
    transfers.append(("wo", wot_hbm, wot_ref))
    for c in range(0, ffn, wc):
        transfers.append((("w1", c), cols(w1_hbm, c, wc), cols(r1_ref, c, wc)))
        transfers.append((("w3", c), cols(w3_hbm, c, wc), cols(r3_ref, c, wc)))
    for c in range(0, ffn, wc):
        transfers.append((("w2", c), cols(w2t_hbm, c, wc), cols(w2t_ref, c, wc)))
    transfers.append(("x_tail", cols(xt_hbm, xc, seq - xc), cols(xt_ref, xc, seq - xc)))
    copies = {name: pltpu.make_async_copy(src, dst, in_sems.at[n])
              for n, (name, src, dst) in enumerate(transfers)}

    def arrive(name):
        copies[name].wait()

    def project(h, grp):
        rows = slice(grp * dm, grp * dm + full)
        both = _paired_dot(h, wqkv_ref[rows, 0:3 * dh], wqkv_ref[rows, 3 * dh:],
                           sqkv_ref[grp * _LANES:(grp + 1) * _LANES, :])
        return [[qkv[:, m * dh:(m + 1) * dh].astype(_BF16) for m in range(3)] for qkv in both]

    def probabilities(qkv, visible, fill):
        probs = []
        for q, k, _ in qkv:
            s = jnp.where(visible, _dot_nt(q, k) * scale, fill)
            p = jnp.exp(s - jnp.max(s, axis=-1, keepdims=True))
            probs.append((p * (1.0 / jnp.sum(p, axis=-1, keepdims=True))).astype(_BF16))
        return probs

    def heads(h, n_streams, fillers=()):
        rows = h.shape[0]
        visible, fill = _mask_tables(n_streams, n_mem, seg)
        qkv, probs = {}, {}
        for t in range(n_grp + _PV_LAG):
            if t < n_grp:
                qkv[t] = project(h, t)
            elif t - n_grp < len(fillers):
                fillers[t - n_grp]()
            if 0 <= t - _QK_LAG < n_grp:
                probs[t - _QK_LAG] = probabilities(qkv[t - _QK_LAG], visible, fill)
            if 0 <= t - _PV_LAG:
                grp = t - _PV_LAG
                outs = [_dot(p, v) for p, (_, _, v) in zip(probs.pop(grp), qkv.pop(grp))]
                for part, out in enumerate(outs + [outs[0] + outs[1]]):
                    col = (part * n_grp + grp) * dh
                    o_ref[0:rows, col:col + dh] = out.astype(_BF16)

    def attend(h, n_streams):
        rows, half, wide = slice(0, h.shape[0]), n_grp * dh, []
        cut_u, cut_v = (n_grp - _PV_LAG) * dh, half + (n_grp - _PV_LAG + 1) * dh

        def part(lo, hi):
            return lambda: wide.append(_output_wide(o_ref, rows, wo_ref, lo, hi))

        heads(h, n_streams, (part(0, cut_u), part(half, cut_v)))
        part(cut_u, half)()
        part(cut_v, 2 * half)()
        wide = (wide[0] + wide[1]) + (wide[2] + wide[3])
        return _output_finish(o_ref, rows, wo_ref, so_ref, wide)

    def pair_gate_up(lo, hi):
        for raw, w_ref, s_ref in ((r1_ref, w1_ref, s1_ref), (r3_ref, w3_ref, s3_ref)):
            w_ref[0:_HALF, lo:hi] = raw[0:_HALF, lo:hi]
            w_ref[_LANES:, lo:hi] = raw[_LANES:full, lo:hi]
            for c in range(lo, hi, fc):
                ca, cb = slice(c, c + fc // 2), slice(c + fc // 2, c + fc)
                w_ref[mid, ca], w_ref[mid, cb], s_ref[:, c // 2:(c + fc) // 2] = _pair_weights(
                    raw[mid, ca], raw[full:, ca], raw[mid, cb], raw[full:, cb])

    def gate_up(f_in, lo=0, hi=ffn):
        for c in range(lo, hi, fc):
            ca, cb = slice(c, c + fc // 2), slice(c + fc // 2, c + fc)
            cs = slice(c // 2, (c + fc) // 2)
            gates = _paired_dot(f_in, w1_ref[0:full, ca], w1_ref[0:full, cb], s1_ref[:, cs])
            ups = _paired_dot(f_in, w3_ref[0:full, ca], w3_ref[0:full, cb], s3_ref[:, cs])
            hids = [gate * jax.nn.sigmoid(gate) * up for gate, up in zip(gates, ups)]
            for part, hid in enumerate(hids + [hids[0] + hids[1]]):
                col = (part * ffn + c) // 2
                hid_ref[0:hid.shape[0], col:col + fc // 2] = hid.astype(_BF16)

    def stage_down(lo, hi):
        for c in range(lo, hi, fc):
            rows_u = slice(c // 2, (c + fc) // 2)
            rows_v = slice((ffn + c) // 2, (ffn + c + fc) // 2)
            w2_ref[rows_u, :], w2_ref[rows_v, :], s2_ref[rows_u, :] = _pair_output_weights(
                w2t_ref[:, c:c + fc // 2], w2t_ref[:, c + fc // 2:c + fc])

    def single_stream_rows(mem, x):
        return _split_lhs(jnp.concatenate([mem, _layernorm(x)], axis=0))

    def write_back(t, size):
        xt_ref[:, t:t + size] = y_ref[t:t + size, :].T
        copy = pltpu.make_async_copy(
            cols(xt_ref, t, size), cols(out_hbm, t, size), out_sems.at[pl.cdiv(t, xc)])
        copy.start()
        return copy

    for copy in copies.values():
        copy.start()
    arrive("x_head")
    x_ref[0:xc, :] = xt_ref[:, 0:xc].T

    pairs = n_heads // 2
    d_chunk = dm // _QKV_DMA_CHUNKS
    for m, (name, raw_ref) in enumerate((("wq", rq_ref), ("wk", rk_ref), ("wv", rv_ref))):
        words = raw_ref.bitcast(jnp.uint32)
        for c in range(_QKV_DMA_CHUNKS):
            arrive((name, c))

            def regroup(quad, carry, m=m, c=c, words=words):
                start = pl.multiple_of(c * d_chunk * pairs + quad * _WORD_TILE, _WORD_TILE)
                view = words.at[pl.ds(start, d_chunk * pairs - pairs + _WORD_TILE), :]
                for r in range(_WORD_TILE):
                    even_d = view[pl.ds(r, d_chunk // 2, stride=n_heads), :]
                    odd_d = view[pl.ds(r + pairs, d_chunk // 2, stride=n_heads), :]
                    lo = (even_d & jnp.uint32(0xFFFF)) | (odd_d << 16)
                    hi = (even_d >> 16) | (odd_d & jnp.uint32(0xFFFF0000))
                    row = (quad * _WORD_TILE + r) * (dm // 2) + c * (d_chunk // 2)
                    for half, val in enumerate((lo, hi)):
                        col = (half * 3 + m) * dh
                        wqkv_ref.ref[pl.ds(pl.multiple_of(row, 8), d_chunk // 2), col:col + dh] = val
                return carry

            jax.lax.fori_loop(0, pairs // _WORD_TILE, regroup, 0)

    def pair_heads(grp, carry):
        ca, cb = slice(0, 3 * dh), slice(3 * dh, 6 * dh)
        mid_rows, tail_rows = (grp * dm + _HALF, _HALF), (grp * dm + full, _HALF)
        (wqkv_ref[mid_rows, ca], wqkv_ref[mid_rows, cb],
         sqkv_ref[(grp * _LANES, _LANES), :]) = _pair_weights(
             wqkv_ref[mid_rows, ca], wqkv_ref[tail_rows, ca],
             wqkv_ref[mid_rows, cb], wqkv_ref[tail_rows, cb])
        return carry

    jax.lax.fori_loop(0, n_grp, pair_heads, 0)

    mem0 = mem0_ref[...].astype(_F32)
    a_ref[0:n_mem, :] = mem0

    def first_segments(s, carry):
        x_s = x_ref[pl.ds(pl.multiple_of(s * seg, seg), seg), :].astype(_F32)
        heads(single_stream_rows(a_ref[0:n_mem, :], x_s), 1)

        @pl.when(s == 0)
        def _():
            arrive("wo")

            def stage_wo(grp, carry):
                rows_u, rows_v = (grp * dh, dh), ((n_grp + grp) * dh, dh)
                wo_ref[rows_u, :], wo_ref[rows_v, :], so_ref[rows_u, :] = _pair_output_weights(
                    wot_ref[2 * grp], wot_ref[2 * grp + 1])
                return carry

            jax.lax.fori_loop(0, n_grp, stage_wo, 0, unroll=2)

        a = _output_dot(o_ref, slice(0, n_mem + seg), wo_ref, so_ref)
        a_ref[0:n_mem, :] = a[:n_mem]
        a_ref[pl.ds(pl.multiple_of(tok0 + (1 - s) * seg, n_mem), seg), :] = a[n_mem:]
        return carry

    jax.lax.fori_loop(0, 2, first_segments, 0)
    a_ref[n_mem:tok0, :] = mem0
    x1 = jnp.concatenate([x_ref[seg:2 * seg, :], x_ref[0:seg, :]], axis=0).astype(_F32)
    x1 = x1 + a_ref[tok0:, :]
    x1_ref[...] = x1
    f_in = _split_lhs(_layernorm(x1))
    for c in range(0, ffn, wc):
        arrive(("w1", c))
        arrive(("w3", c))
        pair_gate_up(c, c + wc)
        gate_up(f_in, c, c + wc)
    both = slice(0, 2 * seg)
    wide = None
    for c in range(0, ffn, wc):
        arrive(("w2", c))
        stage_down(c, c + wc)
        for lo in (c // 2, (ffn + c) // 2):
            part = _output_wide(hid_ref, both, w2_ref, lo, lo + wc // 2)
            wide = part if wide is None else wide + part
    wide_ref[...] = wide

    def feed_forward(out_row):
        y = x1_ref[...] + _output_finish(hid_ref, both, w2_ref, s2_ref, wide_ref[...])
        y_ref[pl.ds(out_row, seg), :] = y[seg:].astype(y_ref.dtype)
        x1 = xa_ref[...] + a_ref[tok0:, :]
        x1_ref[...] = x1
        gate_up(_split_lhs(_layernorm(x1)))
        return y[:seg]

    def attend_both(x_row, x2):
        xa = jnp.concatenate([x_ref[pl.ds(x_row, seg), :].astype(_F32), x2], axis=0)
        xa_ref[...] = xa
        a_ref[...] = attend(
            _split_lhs(jnp.concatenate([a_ref[0:tok0, :], _layernorm(xa)], axis=0)), 2)

    def step(i, carry):
        @pl.when(i == xc // seg - 1)
        def _():
            arrive("x_tail")
            for t in range(xc, seq, xc):
                x_ref[t:t + xc, :] = xt_ref[:, t:t + xc].T

        x2 = feed_forward(pl.multiple_of(jnp.maximum(i - 3, 0) * seg, seg))
        wide_ref[...] = _output_wide(hid_ref, both, w2_ref)
        attend_both(pl.multiple_of((i + 1) * seg, seg), x2)
        return carry

    attend_both(2 * seg, x1_ref[seg:, :] + _output_finish(
        hid_ref, slice(seg, 2 * seg), w2_ref, s2_ref, wide_ref[seg:, :]))
    jax.lax.fori_loop(2, n_seg - 1, step, 0)

    x_s0 = feed_forward(seq - 4 * seg)
    a = attend(single_stream_rows(a_ref[n_mem:tok0, :], x_s0), 1)
    y = x1_ref[...] + _output_dot(hid_ref, both, w2_ref, s2_ref)
    y_ref[seq - 3 * seg:seq - 2 * seg, :] = y[seg:].astype(y_ref.dtype)
    x1_s0 = x_s0 + a[n_mem:]
    last = seq - _LANES
    writes = [write_back(t, min(xc, last - t)) for t in range(0, last, xc)]
    a = attend(single_stream_rows(a[:n_mem], y[:seg]), 1)
    x1 = jnp.concatenate([x1_s0, y[:seg] + a[n_mem:]], axis=0)
    gate_up(_split_lhs(_layernorm(x1)))
    y_ref[seq - 2 * seg:, :] = (x1 + _output_dot(hid_ref, both, w2_ref, s2_ref)).astype(y_ref.dtype)
    writes.append(write_back(last, _LANES))
    for copy in writes:
        copy.wait()


@functools.partial(jax.jit, static_argnames=("A_seg_len",))
def pallas_interleave_layers__memory_aug_recurrent_mem_tr__glu_gated_swiglu__prompt_kernel(
    A_x: jax.Array,
    A_mem0: jax.Array,
    A_Wq: jax.Array,
    A_Wk: jax.Array,
    A_Wv: jax.Array,
    A_Wo: jax.Array,
    A_seg_len: int,
    B_x: jax.Array,
    B_w1: jax.Array,
    B_w3: jax.Array,
    B_w2: jax.Array,
):
    del B_x
    batch, seq, dm = A_x.shape
    _, n_heads, dh = A_Wq.shape
    n_mem = A_mem0.shape[1]
    ffn = B_w1.shape[1]
    seg = int(A_seg_len)
    assert batch == 1 and seq % _XPOSE_CHUNK == 0 and _XPOSE_CHUNK % seg == 0 and _XPOSE_CHUNK >= 3 * seg
    rows = 2 * (n_mem + seg)
    full = dm - _HALF

    vmem = pl.BlockSpec(memory_space=pltpu.VMEM)
    hbm = pl.BlockSpec(memory_space=pltpu.HBM)
    out_t = pl.pallas_call(
        functools.partial(_kernel, seg=seg, n_heads=n_heads, dh=dh),
        out_shape=jax.ShapeDtypeStruct((dm, seq), A_x.dtype),
        in_specs=[hbm, vmem] + [hbm] * 7,
        out_specs=hbm,
        scratch_shapes=[
            pltpu.VMEM((dm, seq), _BF16),
            pltpu.VMEM((seq, dm), _BF16),
            pltpu.VMEM((dm * n_heads, dh), _BF16),
            pltpu.VMEM((dm * n_heads, dh), _BF16),
            pltpu.VMEM((dm * n_heads, dh), _BF16),
            _packed_scratch(n_heads // 2 * dm, 6 * dh),
            pltpu.VMEM((n_heads, dm, dh), _BF16),
            _packed_scratch(n_heads * dh, full),
            pltpu.VMEM((dm, ffn), _BF16),
            pltpu.VMEM((dm, ffn), _BF16),
            _packed_scratch(full, ffn),
            _packed_scratch(full, ffn),
            pltpu.VMEM((dm, ffn), _BF16),
            _packed_scratch(ffn, full),
            _packed_scratch(n_heads // 2 * _LANES, 3 * dh),
            _packed_scratch(_LANES, ffn // 2),
            _packed_scratch(_LANES, ffn // 2),
            _packed_scratch(n_heads * dh // 2, _LANES),
            _packed_scratch(ffn // 2, _LANES),
            _packed_scratch(rows, n_heads * dh * 3 // 2),
            _packed_scratch(2 * seg, ffn * 3 // 2),
            pltpu.VMEM((rows, dm), _F32),
            pltpu.VMEM((2 * seg, dm), _F32),
            pltpu.VMEM((2 * seg, dm), _F32),
            pltpu.VMEM((2 * seg, dm - _HALF - _LANES), _F32),
            pltpu.VMEM((seq, dm), _BF16),
            pltpu.SemaphoreType.DMA((3 + 3 * _QKV_DMA_CHUNKS + 3 * _FFN_DMA_CHUNKS,)),
            pltpu.SemaphoreType.DMA((seq // _XPOSE_CHUNK + 1,)),
        ],
        compiler_params=pltpu.CompilerParams(vmem_limit_bytes=110 * 1024 * 1024),
    )(
        A_x.reshape(seq, dm).T,
        A_mem0.reshape(n_mem, dm),
        A_Wq.reshape(dm * n_heads, dh),
        A_Wk.reshape(dm * n_heads, dh),
        A_Wv.reshape(dm * n_heads, dh),
        A_Wo.transpose(0, 2, 1),
        B_w1,
        B_w3,
        B_w2.T,
    )
    return out_t.T.reshape(batch, seq, dm)
```

```python
import functools

import jax
import jax.numpy as jnp
import numpy as np
import jax.experimental.pallas as pl
import jax.experimental.pallas.tpu as pltpu

_EPS = 1e-5
_MASK_FILL = -1000000000.0
_QK_LAG = 1
_PV_LAG = 3
_FFN_CHUNK = 768
_XPOSE_CHUNK = 256
_FFN_DMA_CHUNKS = 3
_QKV_DMA_CHUNKS = 2
_WORD_TILE = 4

_LANES = 128
_HALF = _LANES // 2
_F32 = jnp.float32
_BF16 = jnp.bfloat16


def _layernorm(x):
    mean = jnp.mean(x, axis=-1, keepdims=True)
    cen = x - mean
    var = jnp.mean(cen * cen, axis=-1, keepdims=True)
    return cen * jax.lax.rsqrt(var + _EPS)


def _dot(a, b):
    return jnp.dot(a, b, preferred_element_type=_F32)


def _dot_nt(a, b):
    return jax.lax.dot_general(a, b, (((1,), (1,)), ((), ())), preferred_element_type=_F32)


class _Packed:
    def __init__(self, ref):
        self.ref = ref
        self.shape = (2 * ref.shape[0], ref.shape[1])

    def _index(self, idx):
        rows, cols = idx
        if isinstance(rows, slice):
            lo, hi, _ = rows.indices(self.shape[0])
            return slice(lo // 2, hi // 2), cols
        start, size = rows
        return pl.ds(pl.multiple_of(start // 2, size // 2), size // 2), cols

    def __getitem__(self, idx):
        return pltpu.bitcast(self.ref[self._index(idx)], _BF16)

    def __setitem__(self, idx, value):
        self.ref[self._index(idx)] = pltpu.bitcast(value, jnp.uint32)


def _packed_scratch(rows, cols):
    return pltpu.VMEM((rows // 2, cols), jnp.uint32)


def _split_lhs(x):
    full = x.shape[1] - _HALF
    first, rest = x[:, :_LANES], x[:, _LANES:full]
    tail = x[:, full:]
    lhs_b0 = jnp.concatenate([first[:, :_HALF], tail], axis=1)
    lhs_s = jnp.concatenate([tail, first[:, _HALF:]], axis=1)
    return jnp.concatenate([first, rest, lhs_b0, lhs_s], axis=1).astype(_BF16)


def _paired_dot(lhs, w_a, w_b, w_s):
    full = w_a.shape[0]
    shared = _dot(lhs[:, full + _LANES:], w_s)
    lhs_b = jnp.concatenate([lhs[:, full:full + _LANES], lhs[:, _LANES:full]], axis=1)
    return _dot(lhs[:, :full], w_a) + shared, _dot(lhs_b, w_b) + shared


def _pair_weights(a_mid, a_tail, b_mid, b_tail):
    a_new = (a_mid.astype(_F32) - b_mid.astype(_F32)).astype(_BF16)
    b_new = (b_tail.astype(_F32) - a_tail.astype(_F32)).astype(_BF16)
    return a_new, b_new, jnp.concatenate([a_tail, b_mid], axis=0)


def _pair_output_weights(ut, vt):
    full = ut.shape[0] - _HALF
    mid = slice(_HALF, _LANES)
    u_new, v_new, shared = _pair_weights(ut[mid], ut[full:], vt[mid], vt[full:])
    u = jnp.concatenate([ut[:_HALF], u_new, ut[_LANES:full]], axis=0)
    v = jnp.concatenate([vt[:_HALF], v_new, vt[_LANES:full]], axis=0)
    return u.T, v.T, shared.T


def _output_wide(lhs_ref, rows, w_ref, lo=0, hi=None):
    hi = w_ref.shape[0] if hi is None else hi
    return _dot(lhs_ref[rows, lo:hi], w_ref[lo:hi, _LANES:])


def _output_edges(lhs_ref, rows, w_ref, s_ref):
    half = s_ref.shape[0]
    shared = _dot(lhs_ref[rows, 2 * half:], s_ref[:, :])
    v0 = _dot(lhs_ref[rows, half:2 * half], w_ref[half:, 0:_LANES])
    u0 = _dot(lhs_ref[rows, 0:half], w_ref[0:half, 0:_LANES])
    is_low = jax.lax.broadcasted_iota(jnp.int32, u0.shape, 1) < _HALF
    return u0 + jnp.where(is_low, v0, shared), v0[:, _HALF:] + shared[:, :_HALF]


def _output_finish(lhs_ref, rows, w_ref, s_ref, wide):
    first, last = _output_edges(lhs_ref, rows, w_ref, s_ref)
    return jnp.concatenate([first, wide, last], axis=1)


def _output_dot(lhs_ref, rows, w_ref, s_ref):
    first, last = _output_edges(lhs_ref, rows, w_ref, s_ref)
    return jnp.concatenate([first, _output_wide(lhs_ref, rows, w_ref), last], axis=1)


def _mask_tables(n_streams, n_mem, seg):
    tok0 = n_streams * n_mem
    rows = tok0 + n_streams * seg

    def split(axis):
        idx = jax.lax.broadcasted_iota(jnp.int32, (rows, rows), axis)
        is_mem = idx < tok0
        stream = jnp.where(is_mem, idx // n_mem, (idx - tok0) // seg)
        pos = jnp.where(is_mem, idx % n_mem, n_mem + (idx - tok0) % seg)
        return stream, pos

    q_stream, q_pos = split(0)
    k_stream, k_pos = split(1)
    same = q_stream == k_stream
    visible = same & ((q_pos < n_mem) | (q_pos >= k_pos))
    fill = jnp.where(same, _MASK_FILL, -jnp.inf).astype(_F32)
    return visible, fill


def _kernel(xt_hbm, mem0_ref, wq_hbm, wk_hbm, wv_hbm, wot_hbm, w1_hbm, w3_hbm, w2t_hbm,
            out_hbm,
            xt_ref, x_ref, rq_ref, rk_ref, rv_ref, wqkv_ref, wot_ref, wo_ref,
            r1_ref, r3_ref, w1_ref, w3_ref, w2t_ref, w2_ref, sqkv_ref, s1_ref, s3_ref, so_ref, s2_ref,
            o_ref, hid_ref, a_ref, xa_ref, x1_ref, wide_ref, y_ref, in_sems, out_sems,
            *, seg, n_heads, dh):
    seq, dm = x_ref.shape
    n_mem = mem0_ref.shape[0]
    n_seg = seq // seg
    ffn = w1_ref.shape[1]
    wqkv_ref, wo_ref, w1_ref, w3_ref, w2_ref = map(
        _Packed, (wqkv_ref, wo_ref, w1_ref, w3_ref, w2_ref))
    sqkv_ref, s1_ref, s3_ref, so_ref, s2_ref = map(
        _Packed, (sqkv_ref, s1_ref, s3_ref, so_ref, s2_ref))
    o_ref, hid_ref = _Packed(o_ref), _Packed(hid_ref)
    scale = dh ** -0.5
    n_grp = n_heads // 2
    tok0 = 2 * n_mem
    full = dm - _HALF
    mid = slice(_HALF, _LANES)
    fc = _FFN_CHUNK
    xc = _XPOSE_CHUNK
    wc = ffn // _FFN_DMA_CHUNKS

    def cols(ref, start, size):
        return ref.at[:, start:start + size]

    def rows_of(ref, start, size):
        return ref.at[start:start + size, :]

    raw_rows = dm * n_heads // _QKV_DMA_CHUNKS
    transfers = [("x_head", cols(xt_hbm, 0, xc), cols(xt_ref, 0, xc))]
    for name, src, dst in (("wq", wq_hbm, rq_ref), ("wk", wk_hbm, rk_ref), ("wv", wv_hbm, rv_ref)):
        for c in range(_QKV_DMA_CHUNKS):
            transfers.append(((name, c), rows_of(src, c * raw_rows, raw_rows),
                              rows_of(dst, c * raw_rows, raw_rows)))
    transfers.append(("wo", wot_hbm, wot_ref))
    for c in range(0, ffn, wc):
        transfers.append((("w1", c), cols(w1_hbm, c, wc), cols(r1_ref, c, wc)))
        transfers.append((("w3", c), cols(w3_hbm, c, wc), cols(r3_ref, c, wc)))
    for c in range(0, ffn, wc):
        transfers.append((("w2", c), cols(w2t_hbm, c, wc), cols(w2t_ref, c, wc)))
    transfers.append(("x_tail", cols(xt_hbm, xc, seq - xc), cols(xt_ref, xc, seq - xc)))
    copies = {name: pltpu.make_async_copy(src, dst, in_sems.at[n])
              for n, (name, src, dst) in enumerate(transfers)}

    def arrive(name):
        copies[name].wait()

    def project(h, grp):
        rows = slice(grp * dm, grp * dm + full)
        both = _paired_dot(h, wqkv_ref[rows, 0:3 * dh], wqkv_ref[rows, 3 * dh:],
                           sqkv_ref[grp * _LANES:(grp + 1) * _LANES, :])
        return [[qkv[:, m * dh:(m + 1) * dh].astype(_BF16) for m in range(3)] for qkv in both]

    def probabilities(qkv, visible, fill):
        probs = []
        for q, k, _ in qkv:
            s = jnp.where(visible, _dot_nt(q, k) * scale, fill)
            p = jnp.exp(s - jnp.max(s, axis=-1, keepdims=True))
            probs.append((p * (1.0 / jnp.sum(p, axis=-1, keepdims=True))).astype(_BF16))
        return probs

    def heads(h, n_streams, fillers=()):
        rows = h.shape[0]
        visible, fill = _mask_tables(n_streams, n_mem, seg)
        qkv, probs = {}, {}
        for t in range(n_grp + _PV_LAG):
            if t < n_grp:
                qkv[t] = project(h, t)
            elif t - n_grp < len(fillers):
                fillers[t - n_grp]()
            if 0 <= t - _QK_LAG < n_grp:
                probs[t - _QK_LAG] = probabilities(qkv[t - _QK_LAG], visible, fill)
            if 0 <= t - _PV_LAG:
                grp = t - _PV_LAG
                outs = [_dot(p, v) for p, (_, _, v) in zip(probs.pop(grp), qkv.pop(grp))]
                for part, out in enumerate(outs + [outs[0] + outs[1]]):
                    col = (part * n_grp + grp) * dh
                    o_ref[0:rows, col:col + dh] = out.astype(_BF16)

    def attend(h, n_streams):
        rows, half, wide = slice(0, h.shape[0]), n_grp * dh, []
        cut_u, cut_v = (n_grp - _PV_LAG) * dh, half + (n_grp - _PV_LAG + 1) * dh

        def part(lo, hi):
            return lambda: wide.append(_output_wide(o_ref, rows, wo_ref, lo, hi))

        heads(h, n_streams, (part(0, cut_u), part(half, cut_v)))
        first, last = _output_edges(o_ref, rows, wo_ref, so_ref)
        part(cut_u, half)()
        part(cut_v, 2 * half)()
        wide = (wide[0] + wide[1]) + (wide[2] + wide[3])
        return jnp.concatenate([first, wide, last], axis=1)

    def pair_gate_up(lo, hi):
        for raw, w_ref, s_ref in ((r1_ref, w1_ref, s1_ref), (r3_ref, w3_ref, s3_ref)):
            w_ref[0:_HALF, lo:hi] = raw[0:_HALF, lo:hi]
            w_ref[_LANES:, lo:hi] = raw[_LANES:full, lo:hi]
            for c in range(lo, hi, fc):
                ca, cb = slice(c, c + fc // 2), slice(c + fc // 2, c + fc)
                w_ref[mid, ca], w_ref[mid, cb], s_ref[:, c // 2:(c + fc) // 2] = _pair_weights(
                    raw[mid, ca], raw[full:, ca], raw[mid, cb], raw[full:, cb])

    def gate_up(f_in, lo=0, hi=ffn):
        for c in range(lo, hi, fc):
            ca, cb = slice(c, c + fc // 2), slice(c + fc // 2, c + fc)
            cs = slice(c // 2, (c + fc) // 2)
            gates = _paired_dot(f_in, w1_ref[0:full, ca], w1_ref[0:full, cb], s1_ref[:, cs])
            ups = _paired_dot(f_in, w3_ref[0:full, ca], w3_ref[0:full, cb], s3_ref[:, cs])
            hids = [gate * jax.nn.sigmoid(gate) * up for gate, up in zip(gates, ups)]
            for part, hid in enumerate(hids + [hids[0] + hids[1]]):
                col = (part * ffn + c) // 2
                hid_ref[0:hid.shape[0], col:col + fc // 2] = hid.astype(_BF16)

    def stage_down(lo, hi):
        for c in range(lo, hi, fc):
            rows_u = slice(c // 2, (c + fc) // 2)
            rows_v = slice((ffn + c) // 2, (ffn + c + fc) // 2)
            w2_ref[rows_u, :], w2_ref[rows_v, :], s2_ref[rows_u, :] = _pair_output_weights(
                w2t_ref[:, c:c + fc // 2], w2t_ref[:, c + fc // 2:c + fc])

    def single_stream_rows(mem, x):
        return _split_lhs(jnp.concatenate([mem, _layernorm(x)], axis=0))

    def write_back(t, size):
        xt_ref[:, t:t + size] = y_ref[t:t + size, :].T
        copy = pltpu.make_async_copy(
            cols(xt_ref, t, size), cols(out_hbm, t, size), out_sems.at[pl.cdiv(t, xc)])
        copy.start()
        return copy

    for copy in copies.values():
        copy.start()
    arrive("x_head")
    x_ref[0:xc, :] = xt_ref[:, 0:xc].T

    pairs = n_heads // 2
    d_chunk = dm // _QKV_DMA_CHUNKS
    for m, (name, raw_ref) in enumerate((("wq", rq_ref), ("wk", rk_ref), ("wv", rv_ref))):
        words = raw_ref.bitcast(jnp.uint32)
        for c in range(_QKV_DMA_CHUNKS):
            arrive((name, c))

            def regroup(quad, carry, m=m, c=c, words=words):
                start = pl.multiple_of(c * d_chunk * pairs + quad * _WORD_TILE, _WORD_TILE)
                view = words.at[pl.ds(start, d_chunk * pairs - pairs + _WORD_TILE), :]
                for r in range(_WORD_TILE):
                    even_d = view[pl.ds(r, d_chunk // 2, stride=n_heads), :]
                    odd_d = view[pl.ds(r + pairs, d_chunk // 2, stride=n_heads), :]
                    lo = (even_d & jnp.uint32(0xFFFF)) | (odd_d << 16)
                    hi = (even_d >> 16) | (odd_d & jnp.uint32(0xFFFF0000))
                    row = (quad * _WORD_TILE + r) * (dm // 2) + c * (d_chunk // 2)
                    for half, val in enumerate((lo, hi)):
                        col = (half * 3 + m) * dh
                        wqkv_ref.ref[pl.ds(pl.multiple_of(row, 8), d_chunk // 2), col:col + dh] = val
                return carry

            jax.lax.fori_loop(0, pairs // _WORD_TILE, regroup, 0)

    def pair_heads(grp, carry):
        ca, cb = slice(0, 3 * dh), slice(3 * dh, 6 * dh)
        mid_rows, tail_rows = (grp * dm + _HALF, _HALF), (grp * dm + full, _HALF)
        (wqkv_ref[mid_rows, ca], wqkv_ref[mid_rows, cb],
         sqkv_ref[(grp * _LANES, _LANES), :]) = _pair_weights(
             wqkv_ref[mid_rows, ca], wqkv_ref[tail_rows, ca],
             wqkv_ref[mid_rows, cb], wqkv_ref[tail_rows, cb])
        return carry

    jax.lax.fori_loop(0, n_grp, pair_heads, 0)

    mem0 = mem0_ref[...].astype(_F32)
    a_ref[0:n_mem, :] = mem0

    def first_segments(s, carry):
        x_s = x_ref[pl.ds(pl.multiple_of(s * seg, seg), seg), :].astype(_F32)
        heads(single_stream_rows(a_ref[0:n_mem, :], x_s), 1)

        @pl.when(s == 0)
        def _():
            arrive("wo")

            def stage_wo(grp, carry):
                rows_u, rows_v = (grp * dh, dh), ((n_grp + grp) * dh, dh)
                wo_ref[rows_u, :], wo_ref[rows_v, :], so_ref[rows_u, :] = _pair_output_weights(
                    wot_ref[2 * grp], wot_ref[2 * grp + 1])
                return carry

            jax.lax.fori_loop(0, n_grp, stage_wo, 0, unroll=2)

        a = _output_dot(o_ref, slice(0, n_mem + seg), wo_ref, so_ref)
        a_ref[0:n_mem, :] = a[:n_mem]
        a_ref[pl.ds(pl.multiple_of(tok0 + (1 - s) * seg, n_mem), seg), :] = a[n_mem:]
        return carry

    jax.lax.fori_loop(0, 2, first_segments, 0)
    a_ref[n_mem:tok0, :] = mem0
    x1 = jnp.concatenate([x_ref[seg:2 * seg, :], x_ref[0:seg, :]], axis=0).astype(_F32)
    x1 = x1 + a_ref[tok0:, :]
    x1_ref[...] = x1
    f_in = _split_lhs(_layernorm(x1))
    for c in range(0, ffn, wc):
        arrive(("w1", c))
        arrive(("w3", c))
        pair_gate_up(c, c + wc)
        gate_up(f_in, c, c + wc)
    both = slice(0, 2 * seg)
    wide = None
    for c in range(0, ffn, wc):
        arrive(("w2", c))
        stage_down(c, c + wc)
        for lo in (c // 2, (ffn + c) // 2):
            part = _output_wide(hid_ref, both, w2_ref, lo, lo + wc // 2)
            wide = part if wide is None else wide + part
    wide_ref[...] = wide

    def feed_forward(out_row):
        y = x1_ref[...] + _output_finish(hid_ref, both, w2_ref, s2_ref, wide_ref[...])
        y_ref[pl.ds(out_row, seg), :] = y[seg:].astype(y_ref.dtype)
        x1 = xa_ref[...] + a_ref[tok0:, :]
        x1_ref[...] = x1
        gate_up(_split_lhs(_layernorm(x1)))
        return y[:seg]

    def attend_both(x_row, x2):
        xa = jnp.concatenate([x_ref[pl.ds(x_row, seg), :].astype(_F32), x2], axis=0)
        xa_ref[...] = xa
        a_ref[...] = attend(
            _split_lhs(jnp.concatenate([a_ref[0:tok0, :], _layernorm(xa)], axis=0)), 2)

    def step(i, carry):
        @pl.when(i == xc // seg - 1)
        def _():
            arrive("x_tail")
            for t in range(xc, seq, xc):
                x_ref[t:t + xc, :] = xt_ref[:, t:t + xc].T

        x2 = feed_forward(pl.multiple_of(jnp.maximum(i - 3, 0) * seg, seg))
        wide_ref[...] = _output_wide(hid_ref, both, w2_ref)
        attend_both(pl.multiple_of((i + 1) * seg, seg), x2)
        return carry

    attend_both(2 * seg, x1_ref[seg:, :] + _output_finish(
        hid_ref, slice(seg, 2 * seg), w2_ref, s2_ref, wide_ref[seg:, :]))
    jax.lax.fori_loop(2, n_seg - 1, step, 0)

    x_s0 = feed_forward(seq - 4 * seg)
    a = attend(single_stream_rows(a_ref[n_mem:tok0, :], x_s0), 1)
    y = x1_ref[...] + _output_dot(hid_ref, both, w2_ref, s2_ref)
    y_ref[seq - 3 * seg:seq - 2 * seg, :] = y[seg:].astype(y_ref.dtype)
    x1_s0 = x_s0 + a[n_mem:]
    last = seq - _LANES
    writes = [write_back(t, min(xc, last - t)) for t in range(0, last, xc)]
    a = attend(single_stream_rows(a[:n_mem], y[:seg]), 1)
    x1 = jnp.concatenate([x1_s0, y[:seg] + a[n_mem:]], axis=0)
    gate_up(_split_lhs(_layernorm(x1)))
    y_ref[seq - 2 * seg:, :] = (x1 + _output_dot(hid_ref, both, w2_ref, s2_ref)).astype(y_ref.dtype)
    writes.append(write_back(last, _LANES))
    for copy in writes:
        copy.wait()


@functools.partial(jax.jit, static_argnames=("A_seg_len",))
def pallas_interleave_layers__memory_aug_recurrent_mem_tr__glu_gated_swiglu__prompt_kernel(
    A_x: jax.Array,
    A_mem0: jax.Array,
    A_Wq: jax.Array,
    A_Wk: jax.Array,
    A_Wv: jax.Array,
    A_Wo: jax.Array,
    A_seg_len: int,
    B_x: jax.Array,
    B_w1: jax.Array,
    B_w3: jax.Array,
    B_w2: jax.Array,
):
    del B_x
    batch, seq, dm = A_x.shape
    _, n_heads, dh = A_Wq.shape
    n_mem = A_mem0.shape[1]
    ffn = B_w1.shape[1]
    seg = int(A_seg_len)
    assert batch == 1 and seq % _XPOSE_CHUNK == 0 and _XPOSE_CHUNK % seg == 0 and _XPOSE_CHUNK >= 3 * seg
    rows = 2 * (n_mem + seg)
    full = dm - _HALF

    vmem = pl.BlockSpec(memory_space=pltpu.VMEM)
    hbm = pl.BlockSpec(memory_space=pltpu.HBM)
    out_t = pl.pallas_call(
        functools.partial(_kernel, seg=seg, n_heads=n_heads, dh=dh),
        out_shape=jax.ShapeDtypeStruct((dm, seq), A_x.dtype),
        in_specs=[hbm, vmem] + [hbm] * 7,
        out_specs=hbm,
        scratch_shapes=[
            pltpu.VMEM((dm, seq), _BF16),
            pltpu.VMEM((seq, dm), _BF16),
            pltpu.VMEM((dm * n_heads, dh), _BF16),
            pltpu.VMEM((dm * n_heads, dh), _BF16),
            pltpu.VMEM((dm * n_heads, dh), _BF16),
            _packed_scratch(n_heads // 2 * dm, 6 * dh),
            pltpu.VMEM((n_heads, dm, dh), _BF16),
            _packed_scratch(n_heads * dh, full),
            pltpu.VMEM((dm, ffn), _BF16),
            pltpu.VMEM((dm, ffn), _BF16),
            _packed_scratch(full, ffn),
            _packed_scratch(full, ffn),
            pltpu.VMEM((dm, ffn), _BF16),
            _packed_scratch(ffn, full),
            _packed_scratch(n_heads // 2 * _LANES, 3 * dh),
            _packed_scratch(_LANES, ffn // 2),
            _packed_scratch(_LANES, ffn // 2),
            _packed_scratch(n_heads * dh // 2, _LANES),
            _packed_scratch(ffn // 2, _LANES),
            _packed_scratch(rows, n_heads * dh * 3 // 2),
            _packed_scratch(2 * seg, ffn * 3 // 2),
            pltpu.VMEM((rows, dm), _F32),
            pltpu.VMEM((2 * seg, dm), _F32),
            pltpu.VMEM((2 * seg, dm), _F32),
            pltpu.VMEM((2 * seg, dm - _HALF - _LANES), _F32),
            pltpu.VMEM((seq, dm), _BF16),
            pltpu.SemaphoreType.DMA((3 + 3 * _QKV_DMA_CHUNKS + 3 * _FFN_DMA_CHUNKS,)),
            pltpu.SemaphoreType.DMA((seq // _XPOSE_CHUNK + 1,)),
        ],
        compiler_params=pltpu.CompilerParams(vmem_limit_bytes=110 * 1024 * 1024),
    )(
        A_x.reshape(seq, dm).T,
        A_mem0.reshape(n_mem, dm),
        A_Wq.reshape(dm * n_heads, dh),
        A_Wk.reshape(dm * n_heads, dh),
        A_Wv.reshape(dm * n_heads, dh),
        A_Wo.transpose(0, 2, 1),
        B_w1,
        B_w3,
        B_w2.T,
    )
    return out_t.T.reshape(batch, seq, dm)
```

```python
import functools

import jax
import jax.numpy as jnp
import numpy as np
import jax.experimental.pallas as pl
import jax.experimental.pallas.tpu as pltpu

_EPS = 1e-5
_MASK_FILL = -1000000000.0
_QK_LAG = 1
_PV_LAG = 3
_X_TAIL_GROUP = 12
_FFN_CHUNK = 768
_XPOSE_CHUNK = 256
_FFN_DMA_CHUNKS = 3
_QKV_DMA_CHUNKS = 2
_WORD_TILE = 4

_LANES = 128
_HALF = _LANES // 2
_F32 = jnp.float32
_BF16 = jnp.bfloat16


def _layernorm(x):
    mean = jnp.mean(x, axis=-1, keepdims=True)
    cen = x - mean
    var = jnp.mean(cen * cen, axis=-1, keepdims=True)
    return cen * jax.lax.rsqrt(var + _EPS)


def _dot(a, b):
    return jnp.dot(a, b, preferred_element_type=_F32)


def _dot_nt(a, b):
    return jax.lax.dot_general(a, b, (((1,), (1,)), ((), ())), preferred_element_type=_F32)


class _Packed:
    def __init__(self, ref):
        self.ref = ref
        self.shape = (2 * ref.shape[0], ref.shape[1])

    def _index(self, idx):
        rows, cols = idx
        if isinstance(rows, slice):
            lo, hi, _ = rows.indices(self.shape[0])
            return slice(lo // 2, hi // 2), cols
        start, size = rows
        return pl.ds(pl.multiple_of(start // 2, size // 2), size // 2), cols

    def __getitem__(self, idx):
        return pltpu.bitcast(self.ref[self._index(idx)], _BF16)

    def __setitem__(self, idx, value):
        self.ref[self._index(idx)] = pltpu.bitcast(value, jnp.uint32)


def _packed_scratch(rows, cols):
    return pltpu.VMEM((rows // 2, cols), jnp.uint32)


def _split_lhs(x):
    full = x.shape[1] - _HALF
    first, rest = x[:, :_LANES], x[:, _LANES:full]
    tail = x[:, full:]
    lhs_b0 = jnp.concatenate([first[:, :_HALF], tail], axis=1)
    lhs_s = jnp.concatenate([tail, first[:, _HALF:]], axis=1)
    return jnp.concatenate([first, rest, lhs_b0, lhs_s], axis=1).astype(_BF16)


def _paired_dot(lhs, w_a, w_b, w_s):
    full = w_a.shape[0]
    shared = _dot(lhs[:, full + _LANES:], w_s)
    lhs_b = jnp.concatenate([lhs[:, full:full + _LANES], lhs[:, _LANES:full]], axis=1)
    return _dot(lhs[:, :full], w_a) + shared, _dot(lhs_b, w_b) + shared


def _pair_weights(a_mid, a_tail, b_mid, b_tail):
    a_new = (a_mid.astype(_F32) - b_mid.astype(_F32)).astype(_BF16)
    b_new = (b_tail.astype(_F32) - a_tail.astype(_F32)).astype(_BF16)
    return a_new, b_new, jnp.concatenate([a_tail, b_mid], axis=0)


def _pair_output_weights(ut, vt):
    full = ut.shape[0] - _HALF
    mid = slice(_HALF, _LANES)
    u_new, v_new, shared = _pair_weights(ut[mid], ut[full:], vt[mid], vt[full:])
    u = jnp.concatenate([ut[:_HALF], u_new, ut[_LANES:full]], axis=0)
    v = jnp.concatenate([vt[:_HALF], v_new, vt[_LANES:full]], axis=0)
    return u.T, v.T, shared.T


def _output_wide(lhs_ref, rows, w_ref, lo=0, hi=None):
    hi = w_ref.shape[0] if hi is None else hi
    return _dot(lhs_ref[rows, lo:hi], w_ref[lo:hi, _LANES:])


def _output_edges(lhs_ref, rows, w_ref, s_ref):
    half = s_ref.shape[0]
    shared = _dot(lhs_ref[rows, 2 * half:], s_ref[:, :])
    v0 = _dot(lhs_ref[rows, half:2 * half], w_ref[half:, 0:_LANES])
    u0 = _dot(lhs_ref[rows, 0:half], w_ref[0:half, 0:_LANES])
    is_low = jax.lax.broadcasted_iota(jnp.int32, u0.shape, 1) < _HALF
    return u0 + jnp.where(is_low, v0, shared), v0[:, _HALF:] + shared[:, :_HALF]


def _output_finish(lhs_ref, rows, w_ref, s_ref, wide):
    first, last = _output_edges(lhs_ref, rows, w_ref, s_ref)
    return jnp.concatenate([first, wide, last], axis=1)


def _output_dot(lhs_ref, rows, w_ref, s_ref):
    first, last = _output_edges(lhs_ref, rows, w_ref, s_ref)
    return jnp.concatenate([first, _output_wide(lhs_ref, rows, w_ref), last], axis=1)


def _mask_tables(n_streams, n_mem, seg):
    tok0 = n_streams * n_mem
    rows = tok0 + n_streams * seg

    def split(axis):
        idx = jax.lax.broadcasted_iota(jnp.int32, (rows, rows), axis)
        is_mem = idx < tok0
        stream = jnp.where(is_mem, idx // n_mem, (idx - tok0) // seg)
        pos = jnp.where(is_mem, idx % n_mem, n_mem + (idx - tok0) % seg)
        return stream, pos

    q_stream, q_pos = split(0)
    k_stream, k_pos = split(1)
    same = q_stream == k_stream
    visible = same & ((q_pos < n_mem) | (q_pos >= k_pos))
    fill = jnp.where(same, _MASK_FILL, -jnp.inf).astype(_F32)
    return visible, fill


def _kernel(xt_hbm, mem0_ref, wq_hbm, wk_hbm, wv_hbm, wot_hbm, w1_hbm, w3_hbm, w2t_hbm,
            out_hbm,
            xt_ref, x_ref, rq_ref, rk_ref, rv_ref, wqkv_ref, wot_ref, wo_ref,
            r1_ref, r3_ref, w1_ref, w3_ref, w2t_ref, w2_ref, sqkv_ref, s1_ref, s3_ref, so_ref, s2_ref,
            o_ref, hid_ref, early_ref, a_ref, xa_ref, x1_ref, wide_ref, y_ref, in_sems, out_sems,
            *, seg, n_heads, dh):
    seq, dm = x_ref.shape
    n_mem = mem0_ref.shape[0]
    n_seg = seq // seg
    ffn = w1_ref.shape[1]
    wqkv_ref, wo_ref, w1_ref, w3_ref, w2_ref = map(
        _Packed, (wqkv_ref, wo_ref, w1_ref, w3_ref, w2_ref))
    sqkv_ref, s1_ref, s3_ref, so_ref, s2_ref = map(
        _Packed, (sqkv_ref, s1_ref, s3_ref, so_ref, s2_ref))
    o_ref, hid_ref, early_ref = map(_Packed, (o_ref, hid_ref, early_ref))
    scale = dh ** -0.5
    n_grp = n_heads // 2
    tok0 = 2 * n_mem
    full = dm - _HALF
    mid = slice(_HALF, _LANES)
    fc = _FFN_CHUNK
    xc = _XPOSE_CHUNK
    wc = ffn // _FFN_DMA_CHUNKS

    def cols(ref, start, size):
        return ref.at[:, start:start + size]

    def rows_of(ref, start, size):
        return ref.at[start:start + size, :]

    raw_rows = dm * n_heads // _QKV_DMA_CHUNKS
    transfers = [("x_head", cols(xt_hbm, 0, xc), cols(xt_ref, 0, xc))]
    for name, src, dst in (("wq", wq_hbm, rq_ref), ("wk", wk_hbm, rk_ref), ("wv", wv_hbm, rv_ref)):
        for c in range(_QKV_DMA_CHUNKS):
            transfers.append(((name, c), rows_of(src, c * raw_rows, raw_rows),
                              rows_of(dst, c * raw_rows, raw_rows)))
    transfers.append(("wo", wot_hbm, wot_ref))
    for c in range(0, ffn, wc):
        transfers.append((("w1", c), cols(w1_hbm, c, wc), cols(r1_ref, c, wc)))
        transfers.append((("w3", c), cols(w3_hbm, c, wc), cols(r3_ref, c, wc)))
    for c in range(0, ffn, wc):
        transfers.append((("w2", c), cols(w2t_hbm, c, wc), cols(w2t_ref, c, wc)))
    transfers.append(("x_tail", cols(xt_hbm, xc, seq - xc), cols(xt_ref, xc, seq - xc)))
    copies = {name: pltpu.make_async_copy(src, dst, in_sems.at[n])
              for n, (name, src, dst) in enumerate(transfers)}

    def arrive(name):
        copies[name].wait()

    def project(h, grp):
        rows = slice(grp * dm, grp * dm + full)
        both = _paired_dot(h, wqkv_ref[rows, 0:3 * dh], wqkv_ref[rows, 3 * dh:],
                           sqkv_ref[grp * _LANES:(grp + 1) * _LANES, :])
        return [[qkv[:, m * dh:(m + 1) * dh].astype(_BF16) for m in range(3)] for qkv in both]

    def probabilities(qkv, visible, fill):
        probs = []
        for q, k, _ in qkv:
            s = jnp.where(visible, _dot_nt(q, k) * scale, fill)
            p = jnp.exp(s - jnp.max(s, axis=-1, keepdims=True))
            probs.append((p * (1.0 / jnp.sum(p, axis=-1, keepdims=True))).astype(_BF16))
        return probs

    def heads(project_group, n_streams, fillers=()):
        rows = n_streams * (n_mem + seg)
        visible, fill = _mask_tables(n_streams, n_mem, seg)
        qkv, probs = {}, {}
        for t in range(n_grp + _PV_LAG):
            if t < n_grp:
                qkv[t] = project_group(t)
            elif t - n_grp < len(fillers):
                fillers[t - n_grp]()
            if 0 <= t - _QK_LAG < n_grp:
                probs[t - _QK_LAG] = probabilities(qkv[t - _QK_LAG], visible, fill)
            if 0 <= t - _PV_LAG:
                grp = t - _PV_LAG
                outs = [_dot(p, v) for p, (_, _, v) in zip(probs.pop(grp), qkv.pop(grp))]
                for part, out in enumerate(outs + [outs[0] + outs[1]]):
                    col = (part * n_grp + grp) * dh
                    o_ref[0:rows, col:col + dh] = out.astype(_BF16)

    def attend(project_group, n_streams):
        rows, half, wide = slice(0, n_streams * (n_mem + seg)), n_grp * dh, []
        cut_u, cut_v = (n_grp - _PV_LAG) * dh, half + (n_grp - _PV_LAG + 1) * dh

        def part(lo, hi):
            return lambda: wide.append(_output_wide(o_ref, rows, wo_ref, lo, hi))

        heads(project_group, n_streams, (part(0, cut_u), part(half, cut_v)))
        first, last = _output_edges(o_ref, rows, wo_ref, so_ref)
        part(cut_u, half)()
        part(cut_v, 2 * half)()
        wide = (wide[0] + wide[1]) + (wide[2] + wide[3])
        return jnp.concatenate([first, wide, last], axis=1)

    def pair_gate_up(lo, hi):
        for raw, w_ref, s_ref in ((r1_ref, w1_ref, s1_ref), (r3_ref, w3_ref, s3_ref)):
            w_ref[0:_HALF, lo:hi] = raw[0:_HALF, lo:hi]
            w_ref[_LANES:, lo:hi] = raw[_LANES:full, lo:hi]
            for c in range(lo, hi, fc):
                ca, cb = slice(c, c + fc // 2), slice(c + fc // 2, c + fc)
                w_ref[mid, ca], w_ref[mid, cb], s_ref[:, c // 2:(c + fc) // 2] = _pair_weights(
                    raw[mid, ca], raw[full:, ca], raw[mid, cb], raw[full:, cb])

    def gate_up(f_in, lo=0, hi=ffn):
        for c in range(lo, hi, fc):
            ca, cb = slice(c, c + fc // 2), slice(c + fc // 2, c + fc)
            cs = slice(c // 2, (c + fc) // 2)
            gates = _paired_dot(f_in, w1_ref[0:full, ca], w1_ref[0:full, cb], s1_ref[:, cs])
            ups = _paired_dot(f_in, w3_ref[0:full, ca], w3_ref[0:full, cb], s3_ref[:, cs])
            hids = [gate * jax.nn.sigmoid(gate) * up for gate, up in zip(gates, ups)]
            for part, hid in enumerate(hids + [hids[0] + hids[1]]):
                col = (part * ffn + c) // 2
                hid_ref[0:hid.shape[0], col:col + fc // 2] = hid.astype(_BF16)

    def stage_down(lo, hi):
        for c in range(lo, hi, fc):
            rows_u = slice(c // 2, (c + fc) // 2)
            rows_v = slice((ffn + c) // 2, (ffn + c + fc) // 2)
            w2_ref[rows_u, :], w2_ref[rows_v, :], s2_ref[rows_u, :] = _pair_output_weights(
                w2t_ref[:, c:c + fc // 2], w2t_ref[:, c + fc // 2:c + fc])

    def projector(mem, x):
        return functools.partial(project, _split_lhs(jnp.concatenate([mem, _layernorm(x)], axis=0)))

    def write_back(t, size):
        xt_ref[:, t:t + size] = y_ref[t:t + size, :].T
        copy = pltpu.make_async_copy(
            cols(xt_ref, t, size), cols(out_hbm, t, size), out_sems.at[pl.cdiv(t, xc)])
        copy.start()
        return copy

    for copy in copies.values():
        copy.start()
    arrive("x_head")
    x_ref[0:xc, :] = xt_ref[:, 0:xc].T

    pairs = n_heads // 2
    d_chunk = dm // _QKV_DMA_CHUNKS
    for m, (name, raw_ref) in enumerate((("wq", rq_ref), ("wk", rk_ref), ("wv", rv_ref))):
        words = raw_ref.bitcast(jnp.uint32)
        for c in range(_QKV_DMA_CHUNKS):
            arrive((name, c))

            def regroup(quad, carry, m=m, c=c, words=words):
                start = pl.multiple_of(c * d_chunk * pairs + quad * _WORD_TILE, _WORD_TILE)
                view = words.at[pl.ds(start, d_chunk * pairs - pairs + _WORD_TILE), :]
                for r in range(_WORD_TILE):
                    even_d = view[pl.ds(r, d_chunk // 2, stride=n_heads), :]
                    odd_d = view[pl.ds(r + pairs, d_chunk // 2, stride=n_heads), :]
                    lo = (even_d & jnp.uint32(0xFFFF)) | (odd_d << 16)
                    hi = (even_d >> 16) | (odd_d & jnp.uint32(0xFFFF0000))
                    row = (quad * _WORD_TILE + r) * (dm // 2) + c * (d_chunk // 2)
                    for half, val in enumerate((lo, hi)):
                        col = (half * 3 + m) * dh
                        wqkv_ref.ref[pl.ds(pl.multiple_of(row, 8), d_chunk // 2), col:col + dh] = val
                return carry

            jax.lax.fori_loop(0, pairs // _WORD_TILE, regroup, 0)

    def pair_heads(grp, carry):
        ca, cb = slice(0, 3 * dh), slice(3 * dh, 6 * dh)
        mid_rows, tail_rows = (grp * dm + _HALF, _HALF), (grp * dm + full, _HALF)
        (wqkv_ref[mid_rows, ca], wqkv_ref[mid_rows, cb],
         sqkv_ref[(grp * _LANES, _LANES), :]) = _pair_weights(
             wqkv_ref[mid_rows, ca], wqkv_ref[tail_rows, ca],
             wqkv_ref[mid_rows, cb], wqkv_ref[tail_rows, cb])
        return carry

    jax.lax.fori_loop(0, n_grp, pair_heads, 0)

    mem0 = mem0_ref[...].astype(_F32)
    a_ref[0:n_mem, :] = mem0

    def first_segments(s, carry):
        x_s = x_ref[pl.ds(pl.multiple_of(s * seg, seg), seg), :].astype(_F32)
        heads(projector(a_ref[0:n_mem, :], x_s), 1)

        @pl.when(s == 0)
        def _():
            arrive("wo")

            def stage_wo(grp, carry):
                rows_u, rows_v = (grp * dh, dh), ((n_grp + grp) * dh, dh)
                wo_ref[rows_u, :], wo_ref[rows_v, :], so_ref[rows_u, :] = _pair_output_weights(
                    wot_ref[2 * grp], wot_ref[2 * grp + 1])
                return carry

            jax.lax.fori_loop(0, n_grp, stage_wo, 0, unroll=2)

        a = _output_dot(o_ref, slice(0, n_mem + seg), wo_ref, so_ref)
        a_ref[0:n_mem, :] = a[:n_mem]
        a_ref[pl.ds(pl.multiple_of(tok0 + (1 - s) * seg, n_mem), seg), :] = a[n_mem:]
        return carry

    jax.lax.fori_loop(0, 2, first_segments, 0)
    a_ref[n_mem:tok0, :] = mem0
    x1 = jnp.concatenate([x_ref[seg:2 * seg, :], x_ref[0:seg, :]], axis=0).astype(_F32)
    x1 = x1 + a_ref[tok0:, :]
    x1_ref[...] = x1
    f_in = _split_lhs(_layernorm(x1))
    for c in range(0, ffn, wc):
        arrive(("w1", c))
        arrive(("w3", c))
        pair_gate_up(c, c + wc)
        gate_up(f_in, c, c + wc)
    both = slice(0, 2 * seg)
    x_s2 = x_ref[2 * seg:3 * seg, :].astype(_F32)
    project_early = projector(a_ref[0:tok0, :], x_s2)
    wide = None
    for n, c in enumerate(range(0, ffn, wc)):
        for grp in range(n * n_grp // _FFN_DMA_CHUNKS, (n + 1) * n_grp // _FFN_DMA_CHUNKS):
            early = [m for qkv in project_early(grp) for m in qkv]
            early_ref[:, grp * 6 * dh:(grp + 1) * 6 * dh] = jnp.concatenate(early, axis=1)
        arrive(("w2", c))
        stage_down(c, c + wc)
        for lo in (c // 2, (ffn + c) // 2):
            part = _output_wide(hid_ref, both, w2_ref, lo, lo + wc // 2)
            wide = part if wide is None else wide + part
    wide_ref[...] = wide
    x2_s0 = x1_ref[seg:, :] + _output_finish(
        hid_ref, slice(seg, 2 * seg), w2_ref, s2_ref, wide[seg:])
    xa_ref[...] = jnp.concatenate([x_s2, x2_s0], axis=0)
    late_rows = _split_lhs(_layernorm(x2_s0))

    def project_first(grp):
        if grp == _X_TAIL_GROUP:
            arrive("x_tail")
            for t in range(xc, seq, xc):
                x_ref[t:t + xc, :] = xt_ref[:, t:t + xc].T
        return [[jnp.concatenate([early_ref[:, ((grp * 2 + hh) * 3 + m) * dh:
                                            ((grp * 2 + hh) * 3 + m + 1) * dh], late], axis=0)
                 for m, late in enumerate(qkv)]
                for hh, qkv in enumerate(project(late_rows, grp))]

    a_ref[...] = attend(project_first, 2)

    def feed_forward(out_row):
        y = x1_ref[...] + _output_finish(hid_ref, both, w2_ref, s2_ref, wide_ref[...])
        y_ref[pl.ds(out_row, seg), :] = y[seg:].astype(y_ref.dtype)
        x1 = xa_ref[...] + a_ref[tok0:, :]
        x1_ref[...] = x1
        gate_up(_split_lhs(_layernorm(x1)))
        return y[:seg]

    def step(i, carry):
        x2 = feed_forward(pl.multiple_of(jnp.maximum(i - 3, 0) * seg, seg))
        wide_ref[...] = _output_wide(hid_ref, both, w2_ref)
        x_next = x_ref[pl.ds(pl.multiple_of((i + 1) * seg, seg), seg), :].astype(_F32)
        xa = jnp.concatenate([x_next, x2], axis=0)
        xa_ref[...] = xa
        a_ref[...] = attend(projector(a_ref[0:tok0, :], xa), 2)
        return carry

    jax.lax.fori_loop(2, n_seg - 1, step, 0)

    x_s0 = feed_forward(seq - 4 * seg)
    a = attend(projector(a_ref[n_mem:tok0, :], x_s0), 1)
    y = x1_ref[...] + _output_dot(hid_ref, both, w2_ref, s2_ref)
    y_ref[seq - 3 * seg:seq - 2 * seg, :] = y[seg:].astype(y_ref.dtype)
    x1_s0 = x_s0 + a[n_mem:]
    last = seq - _LANES
    writes = [write_back(t, min(xc, last - t)) for t in range(0, last, xc)]
    a = attend(projector(a[:n_mem], y[:seg]), 1)
    x1 = jnp.concatenate([x1_s0, y[:seg] + a[n_mem:]], axis=0)
    gate_up(_split_lhs(_layernorm(x1)))
    y_ref[seq - 2 * seg:, :] = (x1 + _output_dot(hid_ref, both, w2_ref, s2_ref)).astype(y_ref.dtype)
    writes.append(write_back(last, _LANES))
    for copy in writes:
        copy.wait()


@functools.partial(jax.jit, static_argnames=("A_seg_len",))
def pallas_interleave_layers__memory_aug_recurrent_mem_tr__glu_gated_swiglu__prompt_kernel(
    A_x: jax.Array,
    A_mem0: jax.Array,
    A_Wq: jax.Array,
    A_Wk: jax.Array,
    A_Wv: jax.Array,
    A_Wo: jax.Array,
    A_seg_len: int,
    B_x: jax.Array,
    B_w1: jax.Array,
    B_w3: jax.Array,
    B_w2: jax.Array,
):
    del B_x
    batch, seq, dm = A_x.shape
    _, n_heads, dh = A_Wq.shape
    n_mem = A_mem0.shape[1]
    ffn = B_w1.shape[1]
    seg = int(A_seg_len)
    assert batch == 1 and seq % _XPOSE_CHUNK == 0 and _XPOSE_CHUNK % seg == 0 and _XPOSE_CHUNK >= 3 * seg
    rows = 2 * (n_mem + seg)
    full = dm - _HALF

    vmem = pl.BlockSpec(memory_space=pltpu.VMEM)
    hbm = pl.BlockSpec(memory_space=pltpu.HBM)
    out_t = pl.pallas_call(
        functools.partial(_kernel, seg=seg, n_heads=n_heads, dh=dh),
        out_shape=jax.ShapeDtypeStruct((dm, seq), A_x.dtype),
        in_specs=[hbm, vmem] + [hbm] * 7,
        out_specs=hbm,
        scratch_shapes=[
            pltpu.VMEM((dm, seq), _BF16),
            pltpu.VMEM((seq, dm), _BF16),
            pltpu.VMEM((dm * n_heads, dh), _BF16),
            pltpu.VMEM((dm * n_heads, dh), _BF16),
            pltpu.VMEM((dm * n_heads, dh), _BF16),
            _packed_scratch(n_heads // 2 * dm, 6 * dh),
            pltpu.VMEM((n_heads, dm, dh), _BF16),
            _packed_scratch(n_heads * dh, full),
            pltpu.VMEM((dm, ffn), _BF16),
            pltpu.VMEM((dm, ffn), _BF16),
            _packed_scratch(full, ffn),
            _packed_scratch(full, ffn),
            pltpu.VMEM((dm, ffn), _BF16),
            _packed_scratch(ffn, full),
            _packed_scratch(n_heads // 2 * _LANES, 3 * dh),
            _packed_scratch(_LANES, ffn // 2),
            _packed_scratch(_LANES, ffn // 2),
            _packed_scratch(n_heads * dh // 2, _LANES),
            _packed_scratch(ffn // 2, _LANES),
            _packed_scratch(rows, n_heads * dh * 3 // 2),
            _packed_scratch(2 * seg, ffn * 3 // 2),
            _packed_scratch(rows - seg, 3 * n_heads * dh),
            pltpu.VMEM((rows, dm), _F32),
            pltpu.VMEM((2 * seg, dm), _F32),
            pltpu.VMEM((2 * seg, dm), _F32),
            pltpu.VMEM((2 * seg, dm - _HALF - _LANES), _F32),
            pltpu.VMEM((seq, dm), _BF16),
            pltpu.SemaphoreType.DMA((3 + 3 * _QKV_DMA_CHUNKS + 3 * _FFN_DMA_CHUNKS,)),
            pltpu.SemaphoreType.DMA((seq // _XPOSE_CHUNK + 1,)),
        ],
        compiler_params=pltpu.CompilerParams(vmem_limit_bytes=110 * 1024 * 1024),
    )(
        A_x.reshape(seq, dm).T,
        A_mem0.reshape(n_mem, dm),
        A_Wq.reshape(dm * n_heads, dh),
        A_Wk.reshape(dm * n_heads, dh),
        A_Wv.reshape(dm * n_heads, dh),
        A_Wo.transpose(0, 2, 1),
        B_w1,
        B_w3,
        B_w2.T,
    )
    return out_t.T.reshape(batch, seq, dm)
```

```python
import functools

import jax
import jax.numpy as jnp
import numpy as np
import jax.experimental.pallas as pl
import jax.experimental.pallas.tpu as pltpu

_EPS = 1e-5
_MASK_FILL = -1000000000.0
_QK_LAG = 1
_PV_LAG = 3
_X_TAIL_GROUP = 12
_FFN_CHUNK = 768
_XPOSE_CHUNK = 256
_FFN_DMA_CHUNKS = 3
_QKV_DMA_CHUNKS = 2
_WORD_TILE = 4

_LANES = 128
_HALF = _LANES // 2
_F32 = jnp.float32
_BF16 = jnp.bfloat16


def _layernorm(x):
    mean = jnp.mean(x, axis=-1, keepdims=True)
    cen = x - mean
    var = jnp.mean(cen * cen, axis=-1, keepdims=True)
    return cen * jax.lax.rsqrt(var + _EPS)


def _dot(a, b):
    return jnp.dot(a, b, preferred_element_type=_F32)


def _dot_nt(a, b):
    return jax.lax.dot_general(a, b, (((1,), (1,)), ((), ())), preferred_element_type=_F32)


class _Packed:
    def __init__(self, ref):
        self.ref = ref
        self.shape = (2 * ref.shape[0], ref.shape[1])

    def _index(self, idx):
        rows, cols = idx
        if isinstance(rows, slice):
            lo, hi, _ = rows.indices(self.shape[0])
            return slice(lo // 2, hi // 2), cols
        start, size = rows
        return pl.ds(pl.multiple_of(start // 2, size // 2), size // 2), cols

    def __getitem__(self, idx):
        return pltpu.bitcast(self.ref[self._index(idx)], _BF16)

    def __setitem__(self, idx, value):
        self.ref[self._index(idx)] = pltpu.bitcast(value, jnp.uint32)


def _packed_scratch(rows, cols):
    return pltpu.VMEM((rows // 2, cols), jnp.uint32)


def _split_lhs(x):
    full = x.shape[1] - _HALF
    first, rest = x[:, :_LANES], x[:, _LANES:full]
    tail = x[:, full:]
    lhs_b0 = jnp.concatenate([first[:, :_HALF], tail], axis=1)
    lhs_s = jnp.concatenate([tail, first[:, _HALF:]], axis=1)
    return jnp.concatenate([first, rest, lhs_b0, lhs_s], axis=1).astype(_BF16)


def _paired_dot(lhs, w_a, w_b, w_s):
    full = w_a.shape[0]
    shared = _dot(lhs[:, full + _LANES:], w_s)
    lhs_b = jnp.concatenate([lhs[:, full:full + _LANES], lhs[:, _LANES:full]], axis=1)
    return _dot(lhs[:, :full], w_a) + shared, _dot(lhs_b, w_b) + shared


def _pair_weights(a_mid, a_tail, b_mid, b_tail):
    a_new = (a_mid.astype(_F32) - b_mid.astype(_F32)).astype(_BF16)
    b_new = (b_tail.astype(_F32) - a_tail.astype(_F32)).astype(_BF16)
    return a_new, b_new, jnp.concatenate([a_tail, b_mid], axis=0)


def _pair_output_weights(ut, vt):
    full = ut.shape[0] - _HALF
    mid = slice(_HALF, _LANES)
    u_new, v_new, shared = _pair_weights(ut[mid], ut[full:], vt[mid], vt[full:])
    u = jnp.concatenate([ut[:_HALF], u_new, ut[_LANES:full]], axis=0)
    v = jnp.concatenate([vt[:_HALF], v_new, vt[_LANES:full]], axis=0)
    return u.T, v.T, shared.T


def _output_wide(lhs_ref, rows, w_ref, lo=0, hi=None):
    hi = w_ref.shape[0] if hi is None else hi
    return _dot(lhs_ref[rows, lo:hi], w_ref[lo:hi, _LANES:])


def _output_edges(lhs_ref, rows, w_ref, s_ref):
    half = s_ref.shape[0]
    shared = _dot(lhs_ref[rows, 2 * half:], s_ref[:, :])
    v0 = _dot(lhs_ref[rows, half:2 * half], w_ref[half:, 0:_LANES])
    u0 = _dot(lhs_ref[rows, 0:half], w_ref[0:half, 0:_LANES])
    is_low = jax.lax.broadcasted_iota(jnp.int32, u0.shape, 1) < _HALF
    return u0 + jnp.where(is_low, v0, shared), v0[:, _HALF:] + shared[:, :_HALF]


def _output_finish(lhs_ref, rows, w_ref, s_ref, wide):
    first, last = _output_edges(lhs_ref, rows, w_ref, s_ref)
    return jnp.concatenate([first, wide, last], axis=1)


def _output_dot(lhs_ref, rows, w_ref, s_ref):
    first, last = _output_edges(lhs_ref, rows, w_ref, s_ref)
    return jnp.concatenate([first, _output_wide(lhs_ref, rows, w_ref), last], axis=1)


def _mask_tables(n_streams, n_mem, seg):
    tok0 = n_streams * n_mem
    rows = tok0 + n_streams * seg

    def split(axis):
        idx = jax.lax.broadcasted_iota(jnp.int32, (rows, rows), axis)
        is_mem = idx < tok0
        stream = jnp.where(is_mem, idx // n_mem, (idx - tok0) // seg)
        pos = jnp.where(is_mem, idx % n_mem, n_mem + (idx - tok0) % seg)
        return stream, pos

    q_stream, q_pos = split(0)
    k_stream, k_pos = split(1)
    same = q_stream == k_stream
    visible = same & ((q_pos < n_mem) | (q_pos >= k_pos))
    fill = jnp.where(same, _MASK_FILL, -jnp.inf).astype(_F32)
    return visible, fill


def _kernel(xt_hbm, mem0_ref, wq_hbm, wk_hbm, wv_hbm, wot_hbm, w1_hbm, w3_hbm, w2t_hbm,
            out_hbm,
            xt_ref, x_ref, rq_ref, rk_ref, rv_ref, wqkv_ref, wot_ref, wo_ref,
            r1_ref, r3_ref, w1_ref, w3_ref, w2t_ref, w2_ref, sqkv_ref, s1_ref, s3_ref, so_ref, s2_ref,
            o_ref, hid_ref, early_ref, a_ref, xa_ref, x1_ref, wide_ref, y_ref, in_sems, out_sems,
            *, seg, n_heads, dh):
    seq, dm = x_ref.shape
    n_mem = mem0_ref.shape[0]
    n_seg = seq // seg
    ffn = w1_ref.shape[1]
    wqkv_ref, wo_ref, w1_ref, w3_ref, w2_ref = map(
        _Packed, (wqkv_ref, wo_ref, w1_ref, w3_ref, w2_ref))
    sqkv_ref, s1_ref, s3_ref, so_ref, s2_ref = map(
        _Packed, (sqkv_ref, s1_ref, s3_ref, so_ref, s2_ref))
    o_ref, hid_ref, early_ref = map(_Packed, (o_ref, hid_ref, early_ref))
    scale = dh ** -0.5
    n_grp = n_heads // 2
    tok0 = 2 * n_mem
    full = dm - _HALF
    mid = slice(_HALF, _LANES)
    fc = _FFN_CHUNK
    xc = _XPOSE_CHUNK
    wc = ffn // _FFN_DMA_CHUNKS

    def cols(ref, start, size):
        return ref.at[:, start:start + size]

    def rows_of(ref, start, size):
        return ref.at[start:start + size, :]

    raw_rows = dm * n_heads // _QKV_DMA_CHUNKS
    transfers = [("x_head", cols(xt_hbm, 0, _LANES), cols(xt_ref, 0, _LANES))]
    for name, src, dst in (("wq", wq_hbm, rq_ref), ("wk", wk_hbm, rk_ref), ("wv", wv_hbm, rv_ref)):
        for c in range(_QKV_DMA_CHUNKS):
            transfers.append(((name, c), rows_of(src, c * raw_rows, raw_rows),
                              rows_of(dst, c * raw_rows, raw_rows)))
    transfers.append(("wo", wot_hbm, wot_ref))
    for c in range(0, ffn, wc):
        transfers.append((("w1", c), cols(w1_hbm, c, wc), cols(r1_ref, c, wc)))
        transfers.append((("w3", c), cols(w3_hbm, c, wc), cols(r3_ref, c, wc)))
    for c in range(0, ffn, wc):
        transfers.append((("w2", c), cols(w2t_hbm, c, wc), cols(w2t_ref, c, wc)))
    transfers.append(("x_tail", cols(xt_hbm, _LANES, seq - _LANES), cols(xt_ref, _LANES, seq - _LANES)))
    copies = {name: pltpu.make_async_copy(src, dst, in_sems.at[n])
              for n, (name, src, dst) in enumerate(transfers)}

    def arrive(name):
        copies[name].wait()

    def project(h, grp):
        rows = slice(grp * dm, grp * dm + full)
        both = _paired_dot(h, wqkv_ref[rows, 0:3 * dh], wqkv_ref[rows, 3 * dh:],
                           sqkv_ref[grp * _LANES:(grp + 1) * _LANES, :])
        return [[qkv[:, m * dh:(m + 1) * dh].astype(_BF16) for m in range(3)] for qkv in both]

    def probabilities(qkv, visible, fill):
        probs = []
        for q, k, _ in qkv:
            s = jnp.where(visible, _dot_nt(q, k) * scale, fill)
            p = jnp.exp(s - jnp.max(s, axis=-1, keepdims=True))
            probs.append((p * (1.0 / jnp.sum(p, axis=-1, keepdims=True))).astype(_BF16))
        return probs

    def heads(project_group, n_streams, fillers=()):
        rows = n_streams * (n_mem + seg)
        visible, fill = _mask_tables(n_streams, n_mem, seg)
        qkv, probs = {}, {}
        for t in range(n_grp + _PV_LAG):
            if t < n_grp:
                qkv[t] = project_group(t)
            elif t - n_grp < len(fillers):
                fillers[t - n_grp]()
            if 0 <= t - _PV_LAG:
                grp = t - _PV_LAG
                outs = [_dot(p, v) for p, (_, _, v) in zip(probs.pop(grp), qkv.pop(grp))]
                for part, out in enumerate(outs + [outs[0] + outs[1]]):
                    col = (part * n_grp + grp) * dh
                    o_ref[0:rows, col:col + dh] = out.astype(_BF16)
            if 0 <= t - _QK_LAG < n_grp:
                probs[t - _QK_LAG] = probabilities(qkv[t - _QK_LAG], visible, fill)

    def attend(project_group, n_streams):
        rows, half, wide = slice(0, n_streams * (n_mem + seg)), n_grp * dh, []
        cut_u, cut_v = (n_grp - _PV_LAG) * dh, half + (n_grp - _PV_LAG + 1) * dh

        def part(lo, hi):
            return lambda: wide.append(_output_wide(o_ref, rows, wo_ref, lo, hi))

        heads(project_group, n_streams, (part(0, cut_u), part(half, cut_v)))
        first, last = _output_edges(o_ref, rows, wo_ref, so_ref)
        part(cut_u, half)()
        part(cut_v, 2 * half)()
        wide = (wide[0] + wide[1]) + (wide[2] + wide[3])
        return jnp.concatenate([first, wide, last], axis=1)

    def pair_gate_up(lo, hi):
        for raw, w_ref, s_ref in ((r1_ref, w1_ref, s1_ref), (r3_ref, w3_ref, s3_ref)):
            w_ref[0:_HALF, lo:hi] = raw[0:_HALF, lo:hi]
            w_ref[_LANES:, lo:hi] = raw[_LANES:full, lo:hi]
            for c in range(lo, hi, fc):
                ca, cb = slice(c, c + fc // 2), slice(c + fc // 2, c + fc)
                w_ref[mid, ca], w_ref[mid, cb], s_ref[:, c // 2:(c + fc) // 2] = _pair_weights(
                    raw[mid, ca], raw[full:, ca], raw[mid, cb], raw[full:, cb])

    def gate_up(f_in, lo=0, hi=ffn):
        for c in range(lo, hi, fc):
            ca, cb = slice(c, c + fc // 2), slice(c + fc // 2, c + fc)
            cs = slice(c // 2, (c + fc) // 2)
            gates = _paired_dot(f_in, w1_ref[0:full, ca], w1_ref[0:full, cb], s1_ref[:, cs])
            ups = _paired_dot(f_in, w3_ref[0:full, ca], w3_ref[0:full, cb], s3_ref[:, cs])
            hids = [gate * jax.nn.sigmoid(gate) * up for gate, up in zip(gates, ups)]
            for part, hid in enumerate(hids + [hids[0] + hids[1]]):
                col = (part * ffn + c) // 2
                hid_ref[0:hid.shape[0], col:col + fc // 2] = hid.astype(_BF16)

    def stage_down(lo, hi):
        for c in range(lo, hi, fc):
            rows_u = slice(c // 2, (c + fc) // 2)
            rows_v = slice((ffn + c) // 2, (ffn + c + fc) // 2)
            w2_ref[rows_u, :], w2_ref[rows_v, :], s2_ref[rows_u, :] = _pair_output_weights(
                w2t_ref[:, c:c + fc // 2], w2t_ref[:, c + fc // 2:c + fc])

    def projector(mem, x):
        return functools.partial(project, _split_lhs(jnp.concatenate([mem, _layernorm(x)], axis=0)))

    def write_back(t, size):
        xt_ref[:, t:t + size] = y_ref[t:t + size, :].T
        copy = pltpu.make_async_copy(
            cols(xt_ref, t, size), cols(out_hbm, t, size), out_sems.at[pl.cdiv(t, xc)])
        copy.start()
        return copy

    for copy in copies.values():
        copy.start()
    arrive("x_head")
    x_ref[0:_LANES, :] = xt_ref[:, 0:_LANES].T

    pairs = n_heads // 2
    d_chunk = dm // _QKV_DMA_CHUNKS
    for m, (name, raw_ref) in enumerate((("wq", rq_ref), ("wk", rk_ref), ("wv", rv_ref))):
        words = raw_ref.bitcast(jnp.uint32)
        for c in range(_QKV_DMA_CHUNKS):
            arrive((name, c))

            def regroup(quad, carry, m=m, c=c, words=words):
                start = pl.multiple_of(c * d_chunk * pairs + quad * _WORD_TILE, _WORD_TILE)
                view = words.at[pl.ds(start, d_chunk * pairs - pairs + _WORD_TILE), :]
                for r in range(_WORD_TILE):
                    even_d = view[pl.ds(r, d_chunk // 2, stride=n_heads), :]
                    odd_d = view[pl.ds(r + pairs, d_chunk // 2, stride=n_heads), :]
                    lo = (even_d & jnp.uint32(0xFFFF)) | (odd_d << 16)
                    hi = (even_d >> 16) | (odd_d & jnp.uint32(0xFFFF0000))
                    row = (quad * _WORD_TILE + r) * (dm // 2) + c * (d_chunk // 2)
                    for half, val in enumerate((lo, hi)):
                        col = (half * 3 + m) * dh
                        wqkv_ref.ref[pl.ds(pl.multiple_of(row, 8), d_chunk // 2), col:col + dh] = val
                return carry

            jax.lax.fori_loop(0, pairs // _WORD_TILE, regroup, 0)

    def pair_heads(grp, carry):
        ca, cb = slice(0, 3 * dh), slice(3 * dh, 6 * dh)
        mid_rows, tail_rows = (grp * dm + _HALF, _HALF), (grp * dm + full, _HALF)
        (wqkv_ref[mid_rows, ca], wqkv_ref[mid_rows, cb],
         sqkv_ref[(grp * _LANES, _LANES), :]) = _pair_weights(
             wqkv_ref[mid_rows, ca], wqkv_ref[tail_rows, ca],
             wqkv_ref[mid_rows, cb], wqkv_ref[tail_rows, cb])
        return carry

    jax.lax.fori_loop(0, n_grp, pair_heads, 0)

    mem0 = mem0_ref[...].astype(_F32)
    a_ref[0:n_mem, :] = mem0

    def first_segments(s, carry):
        x_s = x_ref[pl.ds(pl.multiple_of(s * seg, seg), seg), :].astype(_F32)
        heads(projector(a_ref[0:n_mem, :], x_s), 1)

        @pl.when(s == 0)
        def _():
            arrive("wo")

            def stage_wo(grp, carry):
                rows_u, rows_v = (grp * dh, dh), ((n_grp + grp) * dh, dh)
                wo_ref[rows_u, :], wo_ref[rows_v, :], so_ref[rows_u, :] = _pair_output_weights(
                    wot_ref[2 * grp], wot_ref[2 * grp + 1])
                return carry

            jax.lax.fori_loop(0, n_grp, stage_wo, 0, unroll=2)

        a = _output_dot(o_ref, slice(0, n_mem + seg), wo_ref, so_ref)
        a_ref[0:n_mem, :] = a[:n_mem]
        a_ref[pl.ds(pl.multiple_of(tok0 + (1 - s) * seg, n_mem), seg), :] = a[n_mem:]
        return carry

    jax.lax.fori_loop(0, 2, first_segments, 0)
    a_ref[n_mem:tok0, :] = mem0
    x1 = jnp.concatenate([x_ref[seg:2 * seg, :], x_ref[0:seg, :]], axis=0).astype(_F32)
    x1 = x1 + a_ref[tok0:, :]
    x1_ref[...] = x1
    f_in = _split_lhs(_layernorm(x1))
    for c in range(0, ffn, wc):
        arrive(("w1", c))
        arrive(("w3", c))
        pair_gate_up(c, c + wc)
        gate_up(f_in, c, c + wc)
    both = slice(0, 2 * seg)
    x_s2 = x_ref[2 * seg:3 * seg, :].astype(_F32)
    project_early = projector(a_ref[0:tok0, :], x_s2)
    wide = None
    for n, c in enumerate(range(0, ffn, wc)):
        for grp in range(n * n_grp // _FFN_DMA_CHUNKS, (n + 1) * n_grp // _FFN_DMA_CHUNKS):
            early = [m for qkv in project_early(grp) for m in qkv]
            early_ref[:, grp * 6 * dh:(grp + 1) * 6 * dh] = jnp.concatenate(early, axis=1)
        arrive(("w2", c))
        stage_down(c, c + wc)
        for lo in (c // 2, (ffn + c) // 2):
            part = _output_wide(hid_ref, both, w2_ref, lo, lo + wc // 2)
            wide = part if wide is None else wide + part
    wide_ref[...] = wide
    x2_s0 = x1_ref[seg:, :] + _output_finish(
        hid_ref, slice(seg, 2 * seg), w2_ref, s2_ref, wide[seg:])
    xa_ref[...] = jnp.concatenate([x_s2, x2_s0], axis=0)
    late_rows = _split_lhs(_layernorm(x2_s0))

    def project_first(grp):
        if grp == _X_TAIL_GROUP:
            arrive("x_tail")
            for t in range(_LANES, seq, xc):
                end = min(t + xc, seq)
                x_ref[t:end, :] = xt_ref[:, t:end].T
        return [[jnp.concatenate([early_ref[:, ((grp * 2 + hh) * 3 + m) * dh:
                                            ((grp * 2 + hh) * 3 + m + 1) * dh], late], axis=0)
                 for m, late in enumerate(qkv)]
                for hh, qkv in enumerate(project(late_rows, grp))]

    a_ref[...] = attend(project_first, 2)

    def feed_forward(out_row):
        y = x1_ref[...] + _output_finish(hid_ref, both, w2_ref, s2_ref, wide_ref[...])
        y_ref[pl.ds(out_row, seg), :] = y[seg:].astype(y_ref.dtype)
        x1 = xa_ref[...] + a_ref[tok0:, :]
        x1_ref[...] = x1
        gate_up(_split_lhs(_layernorm(x1)))
        return y[:seg]

    def step(i, carry):
        x2 = feed_forward(pl.multiple_of(jnp.maximum(i - 3, 0) * seg, seg))
        wide_ref[...] = _output_wide(hid_ref, both, w2_ref)
        x_next = x_ref[pl.ds(pl.multiple_of((i + 1) * seg, seg), seg), :].astype(_F32)
        xa = jnp.concatenate([x_next, x2], axis=0)
        xa_ref[...] = xa
        a_ref[...] = attend(projector(a_ref[0:tok0, :], xa), 2)
        return carry

    jax.lax.fori_loop(2, n_seg - 1, step, 0)

    x_s0 = feed_forward(seq - 4 * seg)
    a = attend(projector(a_ref[n_mem:tok0, :], x_s0), 1)
    y = x1_ref[...] + _output_dot(hid_ref, both, w2_ref, s2_ref)
    y_ref[seq - 3 * seg:seq - 2 * seg, :] = y[seg:].astype(y_ref.dtype)
    x1_s0 = x_s0 + a[n_mem:]
    last = seq - _LANES
    writes = [write_back(t, min(xc, last - t)) for t in range(0, last, xc)]
    a = attend(projector(a[:n_mem], y[:seg]), 1)
    x1 = jnp.concatenate([x1_s0, y[:seg] + a[n_mem:]], axis=0)
    gate_up(_split_lhs(_layernorm(x1)))
    y_ref[seq - 2 * seg:, :] = (x1 + _output_dot(hid_ref, both, w2_ref, s2_ref)).astype(y_ref.dtype)
    writes.append(write_back(last, _LANES))
    for copy in writes:
        copy.wait()


@functools.partial(jax.jit, static_argnames=("A_seg_len",))
def pallas_interleave_layers__memory_aug_recurrent_mem_tr__glu_gated_swiglu__prompt_kernel(
    A_x: jax.Array,
    A_mem0: jax.Array,
    A_Wq: jax.Array,
    A_Wk: jax.Array,
    A_Wv: jax.Array,
    A_Wo: jax.Array,
    A_seg_len: int,
    B_x: jax.Array,
    B_w1: jax.Array,
    B_w3: jax.Array,
    B_w2: jax.Array,
):
    del B_x
    batch, seq, dm = A_x.shape
    _, n_heads, dh = A_Wq.shape
    n_mem = A_mem0.shape[1]
    ffn = B_w1.shape[1]
    seg = int(A_seg_len)
    assert batch == 1 and seq % _XPOSE_CHUNK == 0 and _LANES % seg == 0 and _LANES >= 3 * seg
    rows = 2 * (n_mem + seg)
    full = dm - _HALF

    vmem = pl.BlockSpec(memory_space=pltpu.VMEM)
    hbm = pl.BlockSpec(memory_space=pltpu.HBM)
    out_t = pl.pallas_call(
        functools.partial(_kernel, seg=seg, n_heads=n_heads, dh=dh),
        out_shape=jax.ShapeDtypeStruct((dm, seq), A_x.dtype),
        in_specs=[hbm, vmem] + [hbm] * 7,
        out_specs=hbm,
        scratch_shapes=[
            pltpu.VMEM((dm, seq), _BF16),
            pltpu.VMEM((seq, dm), _BF16),
            pltpu.VMEM((dm * n_heads, dh), _BF16),
            pltpu.VMEM((dm * n_heads, dh), _BF16),
            pltpu.VMEM((dm * n_heads, dh), _BF16),
            _packed_scratch(n_heads // 2 * dm, 6 * dh),
            pltpu.VMEM((n_heads, dm, dh), _BF16),
            _packed_scratch(n_heads * dh, full),
            pltpu.VMEM((dm, ffn), _BF16),
            pltpu.VMEM((dm, ffn), _BF16),
            _packed_scratch(full, ffn),
            _packed_scratch(full, ffn),
            pltpu.VMEM((dm, ffn), _BF16),
            _packed_scratch(ffn, full),
            _packed_scratch(n_heads // 2 * _LANES, 3 * dh),
            _packed_scratch(_LANES, ffn // 2),
            _packed_scratch(_LANES, ffn // 2),
            _packed_scratch(n_heads * dh // 2, _LANES),
            _packed_scratch(ffn // 2, _LANES),
            _packed_scratch(rows, n_heads * dh * 3 // 2),
            _packed_scratch(2 * seg, ffn * 3 // 2),
            _packed_scratch(rows - seg, 3 * n_heads * dh),
            pltpu.VMEM((rows, dm), _F32),
            pltpu.VMEM((2 * seg, dm), _F32),
            pltpu.VMEM((2 * seg, dm), _F32),
            pltpu.VMEM((2 * seg, dm - _HALF - _LANES), _F32),
            pltpu.VMEM((seq, dm), _BF16),
            pltpu.SemaphoreType.DMA((3 + 3 * _QKV_DMA_CHUNKS + 3 * _FFN_DMA_CHUNKS,)),
            pltpu.SemaphoreType.DMA((seq // _XPOSE_CHUNK + 1,)),
        ],
        compiler_params=pltpu.CompilerParams(vmem_limit_bytes=110 * 1024 * 1024),
    )(
        A_x.reshape(seq, dm).T,
        A_mem0.reshape(n_mem, dm),
        A_Wq.reshape(dm * n_heads, dh),
        A_Wk.reshape(dm * n_heads, dh),
        A_Wv.reshape(dm * n_heads, dh),
        A_Wo.transpose(0, 2, 1),
        B_w1,
        B_w3,
        B_w2.T,
    )
    return out_t.T.reshape(batch, seq, dm)
```

```python
import functools

import jax
import jax.numpy as jnp
import jax.experimental.pallas as pl
import jax.experimental.pallas.tpu as pltpu

_EPS = 1e-5
_MASK_FILL = -1000000000.0
_QK_LAG = 1
_PV_LAG = 3
_X_TAIL_GROUP = 12
_FFN_CHUNK = 768
_XPOSE_CHUNK = 256
_FFN_DMA_CHUNKS = 3
_QKV_DMA_CHUNKS = 2
_WORD_TILE = 4

_LANES = 128
_HALF = _LANES // 2
_F32 = jnp.float32
_BF16 = jnp.bfloat16


def _layernorm(x):
    mean = jnp.mean(x, axis=-1, keepdims=True)
    cen = x - mean
    var = jnp.mean(cen * cen, axis=-1, keepdims=True)
    return cen * jax.lax.rsqrt(var + _EPS)


def _dot(a, b):
    return jnp.dot(a, b, preferred_element_type=_F32)


def _dot_nt(a, b):
    return jax.lax.dot_general(a, b, (((1,), (1,)), ((), ())), preferred_element_type=_F32)


class _Packed:
    def __init__(self, ref):
        self.ref = ref
        self.shape = (2 * ref.shape[0], ref.shape[1])

    def _index(self, idx):
        rows, cols = idx
        if isinstance(rows, slice):
            lo, hi, _ = rows.indices(self.shape[0])
            return slice(lo // 2, hi // 2), cols
        start, size = rows
        return pl.ds(pl.multiple_of(start // 2, size // 2), size // 2), cols

    def __getitem__(self, idx):
        return pltpu.bitcast(self.ref[self._index(idx)], _BF16)

    def __setitem__(self, idx, value):
        self.ref[self._index(idx)] = pltpu.bitcast(value, jnp.uint32)


def _packed_scratch(rows, cols):
    return pltpu.VMEM((rows // 2, cols), jnp.uint32)


def _split_lhs(x):
    full = x.shape[1] - _HALF
    first, rest = x[:, :_LANES], x[:, _LANES:full]
    tail = x[:, full:]
    lhs_b0 = jnp.concatenate([first[:, :_HALF], tail], axis=1)
    lhs_s = jnp.concatenate([tail, first[:, _HALF:]], axis=1)
    return jnp.concatenate([first, rest, lhs_b0, lhs_s], axis=1).astype(_BF16)


def _paired_dot(lhs, w_a, w_b, w_s):
    full = w_a.shape[0]
    shared = _dot(lhs[:, full + _LANES:], w_s)
    lhs_b = jnp.concatenate([lhs[:, full:full + _LANES], lhs[:, _LANES:full]], axis=1)
    return _dot(lhs[:, :full], w_a) + shared, _dot(lhs_b, w_b) + shared


def _pair_weights(a_mid, a_tail, b_mid, b_tail):
    a_new = (a_mid.astype(_F32) - b_mid.astype(_F32)).astype(_BF16)
    b_new = (b_tail.astype(_F32) - a_tail.astype(_F32)).astype(_BF16)
    return a_new, b_new, jnp.concatenate([a_tail, b_mid], axis=0)


def _pair_output_weights(ut, vt):
    full = ut.shape[0] - _HALF
    mid = slice(_HALF, _LANES)
    u_new, v_new, shared = _pair_weights(ut[mid], ut[full:], vt[mid], vt[full:])
    u = jnp.concatenate([ut[:_HALF], u_new, ut[_LANES:full]], axis=0)
    v = jnp.concatenate([vt[:_HALF], v_new, vt[_LANES:full]], axis=0)
    return u.T, v.T, shared.T


def _output_wide(lhs_ref, rows, w_ref, lo=0, hi=None):
    hi = w_ref.shape[0] if hi is None else hi
    return _dot(lhs_ref[rows, lo:hi], w_ref[lo:hi, _LANES:])


def _output_edges(lhs_ref, rows, w_ref, s_ref):
    half = s_ref.shape[0]
    shared = _dot(lhs_ref[rows, 2 * half:], s_ref[:, :])
    v0 = _dot(lhs_ref[rows, half:2 * half], w_ref[half:, 0:_LANES])
    u0 = _dot(lhs_ref[rows, 0:half], w_ref[0:half, 0:_LANES])
    is_low = jax.lax.broadcasted_iota(jnp.int32, u0.shape, 1) < _HALF
    return u0 + jnp.where(is_low, v0, shared), v0[:, _HALF:] + shared[:, :_HALF]


def _output_finish(lhs_ref, rows, w_ref, s_ref, wide):
    first, last = _output_edges(lhs_ref, rows, w_ref, s_ref)
    return jnp.concatenate([first, wide, last], axis=1)


def _output_dot(lhs_ref, rows, w_ref, s_ref):
    first, last = _output_edges(lhs_ref, rows, w_ref, s_ref)
    return jnp.concatenate([first, _output_wide(lhs_ref, rows, w_ref), last], axis=1)


def _mask_tables(n_streams, n_mem, seg):
    tok0 = n_streams * n_mem
    rows = tok0 + n_streams * seg

    def split(axis):
        idx = jax.lax.broadcasted_iota(jnp.int32, (rows, rows), axis)
        is_mem = idx < tok0
        stream = jnp.where(is_mem, idx // n_mem, (idx - tok0) // seg)
        pos = jnp.where(is_mem, idx % n_mem, n_mem + (idx - tok0) % seg)
        return stream, pos

    q_stream, q_pos = split(0)
    k_stream, k_pos = split(1)
    same = q_stream == k_stream
    visible = same & ((q_pos < n_mem) | (q_pos >= k_pos))
    fill = jnp.where(same, _MASK_FILL, -jnp.inf).astype(_F32)
    return visible, fill


def _kernel(xt_hbm, mem0_ref, wq_hbm, wk_hbm, wv_hbm, wot_hbm, w1_hbm, w3_hbm, w2t_hbm,
            out_hbm,
            xt_ref, x_ref, rq_ref, rk_ref, rv_ref, wqkv_ref, wot_ref, wo_ref,
            r1_ref, r3_ref, w1_ref, w3_ref, w2t_ref, w2_ref, sqkv_ref, s1_ref, s3_ref, so_ref, s2_ref,
            o_ref, hid_ref, early_ref, a_ref, xa_ref, x1_ref, wide_ref, y_ref, in_sems, out_sems,
            *, seg, n_heads, dh):
    seq, dm = x_ref.shape
    n_mem = mem0_ref.shape[0]
    n_seg = seq // seg
    ffn = w1_ref.shape[1]
    wqkv_ref, wo_ref, w1_ref, w3_ref, w2_ref = map(
        _Packed, (wqkv_ref, wo_ref, w1_ref, w3_ref, w2_ref))
    sqkv_ref, s1_ref, s3_ref, so_ref, s2_ref = map(
        _Packed, (sqkv_ref, s1_ref, s3_ref, so_ref, s2_ref))
    o_ref, hid_ref, early_ref = map(_Packed, (o_ref, hid_ref, early_ref))
    scale = dh ** -0.5
    n_grp = n_heads // 2
    tok0 = 2 * n_mem
    full = dm - _HALF
    mid = slice(_HALF, _LANES)
    fc = _FFN_CHUNK
    xc = _XPOSE_CHUNK
    wc = ffn // _FFN_DMA_CHUNKS

    def cols(ref, start, size):
        return ref.at[:, start:start + size]

    def rows_of(ref, start, size):
        return ref.at[start:start + size, :]

    raw_rows = dm * n_heads // _QKV_DMA_CHUNKS
    transfers = [("x_head", cols(xt_hbm, 0, _LANES), cols(xt_ref, 0, _LANES))]
    for name, src, dst in (("wq", wq_hbm, rq_ref), ("wk", wk_hbm, rk_ref), ("wv", wv_hbm, rv_ref)):
        for c in range(_QKV_DMA_CHUNKS):
            transfers.append(((name, c), rows_of(src, c * raw_rows, raw_rows),
                              rows_of(dst, c * raw_rows, raw_rows)))
    transfers.append(("wo", wot_hbm, wot_ref))
    for c in range(0, ffn, wc):
        transfers.append((("w1", c), cols(w1_hbm, c, wc), cols(r1_ref, c, wc)))
        transfers.append((("w3", c), cols(w3_hbm, c, wc), cols(r3_ref, c, wc)))
    for c in range(0, ffn, wc):
        transfers.append((("w2", c), cols(w2t_hbm, c, wc), cols(w2t_ref, c, wc)))
    transfers.append(("x_tail", cols(xt_hbm, _LANES, seq - _LANES), cols(xt_ref, _LANES, seq - _LANES)))
    copies = {name: pltpu.make_async_copy(src, dst, in_sems.at[n])
              for n, (name, src, dst) in enumerate(transfers)}

    def arrive(name):
        copies[name].wait()

    def project(h, grp):
        rows = slice(grp * dm, grp * dm + full)
        both = _paired_dot(h, wqkv_ref[rows, 0:3 * dh], wqkv_ref[rows, 3 * dh:],
                           sqkv_ref[grp * _LANES:(grp + 1) * _LANES, :])
        return [[qkv[:, m * dh:(m + 1) * dh].astype(_BF16) for m in range(3)] for qkv in both]

    def probabilities(qkv, visible, fill):
        probs = []
        for q, k, _ in qkv:
            s = jnp.where(visible, _dot_nt(q, k) * scale, fill)
            p = jnp.exp(s - jnp.max(s, axis=-1, keepdims=True))
            probs.append((p * (1.0 / jnp.sum(p, axis=-1, keepdims=True))).astype(_BF16))
        return probs

    def heads(project_group, n_streams, fillers=()):
        rows = n_streams * (n_mem + seg)
        visible, fill = _mask_tables(n_streams, n_mem, seg)
        qkv, probs = {}, {}
        for t in range(n_grp + _PV_LAG):
            if t < n_grp:
                qkv[t] = project_group(t)
            elif t - n_grp < len(fillers):
                fillers[t - n_grp]()
            if 0 <= t - _PV_LAG:
                grp = t - _PV_LAG
                outs = [_dot(p, v) for p, (_, _, v) in zip(probs.pop(grp), qkv.pop(grp))]
                for part, out in enumerate(outs + [outs[0] + outs[1]]):
                    col = (part * n_grp + grp) * dh
                    o_ref[0:rows, col:col + dh] = out.astype(_BF16)
            if 0 <= t - _QK_LAG < n_grp:
                probs[t - _QK_LAG] = probabilities(qkv[t - _QK_LAG], visible, fill)

    def attend(project_group, n_streams):
        rows, half, wide = slice(0, n_streams * (n_mem + seg)), n_grp * dh, []
        cut_u, cut_v = (n_grp - _PV_LAG) * dh, half + (n_grp - _PV_LAG + 1) * dh

        def part(lo, hi):
            return lambda: wide.append(_output_wide(o_ref, rows, wo_ref, lo, hi))

        heads(project_group, n_streams, (part(0, cut_u), part(half, cut_v)))
        first, last = _output_edges(o_ref, rows, wo_ref, so_ref)
        part(cut_u, half)()
        part(cut_v, 2 * half)()
        wide = (wide[0] + wide[1]) + (wide[2] + wide[3])
        return jnp.concatenate([first, wide, last], axis=1)

    def pair_gate_up(lo, hi):
        for raw, w_ref, s_ref in ((r1_ref, w1_ref, s1_ref), (r3_ref, w3_ref, s3_ref)):
            w_ref[0:_HALF, lo:hi] = raw[0:_HALF, lo:hi]
            w_ref[_LANES:, lo:hi] = raw[_LANES:full, lo:hi]
            for c in range(lo, hi, fc):
                ca, cb = slice(c, c + fc // 2), slice(c + fc // 2, c + fc)
                w_ref[mid, ca], w_ref[mid, cb], s_ref[:, c // 2:(c + fc) // 2] = _pair_weights(
                    raw[mid, ca], raw[full:, ca], raw[mid, cb], raw[full:, cb])

    def gate_up(f_in, lo=0, hi=ffn):
        for c in range(lo, hi, fc):
            ca, cb = slice(c, c + fc // 2), slice(c + fc // 2, c + fc)
            cs = slice(c // 2, (c + fc) // 2)
            gates = _paired_dot(f_in, w1_ref[0:full, ca], w1_ref[0:full, cb], s1_ref[:, cs])
            ups = _paired_dot(f_in, w3_ref[0:full, ca], w3_ref[0:full, cb], s3_ref[:, cs])
            hids = [gate * jax.nn.sigmoid(gate) * up for gate, up in zip(gates, ups)]
            for part, hid in enumerate(hids + [hids[0] + hids[1]]):
                col = (part * ffn + c) // 2
                hid_ref[0:hid.shape[0], col:col + fc // 2] = hid.astype(_BF16)

    def stage_down(lo, hi):
        for c in range(lo, hi, fc):
            rows_u = slice(c // 2, (c + fc) // 2)
            rows_v = slice((ffn + c) // 2, (ffn + c + fc) // 2)
            w2_ref[rows_u, :], w2_ref[rows_v, :], s2_ref[rows_u, :] = _pair_output_weights(
                w2t_ref[:, c:c + fc // 2], w2t_ref[:, c + fc // 2:c + fc])

    def projector(mem, x):
        return functools.partial(project, _split_lhs(jnp.concatenate([mem, _layernorm(x)], axis=0)))

    def write_back(t, size):
        xt_ref[:, t:t + size] = y_ref[t:t + size, :].T
        copy = pltpu.make_async_copy(
            cols(xt_ref, t, size), cols(out_hbm, t, size), out_sems.at[pl.cdiv(t, xc)])
        copy.start()
        return copy

    for copy in copies.values():
        copy.start()
    arrive("x_head")
    x_ref[0:_LANES, :] = xt_ref[:, 0:_LANES].T

    pairs = n_heads // 2
    d_chunk = dm // _QKV_DMA_CHUNKS
    for m, (name, raw_ref) in enumerate((("wq", rq_ref), ("wk", rk_ref), ("wv", rv_ref))):
        words = raw_ref.bitcast(jnp.uint32)
        for c in range(_QKV_DMA_CHUNKS):
            arrive((name, c))

            def regroup(quad, carry, m=m, c=c, words=words):
                start = pl.multiple_of(c * d_chunk * pairs + quad * _WORD_TILE, _WORD_TILE)
                view = words.at[pl.ds(start, d_chunk * pairs - pairs + _WORD_TILE), :]
                for r in range(_WORD_TILE):
                    even_d = view[pl.ds(r, d_chunk // 2, stride=n_heads), :]
                    odd_d = view[pl.ds(r + pairs, d_chunk // 2, stride=n_heads), :]
                    lo = (even_d & jnp.uint32(0xFFFF)) | (odd_d << 16)
                    hi = (even_d >> 16) | (odd_d & jnp.uint32(0xFFFF0000))
                    row = (quad * _WORD_TILE + r) * (dm // 2) + c * (d_chunk // 2)
                    for half, val in enumerate((lo, hi)):
                        col = (half * 3 + m) * dh
                        wqkv_ref.ref[pl.ds(pl.multiple_of(row, 8), d_chunk // 2), col:col + dh] = val
                return carry

            jax.lax.fori_loop(0, pairs // _WORD_TILE, regroup, 0)

    def pair_heads(grp, carry):
        ca, cb = slice(0, 3 * dh), slice(3 * dh, 6 * dh)
        mid_rows, tail_rows = (grp * dm + _HALF, _HALF), (grp * dm + full, _HALF)
        (wqkv_ref[mid_rows, ca], wqkv_ref[mid_rows, cb],
         sqkv_ref[(grp * _LANES, _LANES), :]) = _pair_weights(
             wqkv_ref[mid_rows, ca], wqkv_ref[tail_rows, ca],
             wqkv_ref[mid_rows, cb], wqkv_ref[tail_rows, cb])
        return carry

    jax.lax.fori_loop(0, n_grp, pair_heads, 0)

    mem0 = mem0_ref[...].astype(_F32)
    a_ref[0:n_mem, :] = mem0

    def first_segments(s, carry):
        x_s = x_ref[pl.ds(pl.multiple_of(s * seg, seg), seg), :].astype(_F32)
        heads(projector(a_ref[0:n_mem, :], x_s), 1)

        @pl.when(s == 0)
        def _():
            arrive("wo")

            def stage_wo(grp, carry):
                rows_u, rows_v = (grp * dh, dh), ((n_grp + grp) * dh, dh)
                wo_ref[rows_u, :], wo_ref[rows_v, :], so_ref[rows_u, :] = _pair_output_weights(
                    wot_ref[2 * grp], wot_ref[2 * grp + 1])
                return carry

            jax.lax.fori_loop(0, n_grp, stage_wo, 0, unroll=2)

        a = _output_dot(o_ref, slice(0, n_mem + seg), wo_ref, so_ref)
        a_ref[0:n_mem, :] = a[:n_mem]
        a_ref[pl.ds(pl.multiple_of(tok0 + (1 - s) * seg, n_mem), seg), :] = a[n_mem:]
        return carry

    jax.lax.fori_loop(0, 2, first_segments, 0)
    a_ref[n_mem:tok0, :] = mem0
    x1 = jnp.concatenate([x_ref[seg:2 * seg, :], x_ref[0:seg, :]], axis=0).astype(_F32)
    x1 = x1 + a_ref[tok0:, :]
    x1_ref[...] = x1
    f_in = _split_lhs(_layernorm(x1))
    for c in range(0, ffn, wc):
        arrive(("w1", c))
        arrive(("w3", c))
        pair_gate_up(c, c + wc)
        gate_up(f_in, c, c + wc)
    both = slice(0, 2 * seg)
    x_s2 = x_ref[2 * seg:3 * seg, :].astype(_F32)
    project_early = projector(a_ref[0:tok0, :], x_s2)
    wide = None
    for n, c in enumerate(range(0, ffn, wc)):
        for grp in range(n * n_grp // _FFN_DMA_CHUNKS, (n + 1) * n_grp // _FFN_DMA_CHUNKS):
            early = [m for qkv in project_early(grp) for m in qkv]
            early_ref[:, grp * 6 * dh:(grp + 1) * 6 * dh] = jnp.concatenate(early, axis=1)
        arrive(("w2", c))
        stage_down(c, c + wc)
        for lo in (c // 2, (ffn + c) // 2):
            part = _output_wide(hid_ref, both, w2_ref, lo, lo + wc // 2)
            wide = part if wide is None else wide + part
    wide_ref[...] = wide
    x2_s0 = x1_ref[seg:, :] + _output_finish(
        hid_ref, slice(seg, 2 * seg), w2_ref, s2_ref, wide[seg:])
    xa_ref[...] = jnp.concatenate([x_s2, x2_s0], axis=0)
    late_rows = _split_lhs(_layernorm(x2_s0))

    def project_first(grp):
        if grp == _X_TAIL_GROUP:
            arrive("x_tail")
            for t in range(_LANES, seq, xc):
                end = min(t + xc, seq)
                x_ref[t:end, :] = xt_ref[:, t:end].T
        return [[jnp.concatenate([early_ref[:, ((grp * 2 + hh) * 3 + m) * dh:
                                            ((grp * 2 + hh) * 3 + m + 1) * dh], late], axis=0)
                 for m, late in enumerate(qkv)]
                for hh, qkv in enumerate(project(late_rows, grp))]

    a_ref[...] = attend(project_first, 2)

    def feed_forward(out_row):
        y = x1_ref[...] + _output_finish(hid_ref, both, w2_ref, s2_ref, wide_ref[...])
        y_ref[pl.ds(out_row, seg), :] = y[seg:].astype(y_ref.dtype)
        x1 = xa_ref[...] + a_ref[tok0:, :]
        x1_ref[...] = x1
        gate_up(_split_lhs(_layernorm(x1)))
        return y[:seg]

    def step(i, carry):
        x2 = feed_forward(pl.multiple_of(jnp.maximum(i - 3, 0) * seg, seg))
        wide_ref[...] = _output_wide(hid_ref, both, w2_ref)
        x_next = x_ref[pl.ds(pl.multiple_of((i + 1) * seg, seg), seg), :].astype(_F32)
        xa = jnp.concatenate([x_next, x2], axis=0)
        xa_ref[...] = xa
        a_ref[...] = attend(projector(a_ref[0:tok0, :], xa), 2)
        return carry

    jax.lax.fori_loop(2, n_seg - 1, step, 0)

    x_s0 = feed_forward(seq - 4 * seg)
    a = attend(projector(a_ref[n_mem:tok0, :], x_s0), 1)
    y = x1_ref[...] + _output_dot(hid_ref, both, w2_ref, s2_ref)
    y_ref[seq - 3 * seg:seq - 2 * seg, :] = y[seg:].astype(y_ref.dtype)
    x1_s0 = x_s0 + a[n_mem:]
    last = seq - _LANES
    writes = [write_back(t, min(xc, last - t)) for t in range(0, last, xc)]
    a = attend(projector(a[:n_mem], y[:seg]), 1)
    x1 = jnp.concatenate([x1_s0, y[:seg] + a[n_mem:]], axis=0)
    gate_up(_split_lhs(_layernorm(x1)))
    y_ref[seq - 2 * seg:, :] = (x1 + _output_dot(hid_ref, both, w2_ref, s2_ref)).astype(y_ref.dtype)
    writes.append(write_back(last, _LANES))
    for copy in writes:
        copy.wait()


@functools.partial(jax.jit, static_argnames=("A_seg_len",))
def pallas_interleave_layers__memory_aug_recurrent_mem_tr__glu_gated_swiglu__prompt_kernel(
    A_x: jax.Array,
    A_mem0: jax.Array,
    A_Wq: jax.Array,
    A_Wk: jax.Array,
    A_Wv: jax.Array,
    A_Wo: jax.Array,
    A_seg_len: int,
    B_x: jax.Array,
    B_w1: jax.Array,
    B_w3: jax.Array,
    B_w2: jax.Array,
):
    del B_x
    batch, seq, dm = A_x.shape
    _, n_heads, dh = A_Wq.shape
    n_mem = A_mem0.shape[1]
    ffn = B_w1.shape[1]
    seg = int(A_seg_len)
    assert batch == 1 and seq % _XPOSE_CHUNK == 0
    assert _LANES % seg == 0 and _LANES >= 3 * seg
    assert dm % _LANES == _HALF and dh == _LANES and n_heads // 2 > _X_TAIL_GROUP
    assert ffn % (_FFN_DMA_CHUNKS * _FFN_CHUNK) == 0
    rows = 2 * (n_mem + seg)
    full = dm - _HALF

    vmem = pl.BlockSpec(memory_space=pltpu.VMEM)
    hbm = pl.BlockSpec(memory_space=pltpu.HBM)
    out_t = pl.pallas_call(
        functools.partial(_kernel, seg=seg, n_heads=n_heads, dh=dh),
        out_shape=jax.ShapeDtypeStruct((dm, seq), A_x.dtype),
        in_specs=[hbm, vmem] + [hbm] * 7,
        out_specs=hbm,
        scratch_shapes=[
            pltpu.VMEM((dm, seq), _BF16),
            pltpu.VMEM((seq, dm), _BF16),
            pltpu.VMEM((dm * n_heads, dh), _BF16),
            pltpu.VMEM((dm * n_heads, dh), _BF16),
            pltpu.VMEM((dm * n_heads, dh), _BF16),
            _packed_scratch(n_heads // 2 * dm, 6 * dh),
            pltpu.VMEM((n_heads, dm, dh), _BF16),
            _packed_scratch(n_heads * dh, full),
            pltpu.VMEM((dm, ffn), _BF16),
            pltpu.VMEM((dm, ffn), _BF16),
            _packed_scratch(full, ffn),
            _packed_scratch(full, ffn),
            pltpu.VMEM((dm, ffn), _BF16),
            _packed_scratch(ffn, full),
            _packed_scratch(n_heads // 2 * _LANES, 3 * dh),
            _packed_scratch(_LANES, ffn // 2),
            _packed_scratch(_LANES, ffn // 2),
            _packed_scratch(n_heads * dh // 2, _LANES),
            _packed_scratch(ffn // 2, _LANES),
            _packed_scratch(rows, n_heads * dh * 3 // 2),
            _packed_scratch(2 * seg, ffn * 3 // 2),
            _packed_scratch(rows - seg, 3 * n_heads * dh),
            pltpu.VMEM((rows, dm), _F32),
            pltpu.VMEM((2 * seg, dm), _F32),
            pltpu.VMEM((2 * seg, dm), _F32),
            pltpu.VMEM((2 * seg, dm - _HALF - _LANES), _F32),
            pltpu.VMEM((seq, dm), _BF16),
            pltpu.SemaphoreType.DMA((3 + 3 * _QKV_DMA_CHUNKS + 3 * _FFN_DMA_CHUNKS,)),
            pltpu.SemaphoreType.DMA((seq // _XPOSE_CHUNK + 1,)),
        ],
        compiler_params=pltpu.CompilerParams(vmem_limit_bytes=110 * 1024 * 1024),
    )(
        A_x.reshape(seq, dm).T,
        A_mem0.reshape(n_mem, dm),
        A_Wq.reshape(dm * n_heads, dh),
        A_Wk.reshape(dm * n_heads, dh),
        A_Wv.reshape(dm * n_heads, dh),
        A_Wo.transpose(0, 2, 1),
        B_w1,
        B_w3,
        B_w2.T,
    )
    return out_t.T.reshape(batch, seq, dm)
```

```python
import functools

import jax
import jax.numpy as jnp
import jax.experimental.pallas as pl
import jax.experimental.pallas.tpu as pltpu

_EPS = 1e-5
_MASK_FILL = -1000000000.0
_QK_LAG = 1
_PV_LAG = 3
_X_TAIL_GROUP = 12
_FFN_CHUNK = 768
_XPOSE_CHUNK = 256
_FFN_DMA_CHUNKS = 3
_QKV_DMA_CHUNKS = 2

_LANES = 128
_HALF = _LANES // 2
_F32 = jnp.float32
_BF16 = jnp.bfloat16


def _layernorm(x):
    mean = jnp.mean(x, axis=-1, keepdims=True)
    cen = x - mean
    var = jnp.mean(cen * cen, axis=-1, keepdims=True)
    return cen * jax.lax.rsqrt(var + _EPS)


def _dot(a, b):
    return jnp.dot(a, b, preferred_element_type=_F32)


def _dot_nt(a, b):
    return jax.lax.dot_general(a, b, (((1,), (1,)), ((), ())), preferred_element_type=_F32)


class _Packed:
    def __init__(self, ref):
        self.ref = ref
        self.shape = (2 * ref.shape[0], ref.shape[1])

    def _index(self, idx):
        rows, cols = idx
        if isinstance(rows, slice):
            lo, hi, _ = rows.indices(self.shape[0])
            return slice(lo // 2, hi // 2), cols
        start, size = rows
        return pl.ds(pl.multiple_of(start // 2, size // 2), size // 2), cols

    def __getitem__(self, idx):
        return pltpu.bitcast(self.ref[self._index(idx)], _BF16)

    def __setitem__(self, idx, value):
        self.ref[self._index(idx)] = pltpu.bitcast(value, jnp.uint32)


def _packed_scratch(rows, cols):
    return pltpu.VMEM((rows // 2, cols), jnp.uint32)


def _split_lhs(x):
    full = x.shape[1] - _HALF
    first, rest = x[:, :_LANES], x[:, _LANES:full]
    tail = x[:, full:]
    lhs_b0 = jnp.concatenate([first[:, :_HALF], tail], axis=1)
    lhs_s = jnp.concatenate([tail, first[:, _HALF:]], axis=1)
    return jnp.concatenate([first, rest, lhs_b0, lhs_s], axis=1).astype(_BF16)


def _paired_dot(lhs, w_a, w_b, w_s):
    full = w_a.shape[0]
    shared = _dot(lhs[:, full + _LANES:], w_s)
    lhs_b = jnp.concatenate([lhs[:, full:full + _LANES], lhs[:, _LANES:full]], axis=1)
    return _dot(lhs[:, :full], w_a) + shared, _dot(lhs_b, w_b) + shared


def _pair_weights(a_mid, a_tail, b_mid, b_tail):
    a_new = (a_mid.astype(_F32) - b_mid.astype(_F32)).astype(_BF16)
    b_new = (b_tail.astype(_F32) - a_tail.astype(_F32)).astype(_BF16)
    return a_new, b_new, jnp.concatenate([a_tail, b_mid], axis=0)


def _pair_output_weights(ut, vt):
    full = ut.shape[0] - _HALF
    mid = slice(_HALF, _LANES)
    u_new, v_new, shared = _pair_weights(ut[mid], ut[full:], vt[mid], vt[full:])
    u = jnp.concatenate([ut[:_HALF], u_new, ut[_LANES:full]], axis=0)
    v = jnp.concatenate([vt[:_HALF], v_new, vt[_LANES:full]], axis=0)
    return u.T, v.T, shared.T


def _output_wide(lhs_ref, rows, w_ref, lo=0, hi=None):
    hi = w_ref.shape[0] if hi is None else hi
    return _dot(lhs_ref[rows, lo:hi], w_ref[lo:hi, _LANES:])


def _output_edges(lhs_ref, rows, w_ref, s_ref):
    half = s_ref.shape[0]
    shared = _dot(lhs_ref[rows, 2 * half:], s_ref[:, :])
    v0 = _dot(lhs_ref[rows, half:2 * half], w_ref[half:, 0:_LANES])
    u0 = _dot(lhs_ref[rows, 0:half], w_ref[0:half, 0:_LANES])
    is_low = jax.lax.broadcasted_iota(jnp.int32, u0.shape, 1) < _HALF
    return u0 + jnp.where(is_low, v0, shared), v0[:, _HALF:] + shared[:, :_HALF]


def _output_finish(lhs_ref, rows, w_ref, s_ref, wide):
    first, last = _output_edges(lhs_ref, rows, w_ref, s_ref)
    return jnp.concatenate([first, wide, last], axis=1)


def _output_dot(lhs_ref, rows, w_ref, s_ref):
    first, last = _output_edges(lhs_ref, rows, w_ref, s_ref)
    return jnp.concatenate([first, _output_wide(lhs_ref, rows, w_ref), last], axis=1)


def _mask_tables(n_streams, n_mem, seg):
    tok0 = n_streams * n_mem
    rows = tok0 + n_streams * seg

    def split(axis):
        idx = jax.lax.broadcasted_iota(jnp.int32, (rows, rows), axis)
        is_mem = idx < tok0
        stream = jnp.where(is_mem, idx // n_mem, (idx - tok0) // seg)
        pos = jnp.where(is_mem, idx % n_mem, n_mem + (idx - tok0) % seg)
        return stream, pos

    q_stream, q_pos = split(0)
    k_stream, k_pos = split(1)
    same = q_stream == k_stream
    visible = same & ((q_pos < n_mem) | (q_pos >= k_pos))
    fill = jnp.where(same, _MASK_FILL, -jnp.inf).astype(_F32)
    return visible, fill


def _kernel(xt_hbm, mem0_ref, wq_hbm, wk_hbm, wv_hbm, wot_hbm, w1_hbm, w3_hbm, w2t_hbm,
            out_hbm,
            xt_ref, x_ref, rq_ref, rk_ref, rv_ref, words_ref, wqkv_ref, wot_ref, wo_ref,
            r1_ref, r3_ref, w1_ref, w3_ref, w2t_ref, w2_ref, sqkv_ref, s1_ref, s3_ref, so_ref, s2_ref,
            o_ref, hid_ref, early_ref, a_ref, xa_ref, x1_ref, wide_ref, y_ref, in_sems, out_sems,
            *, seg, n_heads, dh):
    seq, dm = x_ref.shape
    n_mem = mem0_ref.shape[0]
    n_seg = seq // seg
    ffn = w1_ref.shape[1]
    wqkv_ref, wo_ref, w1_ref, w3_ref, w2_ref = map(
        _Packed, (wqkv_ref, wo_ref, w1_ref, w3_ref, w2_ref))
    sqkv_ref, s1_ref, s3_ref, so_ref, s2_ref = map(
        _Packed, (sqkv_ref, s1_ref, s3_ref, so_ref, s2_ref))
    o_ref, hid_ref, early_ref = map(_Packed, (o_ref, hid_ref, early_ref))
    scale = dh ** -0.5
    n_grp = n_heads // 2
    tok0 = 2 * n_mem
    full = dm - _HALF
    mid = slice(_HALF, _LANES)
    fc = _FFN_CHUNK
    xc = _XPOSE_CHUNK
    wc = ffn // _FFN_DMA_CHUNKS

    def cols(ref, start, size):
        return ref.at[:, start:start + size]

    def rows_of(ref, start, size):
        return ref.at[start:start + size, :]

    raw_rows = dm * n_heads // _QKV_DMA_CHUNKS
    transfers = [("x_head", cols(xt_hbm, 0, _LANES), cols(xt_ref, 0, _LANES))]
    for name, src, dst in (("wq", wq_hbm, rq_ref), ("wk", wk_hbm, rk_ref), ("wv", wv_hbm, rv_ref)):
        for c in range(_QKV_DMA_CHUNKS):
            transfers.append(((name, c), rows_of(src, c * raw_rows, raw_rows),
                              rows_of(dst, c * raw_rows, raw_rows)))
    transfers.append(("wo", wot_hbm, wot_ref))
    for c in range(0, ffn, wc):
        transfers.append((("w1", c), cols(w1_hbm, c, wc), cols(r1_ref, c, wc)))
        transfers.append((("w3", c), cols(w3_hbm, c, wc), cols(r3_ref, c, wc)))
    for c in range(0, ffn, wc):
        transfers.append((("w2", c), cols(w2t_hbm, c, wc), cols(w2t_ref, c, wc)))
    transfers.append(("x_tail", cols(xt_hbm, _LANES, seq - _LANES), cols(xt_ref, _LANES, seq - _LANES)))
    copies = {name: pltpu.make_async_copy(src, dst, in_sems.at[n])
              for n, (name, src, dst) in enumerate(transfers)}

    def arrive(name):
        copies[name].wait()

    def project(h, grp):
        rows = slice(grp * dm, grp * dm + full)
        both = _paired_dot(h, wqkv_ref[rows, 0:3 * dh], wqkv_ref[rows, 3 * dh:],
                           sqkv_ref[grp * _LANES:(grp + 1) * _LANES, :])
        return [[qkv[:, m * dh:(m + 1) * dh].astype(_BF16) for m in range(3)] for qkv in both]

    def probabilities(qkv, visible, fill):
        probs = []
        for q, k, _ in qkv:
            s = jnp.where(visible, _dot_nt(q, k) * scale, fill)
            p = jnp.exp(s - jnp.max(s, axis=-1, keepdims=True))
            probs.append((p * (1.0 / jnp.sum(p, axis=-1, keepdims=True))).astype(_BF16))
        return probs

    def heads(project_group, n_streams, fillers=()):
        rows = n_streams * (n_mem + seg)
        visible, fill = _mask_tables(n_streams, n_mem, seg)
        qkv, probs = {}, {}
        for t in range(n_grp + _PV_LAG):
            if t < n_grp:
                qkv[t] = project_group(t)
            elif t - n_grp < len(fillers):
                fillers[t - n_grp]()
            if 0 <= t - _PV_LAG:
                grp = t - _PV_LAG
                outs = [_dot(p, v) for p, (_, _, v) in zip(probs.pop(grp), qkv.pop(grp))]
                for part, out in enumerate(outs + [outs[0] + outs[1]]):
                    col = (part * n_grp + grp) * dh
                    o_ref[0:rows, col:col + dh] = out.astype(_BF16)
            if 0 <= t - _QK_LAG < n_grp:
                probs[t - _QK_LAG] = probabilities(qkv[t - _QK_LAG], visible, fill)

    def attend(project_group, n_streams):
        rows, half, wide = slice(0, n_streams * (n_mem + seg)), n_grp * dh, []
        cut_u, cut_v = (n_grp - _PV_LAG) * dh, half + (n_grp - _PV_LAG + 1) * dh

        def part(lo, hi):
            return lambda: wide.append(_output_wide(o_ref, rows, wo_ref, lo, hi))

        heads(project_group, n_streams, (part(0, cut_u), part(half, cut_v)))
        first, last = _output_edges(o_ref, rows, wo_ref, so_ref)
        part(cut_u, half)()
        part(cut_v, 2 * half)()
        wide = (wide[0] + wide[1]) + (wide[2] + wide[3])
        return jnp.concatenate([first, wide, last], axis=1)

    def pair_gate_up(lo, hi):
        for raw, w_ref, s_ref in ((r1_ref, w1_ref, s1_ref), (r3_ref, w3_ref, s3_ref)):
            w_ref[0:_HALF, lo:hi] = raw[0:_HALF, lo:hi]
            w_ref[_LANES:, lo:hi] = raw[_LANES:full, lo:hi]
            for c in range(lo, hi, fc):
                ca, cb = slice(c, c + fc // 2), slice(c + fc // 2, c + fc)
                w_ref[mid, ca], w_ref[mid, cb], s_ref[:, c // 2:(c + fc) // 2] = _pair_weights(
                    raw[mid, ca], raw[full:, ca], raw[mid, cb], raw[full:, cb])

    def gate_up(f_in, lo=0, hi=ffn):
        for c in range(lo, hi, fc):
            ca, cb = slice(c, c + fc // 2), slice(c + fc // 2, c + fc)
            cs = slice(c // 2, (c + fc) // 2)
            gates = _paired_dot(f_in, w1_ref[0:full, ca], w1_ref[0:full, cb], s1_ref[:, cs])
            ups = _paired_dot(f_in, w3_ref[0:full, ca], w3_ref[0:full, cb], s3_ref[:, cs])
            hids = [gate * jax.nn.sigmoid(gate) * up for gate, up in zip(gates, ups)]
            for part, hid in enumerate(hids + [hids[0] + hids[1]]):
                col = (part * ffn + c) // 2
                hid_ref[0:hid.shape[0], col:col + fc // 2] = hid.astype(_BF16)

    def stage_down(lo, hi):
        for c in range(lo, hi, fc):
            rows_u = slice(c // 2, (c + fc) // 2)
            rows_v = slice((ffn + c) // 2, (ffn + c + fc) // 2)
            w2_ref[rows_u, :], w2_ref[rows_v, :], s2_ref[rows_u, :] = _pair_output_weights(
                w2t_ref[:, c:c + fc // 2], w2t_ref[:, c + fc // 2:c + fc])

    def projector(mem, x):
        return functools.partial(project, _split_lhs(jnp.concatenate([mem, _layernorm(x)], axis=0)))

    def write_back(t, size):
        xt_ref[:, t:t + size] = y_ref[t:t + size, :].T
        copy = pltpu.make_async_copy(
            cols(xt_ref, t, size), cols(out_hbm, t, size), out_sems.at[pl.cdiv(t, xc)])
        copy.start()
        return copy

    for copy in copies.values():
        copy.start()
    arrive("x_head")
    x_ref[0:_LANES, :] = xt_ref[:, 0:_LANES].T

    d_chunk = dm // _QKV_DMA_CHUNKS
    word_rows = _XPOSE_CHUNK // 2
    for m, (name, raw_ref) in enumerate((("wq", rq_ref), ("wk", rk_ref), ("wv", rv_ref))):
        for c in range(_QKV_DMA_CHUNKS):
            arrive((name, c))

            def to_words(n, carry, c=c, raw_ref=raw_ref):
                src = pl.multiple_of(c * raw_rows + n * 2 * word_rows, 2 * word_rows)
                words_ref[pl.ds(pl.multiple_of(n * word_rows, word_rows), word_rows), :] = (
                    pltpu.bitcast(raw_ref[pl.ds(src, 2 * word_rows), :], jnp.uint32))
                return carry

            def regroup(grp, carry, m=m, c=c):
                even_d = words_ref[pl.ds(grp, d_chunk // 2, stride=n_heads), :]
                odd_d = words_ref[pl.ds(grp + n_grp, d_chunk // 2, stride=n_heads), :]
                lo = (even_d & jnp.uint32(0xFFFF)) | (odd_d << 16)
                hi = (even_d >> 16) | (odd_d & jnp.uint32(0xFFFF0000))
                row = pl.multiple_of(grp * (dm // 2) + c * (d_chunk // 2), 8)
                for half, val in enumerate((lo, hi)):
                    col = (half * 3 + m) * dh
                    wqkv_ref.ref[pl.ds(row, d_chunk // 2), col:col + dh] = val
                return carry

            jax.lax.fori_loop(0, raw_rows // (2 * word_rows), to_words, 0, unroll=4)
            jax.lax.fori_loop(0, n_grp, regroup, 0)

    def pair_heads(grp, carry):
        ca, cb = slice(0, 3 * dh), slice(3 * dh, 6 * dh)
        mid_rows, tail_rows = (grp * dm + _HALF, _HALF), (grp * dm + full, _HALF)
        (wqkv_ref[mid_rows, ca], wqkv_ref[mid_rows, cb],
         sqkv_ref[(grp * _LANES, _LANES), :]) = _pair_weights(
             wqkv_ref[mid_rows, ca], wqkv_ref[tail_rows, ca],
             wqkv_ref[mid_rows, cb], wqkv_ref[tail_rows, cb])
        return carry

    jax.lax.fori_loop(0, n_grp, pair_heads, 0)

    mem0 = mem0_ref[...].astype(_F32)
    a_ref[0:n_mem, :] = mem0

    def first_segments(s, carry):
        x_s = x_ref[pl.ds(pl.multiple_of(s * seg, seg), seg), :].astype(_F32)
        heads(projector(a_ref[0:n_mem, :], x_s), 1)

        @pl.when(s == 0)
        def _():
            arrive("wo")

            def stage_wo(grp, carry):
                rows_u, rows_v = (grp * dh, dh), ((n_grp + grp) * dh, dh)
                wo_ref[rows_u, :], wo_ref[rows_v, :], so_ref[rows_u, :] = _pair_output_weights(
                    wot_ref[2 * grp], wot_ref[2 * grp + 1])
                return carry

            jax.lax.fori_loop(0, n_grp, stage_wo, 0, unroll=2)

        a = _output_dot(o_ref, slice(0, n_mem + seg), wo_ref, so_ref)
        a_ref[0:n_mem, :] = a[:n_mem]
        a_ref[pl.ds(pl.multiple_of(tok0 + (1 - s) * seg, n_mem), seg), :] = a[n_mem:]
        return carry

    jax.lax.fori_loop(0, 2, first_segments, 0)
    a_ref[n_mem:tok0, :] = mem0
    x1 = jnp.concatenate([x_ref[seg:2 * seg, :], x_ref[0:seg, :]], axis=0).astype(_F32)
    x1 = x1 + a_ref[tok0:, :]
    x1_ref[...] = x1
    f_in = _split_lhs(_layernorm(x1))
    for c in range(0, ffn, wc):
        arrive(("w1", c))
        arrive(("w3", c))
        pair_gate_up(c, c + wc)
        gate_up(f_in, c, c + wc)
    both = slice(0, 2 * seg)
    x_s2 = x_ref[2 * seg:3 * seg, :].astype(_F32)
    project_early = projector(a_ref[0:tok0, :], x_s2)
    wide = None
    for n, c in enumerate(range(0, ffn, wc)):
        for grp in range(n * n_grp // _FFN_DMA_CHUNKS, (n + 1) * n_grp // _FFN_DMA_CHUNKS):
            early = [m for qkv in project_early(grp) for m in qkv]
            early_ref[:, grp * 6 * dh:(grp + 1) * 6 * dh] = jnp.concatenate(early, axis=1)
        arrive(("w2", c))
        stage_down(c, c + wc)
        for lo in (c // 2, (ffn + c) // 2):
            part = _output_wide(hid_ref, both, w2_ref, lo, lo + wc // 2)
            wide = part if wide is None else wide + part
    wide_ref[...] = wide
    x2_s0 = x1_ref[seg:, :] + _output_finish(
        hid_ref, slice(seg, 2 * seg), w2_ref, s2_ref, wide[seg:])
    xa_ref[...] = jnp.concatenate([x_s2, x2_s0], axis=0)
    late_rows = _split_lhs(_layernorm(x2_s0))

    def project_first(grp):
        if grp == _X_TAIL_GROUP:
            arrive("x_tail")
            for t in range(_LANES, seq, xc):
                end = min(t + xc, seq)
                x_ref[t:end, :] = xt_ref[:, t:end].T
        return [[jnp.concatenate([early_ref[:, ((grp * 2 + hh) * 3 + m) * dh:
                                            ((grp * 2 + hh) * 3 + m + 1) * dh], late], axis=0)
                 for m, late in enumerate(qkv)]
                for hh, qkv in enumerate(project(late_rows, grp))]

    a_ref[...] = attend(project_first, 2)

    def feed_forward(out_row):
        y = x1_ref[...] + _output_finish(hid_ref, both, w2_ref, s2_ref, wide_ref[...])
        y_ref[pl.ds(out_row, seg), :] = y[seg:].astype(y_ref.dtype)
        x1 = xa_ref[...] + a_ref[tok0:, :]
        x1_ref[...] = x1
        gate_up(_split_lhs(_layernorm(x1)))
        return y[:seg]

    def step(i, carry):
        x2 = feed_forward(pl.multiple_of(jnp.maximum(i - 3, 0) * seg, seg))
        wide_ref[...] = _output_wide(hid_ref, both, w2_ref)
        x_next = x_ref[pl.ds(pl.multiple_of((i + 1) * seg, seg), seg), :].astype(_F32)
        xa = jnp.concatenate([x_next, x2], axis=0)
        xa_ref[...] = xa
        a_ref[...] = attend(projector(a_ref[0:tok0, :], xa), 2)
        return carry

    jax.lax.fori_loop(2, n_seg - 1, step, 0)

    x_s0 = feed_forward(seq - 4 * seg)
    a = attend(projector(a_ref[n_mem:tok0, :], x_s0), 1)
    y = x1_ref[...] + _output_dot(hid_ref, both, w2_ref, s2_ref)
    y_ref[seq - 3 * seg:seq - 2 * seg, :] = y[seg:].astype(y_ref.dtype)
    x1_s0 = x_s0 + a[n_mem:]
    last = seq - _LANES
    writes = [write_back(t, min(xc, last - t)) for t in range(0, last, xc)]
    a = attend(projector(a[:n_mem], y[:seg]), 1)
    x1 = jnp.concatenate([x1_s0, y[:seg] + a[n_mem:]], axis=0)
    gate_up(_split_lhs(_layernorm(x1)))
    y_ref[seq - 2 * seg:, :] = (x1 + _output_dot(hid_ref, both, w2_ref, s2_ref)).astype(y_ref.dtype)
    writes.append(write_back(last, _LANES))
    for copy in writes:
        copy.wait()


@functools.partial(jax.jit, static_argnames=("A_seg_len",))
def pallas_interleave_layers__memory_aug_recurrent_mem_tr__glu_gated_swiglu__prompt_kernel(
    A_x: jax.Array,
    A_mem0: jax.Array,
    A_Wq: jax.Array,
    A_Wk: jax.Array,
    A_Wv: jax.Array,
    A_Wo: jax.Array,
    A_seg_len: int,
    B_x: jax.Array,
    B_w1: jax.Array,
    B_w3: jax.Array,
    B_w2: jax.Array,
):
    del B_x
    batch, seq, dm = A_x.shape
    _, n_heads, dh = A_Wq.shape
    n_mem = A_mem0.shape[1]
    ffn = B_w1.shape[1]
    seg = int(A_seg_len)
    assert batch == 1 and seq % _XPOSE_CHUNK == 0
    assert _LANES % seg == 0 and _LANES >= 3 * seg
    assert dm % _LANES == _HALF and dh == _LANES and n_heads // 2 > _X_TAIL_GROUP
    assert ffn % (_FFN_DMA_CHUNKS * _FFN_CHUNK) == 0
    rows = 2 * (n_mem + seg)
    full = dm - _HALF

    vmem = pl.BlockSpec(memory_space=pltpu.VMEM)
    hbm = pl.BlockSpec(memory_space=pltpu.HBM)
    out_t = pl.pallas_call(
        functools.partial(_kernel, seg=seg, n_heads=n_heads, dh=dh),
        out_shape=jax.ShapeDtypeStruct((dm, seq), A_x.dtype),
        in_specs=[hbm, vmem] + [hbm] * 7,
        out_specs=hbm,
        scratch_shapes=[
            pltpu.VMEM((dm, seq), _BF16),
            pltpu.VMEM((seq, dm), _BF16),
            pltpu.VMEM((dm * n_heads, dh), _BF16),
            pltpu.VMEM((dm * n_heads, dh), _BF16),
            pltpu.VMEM((dm * n_heads, dh), _BF16),
            _packed_scratch(dm * n_heads // _QKV_DMA_CHUNKS, dh),
            _packed_scratch(n_heads // 2 * dm, 6 * dh),
            pltpu.VMEM((n_heads, dm, dh), _BF16),
            _packed_scratch(n_heads * dh, full),
            pltpu.VMEM((dm, ffn), _BF16),
            pltpu.VMEM((dm, ffn), _BF16),
            _packed_scratch(full, ffn),
            _packed_scratch(full, ffn),
            pltpu.VMEM((dm, ffn), _BF16),
            _packed_scratch(ffn, full),
            _packed_scratch(n_heads // 2 * _LANES, 3 * dh),
            _packed_scratch(_LANES, ffn // 2),
            _packed_scratch(_LANES, ffn // 2),
            _packed_scratch(n_heads * dh // 2, _LANES),
            _packed_scratch(ffn // 2, _LANES),
            _packed_scratch(rows, n_heads * dh * 3 // 2),
            _packed_scratch(2 * seg, ffn * 3 // 2),
            _packed_scratch(rows - seg, 3 * n_heads * dh),
            pltpu.VMEM((rows, dm), _F32),
            pltpu.VMEM((2 * seg, dm), _F32),
            pltpu.VMEM((2 * seg, dm), _F32),
            pltpu.VMEM((2 * seg, dm - _HALF - _LANES), _F32),
            pltpu.VMEM((seq, dm), _BF16),
            pltpu.SemaphoreType.DMA((3 + 3 * _QKV_DMA_CHUNKS + 3 * _FFN_DMA_CHUNKS,)),
            pltpu.SemaphoreType.DMA((seq // _XPOSE_CHUNK + 1,)),
        ],
        compiler_params=pltpu.CompilerParams(vmem_limit_bytes=110 * 1024 * 1024),
    )(
        A_x.reshape(seq, dm).T,
        A_mem0.reshape(n_mem, dm),
        A_Wq.reshape(dm * n_heads, dh),
        A_Wk.reshape(dm * n_heads, dh),
        A_Wv.reshape(dm * n_heads, dh),
        A_Wo.transpose(0, 2, 1),
        B_w1,
        B_w3,
        B_w2.T,
    )
    return out_t.T.reshape(batch, seq, dm)
```

```python
import functools

import jax
import jax.numpy as jnp
import jax.experimental.pallas as pl
import jax.experimental.pallas.tpu as pltpu

_EPS = 1e-5
_MASK_FILL = -1000000000.0
_QK_LAG = 1
_PV_LAG = 3
_X_TAIL_GROUP = 12
_FFN_CHUNK = 768
_XPOSE_CHUNK = 256
_FFN_DMA_CHUNKS = 3
_QKV_DMA_CHUNKS = 2

_LANES = 128
_HALF = _LANES // 2
_F32 = jnp.float32
_BF16 = jnp.bfloat16


def _layernorm(x):
    mean = jnp.mean(x, axis=-1, keepdims=True)
    cen = x - mean
    var = jnp.mean(cen * cen, axis=-1, keepdims=True)
    return cen * jax.lax.rsqrt(var + _EPS)


def _dot(a, b):
    return jnp.dot(a, b, preferred_element_type=_F32)


def _dot_nt(a, b):
    return jax.lax.dot_general(a, b, (((1,), (1,)), ((), ())), preferred_element_type=_F32)


class _Packed:
    def __init__(self, ref):
        self.ref = ref
        self.shape = (2 * ref.shape[0], ref.shape[1])

    def _index(self, idx):
        rows, cols = idx
        if isinstance(rows, slice):
            lo, hi, _ = rows.indices(self.shape[0])
            return slice(lo // 2, hi // 2), cols
        start, size = rows
        return pl.ds(pl.multiple_of(start // 2, size // 2), size // 2), cols

    def __getitem__(self, idx):
        return pltpu.bitcast(self.ref[self._index(idx)], _BF16)

    def __setitem__(self, idx, value):
        self.ref[self._index(idx)] = pltpu.bitcast(value, jnp.uint32)


def _packed_scratch(rows, cols):
    return pltpu.VMEM((rows // 2, cols), jnp.uint32)


def _split_lhs(x):
    full = x.shape[1] - _HALF
    first, rest = x[:, :_LANES], x[:, _LANES:full]
    tail = x[:, full:]
    lhs_b0 = jnp.concatenate([first[:, :_HALF], tail], axis=1)
    lhs_s = jnp.concatenate([tail, first[:, _HALF:]], axis=1)
    return jnp.concatenate([first, rest, lhs_b0, lhs_s], axis=1).astype(_BF16)


def _paired_dot(lhs, w_a, w_b, w_s):
    full = w_a.shape[0]
    shared = _dot(lhs[:, full + _LANES:], w_s)
    lhs_b = jnp.concatenate([lhs[:, full:full + _LANES], lhs[:, _LANES:full]], axis=1)
    return _dot(lhs[:, :full], w_a) + shared, _dot(lhs_b, w_b) + shared


def _pair_weights(a_mid, a_tail, b_mid, b_tail):
    a_new = (a_mid.astype(_F32) - b_mid.astype(_F32)).astype(_BF16)
    b_new = (b_tail.astype(_F32) - a_tail.astype(_F32)).astype(_BF16)
    return a_new, b_new, jnp.concatenate([a_tail, b_mid], axis=0)


def _pair_output_weights(ut, vt):
    full = ut.shape[0] - _HALF
    mid = slice(_HALF, _LANES)
    u_new, v_new, shared = _pair_weights(ut[mid], ut[full:], vt[mid], vt[full:])
    u = jnp.concatenate([ut[:_HALF], u_new, ut[_LANES:full]], axis=0)
    v = jnp.concatenate([vt[:_HALF], v_new, vt[_LANES:full]], axis=0)
    return u.T, v.T, shared.T


def _output_wide(lhs_ref, rows, w_ref, lo=0, hi=None):
    hi = w_ref.shape[0] if hi is None else hi
    return _dot(lhs_ref[rows, lo:hi], w_ref[lo:hi, _LANES:])


def _output_edges(lhs_ref, rows, w_ref, s_ref):
    half = s_ref.shape[0]
    shared = _dot(lhs_ref[rows, 2 * half:], s_ref[:, :])
    v0 = _dot(lhs_ref[rows, half:2 * half], w_ref[half:, 0:_LANES])
    u0 = _dot(lhs_ref[rows, 0:half], w_ref[0:half, 0:_LANES])
    is_low = jax.lax.broadcasted_iota(jnp.int32, u0.shape, 1) < _HALF
    return u0 + jnp.where(is_low, v0, shared), v0[:, _HALF:] + shared[:, :_HALF]


def _output_finish(lhs_ref, rows, w_ref, s_ref, wide):
    first, last = _output_edges(lhs_ref, rows, w_ref, s_ref)
    return jnp.concatenate([first, wide, last], axis=1)


def _output_dot(lhs_ref, rows, w_ref, s_ref):
    first, last = _output_edges(lhs_ref, rows, w_ref, s_ref)
    return jnp.concatenate([first, _output_wide(lhs_ref, rows, w_ref), last], axis=1)


def _mask_tables(n_streams, n_mem, seg):
    tok0 = n_streams * n_mem
    rows = tok0 + n_streams * seg

    def split(axis):
        idx = jax.lax.broadcasted_iota(jnp.int32, (rows, rows), axis)
        is_mem = idx < tok0
        stream = jnp.where(is_mem, idx // n_mem, (idx - tok0) // seg)
        pos = jnp.where(is_mem, idx % n_mem, n_mem + (idx - tok0) % seg)
        return stream, pos

    q_stream, q_pos = split(0)
    k_stream, k_pos = split(1)
    same = q_stream == k_stream
    visible = same & ((q_pos < n_mem) | (q_pos >= k_pos))
    fill = jnp.where(same, _MASK_FILL, -jnp.inf).astype(_F32)
    return visible, fill


def _last_segment_mask(n_mem, seg):
    q_pos = jax.lax.broadcasted_iota(jnp.int32, (seg, seg + n_mem), 0)
    k_pos = jax.lax.broadcasted_iota(jnp.int32, (seg, seg + n_mem), 1)
    return (k_pos >= seg) | (q_pos >= k_pos), _MASK_FILL


def _kernel(xt_hbm, mem0_ref, wq_hbm, wk_hbm, wv_hbm, wot_hbm, w1_hbm, w3_hbm, w2t_hbm,
            out_hbm,
            xt_ref, x_ref, rq_ref, rk_ref, rv_ref, words_ref, wqkv_ref, wot_ref, wo_ref,
            r1_ref, r3_ref, w1_ref, w3_ref, w2t_ref, w2_ref, sqkv_ref, s1_ref, s3_ref, so_ref, s2_ref,
            o_ref, hid_ref, early_ref, a_ref, xa_ref, x1_ref, wide_ref, y_ref, in_sems, out_sems,
            *, seg, n_heads, dh):
    seq, dm = x_ref.shape
    n_mem = mem0_ref.shape[0]
    n_seg = seq // seg
    ffn = w1_ref.shape[1]
    wqkv_ref, wo_ref, w1_ref, w3_ref, w2_ref = map(
        _Packed, (wqkv_ref, wo_ref, w1_ref, w3_ref, w2_ref))
    sqkv_ref, s1_ref, s3_ref, so_ref, s2_ref = map(
        _Packed, (sqkv_ref, s1_ref, s3_ref, so_ref, s2_ref))
    o_ref, hid_ref, early_ref = map(_Packed, (o_ref, hid_ref, early_ref))
    scale = dh ** -0.5
    n_grp = n_heads // 2
    tok0 = 2 * n_mem
    full = dm - _HALF
    mid = slice(_HALF, _LANES)
    fc = _FFN_CHUNK
    xc = _XPOSE_CHUNK
    wc = ffn // _FFN_DMA_CHUNKS

    def cols(ref, start, size):
        return ref.at[:, start:start + size]

    def rows_of(ref, start, size):
        return ref.at[start:start + size, :]

    raw_rows = dm * n_heads // _QKV_DMA_CHUNKS
    transfers = [("x_head", cols(xt_hbm, 0, _LANES), cols(xt_ref, 0, _LANES))]
    for name, src, dst in (("wq", wq_hbm, rq_ref), ("wk", wk_hbm, rk_ref), ("wv", wv_hbm, rv_ref)):
        for c in range(_QKV_DMA_CHUNKS):
            transfers.append(((name, c), rows_of(src, c * raw_rows, raw_rows),
                              rows_of(dst, c * raw_rows, raw_rows)))
    transfers.append(("wo", wot_hbm, wot_ref))
    for c in range(0, ffn, wc):
        transfers.append((("w1", c), cols(w1_hbm, c, wc), cols(r1_ref, c, wc)))
        transfers.append((("w3", c), cols(w3_hbm, c, wc), cols(r3_ref, c, wc)))
    for c in range(0, ffn, wc):
        transfers.append((("w2", c), cols(w2t_hbm, c, wc), cols(w2t_ref, c, wc)))
    transfers.append(("x_tail", cols(xt_hbm, _LANES, seq - _LANES), cols(xt_ref, _LANES, seq - _LANES)))
    copies = {name: pltpu.make_async_copy(src, dst, in_sems.at[n])
              for n, (name, src, dst) in enumerate(transfers)}

    def arrive(name):
        copies[name].wait()

    def project(h, grp):
        rows = slice(grp * dm, grp * dm + full)
        both = _paired_dot(h, wqkv_ref[rows, 0:3 * dh], wqkv_ref[rows, 3 * dh:],
                           sqkv_ref[grp * _LANES:(grp + 1) * _LANES, :])
        return [[qkv[:, m * dh:(m + 1) * dh].astype(_BF16) for m in range(3)] for qkv in both]

    def probabilities(qkv, visible, fill):
        probs = []
        for q, k, _ in qkv:
            s = jnp.where(visible, _dot_nt(q[:visible.shape[0]], k) * scale, fill)
            p = jnp.exp(s - jnp.max(s, axis=-1, keepdims=True))
            probs.append((p * (1.0 / jnp.sum(p, axis=-1, keepdims=True))).astype(_BF16))
        return probs

    def heads(project_group, mask, fillers=()):
        visible, fill = mask
        rows = visible.shape[0]
        qkv, probs = {}, {}
        for t in range(n_grp + _PV_LAG):
            if t < n_grp:
                qkv[t] = project_group(t)
            elif t - n_grp < len(fillers):
                fillers[t - n_grp]()
            if 0 <= t - _PV_LAG:
                grp = t - _PV_LAG
                outs = [_dot(p, v) for p, (_, _, v) in zip(probs.pop(grp), qkv.pop(grp))]
                for part, out in enumerate(outs + [outs[0] + outs[1]]):
                    col = (part * n_grp + grp) * dh
                    o_ref[0:rows, col:col + dh] = out.astype(_BF16)
            if 0 <= t - _QK_LAG < n_grp:
                probs[t - _QK_LAG] = probabilities(qkv[t - _QK_LAG], visible, fill)

    def attend(project_group, mask):
        rows, half, wide = slice(0, mask[0].shape[0]), n_grp * dh, []
        cut_u, cut_v = (n_grp - _PV_LAG) * dh, half + (n_grp - _PV_LAG + 1) * dh

        def part(lo, hi):
            return lambda: wide.append(_output_wide(o_ref, rows, wo_ref, lo, hi))

        heads(project_group, mask, (part(0, cut_u), part(half, cut_v)))
        first, last = _output_edges(o_ref, rows, wo_ref, so_ref)
        part(cut_u, half)()
        part(cut_v, 2 * half)()
        wide = (wide[0] + wide[1]) + (wide[2] + wide[3])
        return jnp.concatenate([first, wide, last], axis=1)

    def pair_gate_up(lo, hi):
        for raw, w_ref, s_ref in ((r1_ref, w1_ref, s1_ref), (r3_ref, w3_ref, s3_ref)):
            w_ref[0:_HALF, lo:hi] = raw[0:_HALF, lo:hi]
            w_ref[_LANES:, lo:hi] = raw[_LANES:full, lo:hi]
            for c in range(lo, hi, fc):
                ca, cb = slice(c, c + fc // 2), slice(c + fc // 2, c + fc)
                w_ref[mid, ca], w_ref[mid, cb], s_ref[:, c // 2:(c + fc) // 2] = _pair_weights(
                    raw[mid, ca], raw[full:, ca], raw[mid, cb], raw[full:, cb])

    def gate_up(f_in, lo=0, hi=ffn):
        for c in range(lo, hi, fc):
            ca, cb = slice(c, c + fc // 2), slice(c + fc // 2, c + fc)
            cs = slice(c // 2, (c + fc) // 2)
            gates = _paired_dot(f_in, w1_ref[0:full, ca], w1_ref[0:full, cb], s1_ref[:, cs])
            ups = _paired_dot(f_in, w3_ref[0:full, ca], w3_ref[0:full, cb], s3_ref[:, cs])
            hids = [gate * jax.nn.sigmoid(gate) * up for gate, up in zip(gates, ups)]
            for part, hid in enumerate(hids + [hids[0] + hids[1]]):
                col = (part * ffn + c) // 2
                hid_ref[0:hid.shape[0], col:col + fc // 2] = hid.astype(_BF16)

    def stage_down(lo, hi):
        for c in range(lo, hi, fc):
            rows_u = slice(c // 2, (c + fc) // 2)
            rows_v = slice((ffn + c) // 2, (ffn + c + fc) // 2)
            w2_ref[rows_u, :], w2_ref[rows_v, :], s2_ref[rows_u, :] = _pair_output_weights(
                w2t_ref[:, c:c + fc // 2], w2t_ref[:, c + fc // 2:c + fc])

    def projector(mem, x):
        return functools.partial(project, _split_lhs(jnp.concatenate([mem, _layernorm(x)], axis=0)))

    def write_back(t, size):
        xt_ref[:, t:t + size] = y_ref[t:t + size, :].T
        copy = pltpu.make_async_copy(
            cols(xt_ref, t, size), cols(out_hbm, t, size), out_sems.at[pl.cdiv(t, xc)])
        copy.start()
        return copy

    for copy in copies.values():
        copy.start()
    arrive("x_head")
    x_ref[0:_LANES, :] = xt_ref[:, 0:_LANES].T

    d_chunk = dm // _QKV_DMA_CHUNKS
    word_rows = _XPOSE_CHUNK // 2
    for m, (name, raw_ref) in enumerate((("wq", rq_ref), ("wk", rk_ref), ("wv", rv_ref))):
        for c in range(_QKV_DMA_CHUNKS):
            arrive((name, c))

            def to_words(n, carry, c=c, raw_ref=raw_ref):
                src = pl.multiple_of(c * raw_rows + n * 2 * word_rows, 2 * word_rows)
                words_ref[pl.ds(pl.multiple_of(n * word_rows, word_rows), word_rows), :] = (
                    pltpu.bitcast(raw_ref[pl.ds(src, 2 * word_rows), :], jnp.uint32))
                return carry

            def regroup(grp, carry, m=m, c=c):
                even_d = words_ref[pl.ds(grp, d_chunk // 2, stride=n_heads), :]
                odd_d = words_ref[pl.ds(grp + n_grp, d_chunk // 2, stride=n_heads), :]
                lo = (even_d & jnp.uint32(0xFFFF)) | (odd_d << 16)
                hi = (even_d >> 16) | (odd_d & jnp.uint32(0xFFFF0000))
                row = pl.multiple_of(grp * (dm // 2) + c * (d_chunk // 2), 8)
                for half, val in enumerate((lo, hi)):
                    col = (half * 3 + m) * dh
                    wqkv_ref.ref[pl.ds(row, d_chunk // 2), col:col + dh] = val
                return carry

            jax.lax.fori_loop(0, raw_rows // (2 * word_rows), to_words, 0, unroll=4)
            jax.lax.fori_loop(0, n_grp, regroup, 0)

    def pair_heads(grp, carry):
        ca, cb = slice(0, 3 * dh), slice(3 * dh, 6 * dh)
        mid_rows, tail_rows = (grp * dm + _HALF, _HALF), (grp * dm + full, _HALF)
        (wqkv_ref[mid_rows, ca], wqkv_ref[mid_rows, cb],
         sqkv_ref[(grp * _LANES, _LANES), :]) = _pair_weights(
             wqkv_ref[mid_rows, ca], wqkv_ref[tail_rows, ca],
             wqkv_ref[mid_rows, cb], wqkv_ref[tail_rows, cb])
        return carry

    jax.lax.fori_loop(0, n_grp, pair_heads, 0)

    mem0 = mem0_ref[...].astype(_F32)
    a_ref[0:n_mem, :] = mem0

    def first_segments(s, carry):
        x_s = x_ref[pl.ds(pl.multiple_of(s * seg, seg), seg), :].astype(_F32)
        heads(projector(a_ref[0:n_mem, :], x_s), _mask_tables(1, n_mem, seg))

        @pl.when(s == 0)
        def _():
            arrive("wo")

            def stage_wo(grp, carry):
                rows_u, rows_v = (grp * dh, dh), ((n_grp + grp) * dh, dh)
                wo_ref[rows_u, :], wo_ref[rows_v, :], so_ref[rows_u, :] = _pair_output_weights(
                    wot_ref[2 * grp], wot_ref[2 * grp + 1])
                return carry

            jax.lax.fori_loop(0, n_grp, stage_wo, 0, unroll=2)

        a = _output_dot(o_ref, slice(0, n_mem + seg), wo_ref, so_ref)
        a_ref[0:n_mem, :] = a[:n_mem]
        a_ref[pl.ds(pl.multiple_of(tok0 + (1 - s) * seg, n_mem), seg), :] = a[n_mem:]
        return carry

    jax.lax.fori_loop(0, 2, first_segments, 0)
    a_ref[n_mem:tok0, :] = mem0
    x1 = jnp.concatenate([x_ref[seg:2 * seg, :], x_ref[0:seg, :]], axis=0).astype(_F32)
    x1 = x1 + a_ref[tok0:, :]
    x1_ref[...] = x1
    f_in = _split_lhs(_layernorm(x1))
    for c in range(0, ffn, wc):
        arrive(("w1", c))
        arrive(("w3", c))
        pair_gate_up(c, c + wc)
        gate_up(f_in, c, c + wc)
    both = slice(0, 2 * seg)
    x_s2 = x_ref[2 * seg:3 * seg, :].astype(_F32)
    project_early = projector(a_ref[0:tok0, :], x_s2)
    wide = None
    for n, c in enumerate(range(0, ffn, wc)):
        for grp in range(n * n_grp // _FFN_DMA_CHUNKS, (n + 1) * n_grp // _FFN_DMA_CHUNKS):
            early = [m for qkv in project_early(grp) for m in qkv]
            early_ref[:, grp * 6 * dh:(grp + 1) * 6 * dh] = jnp.concatenate(early, axis=1)
        arrive(("w2", c))
        stage_down(c, c + wc)
        for lo in (c // 2, (ffn + c) // 2):
            part = _output_wide(hid_ref, both, w2_ref, lo, lo + wc // 2)
            wide = part if wide is None else wide + part
    wide_ref[...] = wide
    x2_s0 = x1_ref[seg:, :] + _output_finish(
        hid_ref, slice(seg, 2 * seg), w2_ref, s2_ref, wide[seg:])
    xa_ref[...] = jnp.concatenate([x_s2, x2_s0], axis=0)
    late_rows = _split_lhs(_layernorm(x2_s0))

    def project_first(grp):
        if grp == _X_TAIL_GROUP:
            arrive("x_tail")
            for t in range(_LANES, seq, xc):
                end = min(t + xc, seq)
                x_ref[t:end, :] = xt_ref[:, t:end].T
        return [[jnp.concatenate([early_ref[:, ((grp * 2 + hh) * 3 + m) * dh:
                                            ((grp * 2 + hh) * 3 + m + 1) * dh], late], axis=0)
                 for m, late in enumerate(qkv)]
                for hh, qkv in enumerate(project(late_rows, grp))]

    a_ref[...] = attend(project_first, _mask_tables(2, n_mem, seg))

    def feed_forward(out_row):
        y = x1_ref[...] + _output_finish(hid_ref, both, w2_ref, s2_ref, wide_ref[...])
        y_ref[pl.ds(out_row, seg), :] = y[seg:].astype(y_ref.dtype)
        x1 = xa_ref[...] + a_ref[tok0:, :]
        x1_ref[...] = x1
        gate_up(_split_lhs(_layernorm(x1)))
        return y[:seg]

    def step(i, carry):
        x2 = feed_forward(pl.multiple_of(jnp.maximum(i - 3, 0) * seg, seg))
        wide_ref[...] = _output_wide(hid_ref, both, w2_ref)
        x_next = x_ref[pl.ds(pl.multiple_of((i + 1) * seg, seg), seg), :].astype(_F32)
        xa = jnp.concatenate([x_next, x2], axis=0)
        xa_ref[...] = xa
        a_ref[...] = attend(projector(a_ref[0:tok0, :], xa), _mask_tables(2, n_mem, seg))
        return carry

    jax.lax.fori_loop(2, n_seg - 1, step, 0)

    x_s0 = feed_forward(seq - 4 * seg)
    a = attend(projector(a_ref[n_mem:tok0, :], x_s0), _mask_tables(1, n_mem, seg))
    y = x1_ref[...] + _output_dot(hid_ref, both, w2_ref, s2_ref)
    y_ref[seq - 3 * seg:seq - 2 * seg, :] = y[seg:].astype(y_ref.dtype)
    x1_s0 = x_s0 + a[n_mem:]
    last = seq - _LANES
    writes = [write_back(t, min(xc, last - t)) for t in range(0, last, xc)]
    h_last = _split_lhs(jnp.concatenate([_layernorm(y[:seg]), a[:n_mem]], axis=0))
    a = attend(functools.partial(project, h_last), _last_segment_mask(n_mem, seg))
    x1 = jnp.concatenate([x1_s0, y[:seg] + a], axis=0)
    gate_up(_split_lhs(_layernorm(x1)))
    y_ref[seq - 2 * seg:, :] = (x1 + _output_dot(hid_ref, both, w2_ref, s2_ref)).astype(y_ref.dtype)
    writes.append(write_back(last, _LANES))
    for copy in writes:
        copy.wait()


@functools.partial(jax.jit, static_argnames=("A_seg_len",))
def pallas_interleave_layers__memory_aug_recurrent_mem_tr__glu_gated_swiglu__prompt_kernel(
    A_x: jax.Array,
    A_mem0: jax.Array,
    A_Wq: jax.Array,
    A_Wk: jax.Array,
    A_Wv: jax.Array,
    A_Wo: jax.Array,
    A_seg_len: int,
    B_x: jax.Array,
    B_w1: jax.Array,
    B_w3: jax.Array,
    B_w2: jax.Array,
):
    del B_x
    batch, seq, dm = A_x.shape
    _, n_heads, dh = A_Wq.shape
    n_mem = A_mem0.shape[1]
    ffn = B_w1.shape[1]
    seg = int(A_seg_len)
    assert batch == 1 and seq % _XPOSE_CHUNK == 0
    assert _LANES % seg == 0 and _LANES >= 3 * seg
    assert dm % _LANES == _HALF and dh == _LANES and n_heads // 2 > _X_TAIL_GROUP
    assert ffn % (_FFN_DMA_CHUNKS * _FFN_CHUNK) == 0
    rows = 2 * (n_mem + seg)
    full = dm - _HALF

    vmem = pl.BlockSpec(memory_space=pltpu.VMEM)
    hbm = pl.BlockSpec(memory_space=pltpu.HBM)
    out_t = pl.pallas_call(
        functools.partial(_kernel, seg=seg, n_heads=n_heads, dh=dh),
        out_shape=jax.ShapeDtypeStruct((dm, seq), A_x.dtype),
        in_specs=[hbm, vmem] + [hbm] * 7,
        out_specs=hbm,
        scratch_shapes=[
            pltpu.VMEM((dm, seq), _BF16),
            pltpu.VMEM((seq, dm), _BF16),
            pltpu.VMEM((dm * n_heads, dh), _BF16),
            pltpu.VMEM((dm * n_heads, dh), _BF16),
            pltpu.VMEM((dm * n_heads, dh), _BF16),
            _packed_scratch((dm // _QKV_DMA_CHUNKS + 2) * n_heads, dh),
            _packed_scratch(n_heads // 2 * dm, 6 * dh),
            pltpu.VMEM((n_heads, dm, dh), _BF16),
            _packed_scratch(n_heads * dh, full),
            pltpu.VMEM((dm, ffn), _BF16),
            pltpu.VMEM((dm, ffn), _BF16),
            _packed_scratch(full, ffn),
            _packed_scratch(full, ffn),
            pltpu.VMEM((dm, ffn), _BF16),
            _packed_scratch(ffn, full),
            _packed_scratch(n_heads // 2 * _LANES, 3 * dh),
            _packed_scratch(_LANES, ffn // 2),
            _packed_scratch(_LANES, ffn // 2),
            _packed_scratch(n_heads * dh // 2, _LANES),
            _packed_scratch(ffn // 2, _LANES),
            _packed_scratch(rows, n_heads * dh * 3 // 2),
            _packed_scratch(2 * seg, ffn * 3 // 2),
            _packed_scratch(rows - seg, 3 * n_heads * dh),
            pltpu.VMEM((rows, dm), _F32),
            pltpu.VMEM((2 * seg, dm), _F32),
            pltpu.VMEM((2 * seg, dm), _F32),
            pltpu.VMEM((2 * seg, dm - _HALF - _LANES), _F32),
            pltpu.VMEM((seq, dm), _BF16),
            pltpu.SemaphoreType.DMA((3 + 3 * _QKV_DMA_CHUNKS + 3 * _FFN_DMA_CHUNKS,)),
            pltpu.SemaphoreType.DMA((seq // _XPOSE_CHUNK + 1,)),
        ],
        compiler_params=pltpu.CompilerParams(vmem_limit_bytes=110 * 1024 * 1024),
    )(
        A_x.reshape(seq, dm).T,
        A_mem0.reshape(n_mem, dm),
        A_Wq.reshape(dm * n_heads, dh),
        A_Wk.reshape(dm * n_heads, dh),
        A_Wv.reshape(dm * n_heads, dh),
        A_Wo.transpose(0, 2, 1),
        B_w1,
        B_w3,
        B_w2.T,
    )
    return out_t.T.reshape(batch, seq, dm)
```
